```python
import jax
import jax.numpy as jnp

def _softmax(x, axis=-1):
    return jax.nn.softmax(x, axis=axis)
def _gelu(x):
    return jax.nn.gelu(x, approximate=True)
def _silu(x):
    return jax.nn.silu(x)
def _sigmoid(x):
    return jax.nn.sigmoid(x)
def _layernorm(x, axis=-1, eps=1e-5):
    m = jnp.mean(x, axis=axis, keepdims=True)
    v = jnp.var(x, axis=axis, keepdims=True)
    return (x - m) / jnp.sqrt(v + eps)
def _scatter_add(tgt, idx, src, axis=0):
    return tgt.at[idx].add(src)
def _segment_sum(src, seg, n):
    return jax.ops.segment_sum(src, seg, n)
class _Rng:
    def __init__(self, key):
        self._k = key
    def _next(self):
        self._k, sub = jax.random.split(self._k)
        return sub
    def normal(self, shape):
        return jax.random.normal(self._next(), shape, dtype=jnp.bfloat16)
    def randint(self, lo, hi, shape):
        return jax.random.randint(self._next(), shape, lo, hi, dtype=jnp.int32)
    def uniform(self, shape, lo=0.0, hi=1.0):
        return jax.random.uniform(self._next(), shape, jnp.bfloat16, lo, hi)
    def permutation(self, n):
        return jax.random.permutation(self._next(), n)


kernel_name = 'concat_heads__compressed_kv_cla__spectral_gfnet__prompt'

def setup_inputs():
    _rng = _Rng(jax.random.key(int.from_bytes(__import__("os").urandom(4), "little")))
    _w = (lambda a: (lambda t: t.astype(jnp.bfloat16) if jnp.issubdtype(t.dtype, jnp.floating) else t)(jnp.asarray(a)))
    def _A_setup():
        B, H, Sq, Sk, D, M = 1, 32, 2048, 2048, 128, 1024
        Dc = 4 * D
        return {
            "x": _w((lambda *s: _rng.normal(s) * 0.05)(B, Sq, M)),
            "c_kv": _w((lambda *s: _rng.normal(s) * 0.05)(B, Sk, Dc)),
            "w_q": _w((lambda *s: _rng.normal(s) * 0.05)(M, H, D) * (M ** -0.5)),
            "w_uk": _w((lambda *s: _rng.normal(s) * 0.05)(Dc, H, D) * (Dc ** -0.5)),
            "w_uv": _w((lambda *s: _rng.normal(s) * 0.05)(Dc, H, D) * (Dc ** -0.5)),
            "w_o": _w((lambda *s: _rng.normal(s) * 0.05)(H, D, M) * ((H * D) ** -0.5)),
        }
    _A_in = _A_setup()

    def _B_setup():
        B, S, D = 1, 2048, 1024
        Df = D // 2 + 1
        return {
            "x": _w((lambda *s: _rng.normal(s) * 0.05)(B, S, D)),
            "w_r": _w((lambda *s: _rng.normal(s) * 0.05)(S, Df) * 0.02),
            "w_i": _w((lambda *s: _rng.normal(s) * 0.05)(S, Df) * 0.02),
        }
    _B_in = _B_setup()

    return {
        "A_x": _A_in["x"],
        "A_c_kv": _A_in["c_kv"],
        "A_w_q": _A_in["w_q"],
        "A_w_uk": _A_in["w_uk"],
        "A_w_uv": _A_in["w_uv"],
        "A_w_o": _A_in["w_o"],
        "B_x": _B_in["x"],
        "B_w_r": _B_in["w_r"],
        "B_w_i": _B_in["w_i"],
    }

def reference(A_x, A_c_kv, A_w_q, A_w_uk, A_w_uv, A_w_o, B_x, B_w_r, B_w_i):
    def _A_ref(x, c_kv, w_q, w_uk, w_uv, w_o):
        B, Sq, M = x.shape[0], x.shape[1], x.shape[2]
        Sk = c_kv.shape[1]
        H, D = w_q.shape[1], w_q.shape[2]
        q = jnp.einsum("bqm,mhd->bhqd", x, w_q)
        k = jnp.einsum("bkc,chd->bhkd", c_kv, w_uk)
        v = jnp.einsum("bkc,chd->bhkd", c_kv, w_uv)
        scores = jnp.einsum("bhqd,bhkd->bhqk", q, k) * (D ** -0.5)
        off = Sk - Sq
        qi = jnp.arange(Sq)[:, None]
        kj = jnp.arange(Sk)[None, :]
        cmask = kj <= (qi + off)
        scores = jnp.where(cmask[None, None], scores, -1e9)
        p = _softmax(scores, axis=-1)
        ctx = jnp.einsum("bhqk,bhkd->bhqd", p, v)
        return jnp.einsum("bhqd,hdm->bqm", ctx, w_o)

    def _B_ref(x, w_r, w_i):
        B, S, D = x.shape
        X = (lambda x, axes=(-2,-1): jnp.fft.rfft2(x.astype(jnp.float32), axes=axes))(x, axes=(-2, -1))
        W = w_r + 1j * w_i
        X = X * W
        y = (lambda x, s, axes=(-2,-1): jnp.fft.irfft2(x, s=s, axes=axes).astype(jnp.bfloat16))(X, (S, D), axes=(-2, -1))
        return y

    a = _A_ref(A_x, A_c_kv, A_w_q, A_w_uk, A_w_uv, A_w_o)
    b = _B_ref(B_x, B_w_r, B_w_i)
    return jnp.concatenate([a, b], axis=-1)
```

```python
import functools

import numpy as np
import jax
import jax.numpy as jnp
import jax.experimental.pallas as pl
import jax.experimental.pallas.tpu as pltpu

S = 2048
M = 1024
H = 32
HD = 128
DC = 512
BD = 1024
NG = 8

_U32 = jnp.uint32
_BF16 = jnp.bfloat16
_F32 = jnp.float32
_NT = (((1,), (1,)), ((), ()))
_QSCALE = float(HD ** -0.5 * np.log2(np.e))
_MASKED = -1e9


def _to_bf16_bits(a):
    u = np.ascontiguousarray(a, dtype=np.float32).view(np.uint32).astype(np.uint64)
    r = (u + 0x7FFF + ((u >> 16) & 1)) >> 16
    return r.astype(np.uint32) & 0xFFFF


def _pack_rows(a):
    b = _to_bf16_bits(a)
    return (b[0::2] | (b[1::2] << 16)).astype(np.uint32)


def _neg(p):
    return None if p is None else (-p[0], p[1])


def _add(p, q):
    if p is None:
        return q
    if q is None:
        return p
    if p[0] == q[0]:
        return (p[0], p[1] + q[1])
    if p[0] > 0:
        return (1, p[1] - q[1])
    return (1, q[1] - p[1])


def _sub(p, q):
    return _add(p, _neg(q))


def _scale(p, f):
    if p is None:
        return None
    return (p[0] * (1 if f > 0 else -1), p[1] * abs(f))


def _cadd(x, y):
    return (_add(x[0], y[0]), _add(x[1], y[1]))


def _csub(x, y):
    return (_sub(x[0], y[0]), _sub(x[1], y[1]))


def _cmul_i(x, s):
    return (_neg(x[1]), x[0]) if s > 0 else (x[1], _neg(x[0]))


def _cmul_w(x, n, sgn):
    n = n % 16
    if n == 0:
        return x
    if n == 4:
        return _cmul_i(x, sgn)
    if n == 8:
        return (_neg(x[0]), _neg(x[1]))
    if n == 12:
        return _cmul_i(x, -sgn)
    wr = float(np.cos(2 * np.pi * n / 16))
    wi = float(sgn * np.sin(2 * np.pi * n / 16))
    re, im = x
    if n % 2 == 0:
        r = abs(wr)
        sr = 1 if wr > 0 else -1
        si = 1 if wi > 0 else -1
        a = _sub(re if sr > 0 else _neg(re), im if si > 0 else _neg(im))
        b = _add(re if si > 0 else _neg(re), im if sr > 0 else _neg(im))
        return (_scale(a, r), _scale(b, r))
    return (_sub(_scale(re, wr), _scale(im, wi)), _add(_scale(re, wi), _scale(im, wr)))


def _dft4(x0, x1, x2, x3, sgn):
    s02, d02 = _cadd(x0, x2), _csub(x0, x2)
    s13, d13 = _cadd(x1, x3), _csub(x1, x3)
    r = _cmul_i(d13, sgn)
    return [_cadd(s02, s13), _cadd(d02, r), _csub(s02, s13), _csub(d02, r)]


def _fft16(xs, sgn):
    t = [_dft4(xs[a0], xs[4 + a0], xs[8 + a0], xs[12 + a0], sgn) for a0 in range(4)]
    t = [[_cmul_w(t[a0][j0], a0 * j0, sgn) for j0 in range(4)] for a0 in range(4)]
    out = [None] * 16
    for j0 in range(4):
        r = _dft4(t[0][j0], t[1][j0], t[2][j0], t[3][j0], sgn)
        for j1 in range(4):
            out[j0 + 4 * j1] = r[j1]
    return out


def _net_signs(sgn):
    out = _fft16([((1, 1.0), (1, 1.0)) for _ in range(16)], sgn)
    return [(o[0][0], o[1][0]) for o in out]


_INV_SIGNS = _net_signs(+1)
_CLS = ((0, 4), (1, 7), (2, 6), (3, 5))
_R2 = float(np.sqrt(0.5))


def _build_consts():
    n2 = np.arange(128)
    kap = np.arange(64)

    def wl(l):
        return np.exp(-2j * np.pi * np.outer(l, n2) / 1024)

    fc = np.zeros((4, 256, 256))
    w = wl(8 * kap)
    fc[0, 0:64, 0:128] = w.real
    fc[0, 64:128, 0:128] = w.imag
    fc[0, 64, 0:128] = (-1.0) ** n2
    w = wl(4 + 8 * kap)
    fc[0, 0:64, 128:256] = w.real
    fc[0, 64:128, 128:256] = w.imag
    for j in (1, 2, 3):
        si = 1.0 if j == 3 else -1.0
        w1, w2 = wl(j + 8 * kap), wl(8 - j + 8 * kap)
        fc[j, 0:64, 0:128], fc[j, 0:64, 128:] = w1.real, -w1.imag * si
        fc[j, 64:128, 0:128], fc[j, 64:128, 128:] = w2.real, w2.imag * si
        fc[j, 128:192, 0:128], fc[j, 128:192, 128:] = w1.imag, w1.real * si
        fc[j, 192:256, 0:128], fc[j, 192:256, 128:] = w2.imag, -w2.real * si

    def cs(l, c):
        ph = 2 * np.pi * np.outer(l, n2) / 1024
        return c[:, None] * np.cos(ph) / 1024, c[:, None] * np.sin(ph) / 1024

    ic = np.zeros((4, 256, 256))
    two = np.full(64, 2.0)
    co, si = cs(8 * kap, np.where(kap == 0, 1.0, 2.0))
    ic[0, 0:64, 0:128], ic[0, 128:192, 0:128] = co, -si
    ic[0, 128, 0:128] = (-1.0) ** n2 / 1024
    co, si = cs(4 + 8 * kap, two)
    ic[0, 64:128, 128:], ic[0, 192:256, 128:] = co, -si
    for j in (1, 2, 3):
        co, si = cs(j + 8 * kap, two)
        ic[j, 0:64, 0:128], ic[j, 128:192, 0:128] = co, -si
        ic[j, 0:64, 128:], ic[j, 128:192, 128:] = si, co
        co, si = cs(8 - j + 8 * kap, two)
        ic[j, 64:128, 0:128], ic[j, 192:256, 0:128] = co, -si
        ic[j, 64:128, 128:], ic[j, 192:256, 128:] = -si, -co

    gf = np.zeros((16, 256, 256))
    for ap in range(16):
        g = np.exp(-2j * np.pi * (16 * np.outer(n2, n2) + ap * n2[None, :]) / 2048)
        gf[ap] = np.block([[g.real, g.imag], [-g.imag, g.real]])

    def pk(m):
        return np.stack([_pack_rows(x) for x in m])

    return pk(fc), pk(ic / 2048), pk(gf)


_FC, _IC, _GF = _build_consts()
assert all(sg == (1, 1) for sg in _INV_SIGNS)


def _bf(x_u32):
    return pltpu.bitcast(x_u32, _BF16)


def _pk(x_f32):
    return pltpu.bitcast(x_f32.astype(_BF16), _U32)


def _dot(a, b):
    return jnp.dot(a, b, preferred_element_type=_F32)


def _val(p, like):
    if p is None:
        return jnp.zeros_like(like)
    return p[1] if p[0] > 0 else -p[1]


def _attention(q, k, v, bq):
    outs = []
    row = jax.lax.broadcasted_iota(jnp.int32, (128, 128), 0)
    col = jax.lax.broadcasted_iota(jnp.int32, (128, 128), 1)
    causal = col <= row
    for i in range(S // bq):
        q0 = i * bq
        qq = q[q0:q0 + bq]
        nt = (q0 + bq) // 128
        mx = None
        ss = []
        for j in range(nt):
            r0 = max(0, j * 128 - q0)
            s = jax.lax.dot_general(qq[r0:], k[j * 128:(j + 1) * 128], _NT,
                                    preferred_element_type=_F32)
            if j * 128 >= q0:
                sd = jnp.where(causal, s[:128], _MASKED)
                s = jnp.concatenate([sd, s[128:]], axis=0) if s.shape[0] > 128 else sd
            ss.append(s)
            if mx is None:
                mx = s
            elif r0 == 0:
                mx = jnp.maximum(mx, s)
            else:
                mx = jnp.concatenate([mx[:r0], jnp.maximum(mx[r0:], s)], axis=0)
        m = jnp.max(mx, axis=1, keepdims=True)
        acc = None
        lsum = None
        for j in range(nt):
            r0 = max(0, j * 128 - q0)
            p = jnp.exp2(ss[j] - m[r0:])
            pv = _dot(p.astype(_BF16), v[j * 128:(j + 1) * 128])
            if acc is None:
                acc, lsum = pv, p
            elif r0 == 0:
                acc, lsum = acc + pv, lsum + p
            else:
                acc = jnp.concatenate([acc[:r0], acc[r0:] + pv], axis=0)
                lsum = jnp.concatenate([lsum[:r0], lsum[r0:] + p], axis=0)
        l = jnp.sum(lsum, axis=1, keepdims=True)
        outs.append(acc / l)
    return outs


def _kernel(flag_ref, x_hbm, c_hbm, wq_hbm, wk_hbm, wv_hbm, wo_hbm, bx_hbm, wr_hbm, wi_hbm,
            fc_hbm, ic_hbm, gf_hbm,
            out_hbm,
            x_s, c_s, wo_s, wq_s, wk_s, wv_s, ctx_s, oa_s,
            bx_s, wr_s, wi_s, wnr_s, wni_s, fc_s, ic_s, gf_s, x1_s, nq_s, v_s, ob_s, u0_s, u1_s, u2_s, u3_s, q0_s, q1_s, vc_s,
            sem_bx, sem_misc, sem_w, sem_pair, sem_ob, sem_oa, *, bq, do_a, do_b, rg_rows, n_pre):
    xh = x_hbm.bitcast(_U32)
    ch = c_hbm.bitcast(_U32)
    wqh = wq_hbm.bitcast(_U32)
    wkh = wk_hbm.bitcast(_U32)
    wvh = wv_hbm.bitcast(_U32)
    woh = wo_hbm.bitcast(_U32)
    bxh = bx_hbm.bitcast(_U32)
    wrh = wr_hbm.at[pl.ds(0, 512)].bitcast(_U32)
    wih = wi_hbm.at[pl.ds(0, 512)].bitcast(_U32)
    outh = out_hbm.bitcast(_U32)

    def bx_cp(p, par):
        return pltpu.make_async_copy(bxh.at[:, par * 8 + p], bx_s.at[p, par], sem_bx.at[2 * p + par])

    def w_cp(j, which):
        src, dst = (wrh, wr_s) if which == 0 else (wih, wi_s)
        return pltpu.make_async_copy(src.at[:, pl.ds(128 * j, 128)], dst.at[j], sem_w.at[2 * j + which])

    fc_cp = pltpu.make_async_copy(fc_hbm, fc_s, sem_misc.at[0])
    ic_cp = pltpu.make_async_copy(ic_hbm, ic_s, sem_misc.at[1])
    wnr_cp = pltpu.make_async_copy(wr_hbm.at[pl.ds(512, 1)], wnr_s, sem_misc.at[2])
    gf_cp = pltpu.make_async_copy(gf_hbm, gf_s, sem_misc.at[3])
    x_cp = pltpu.make_async_copy(xh, x_s, sem_misc.at[5])
    c_cp = pltpu.make_async_copy(ch, c_s, sem_misc.at[6])
    wo_cp = pltpu.make_async_copy(woh, wo_s, sem_misc.at[7])
    wni_cp = pltpu.make_async_copy(wi_hbm.at[pl.ds(512, 1)], wni_s, sem_misc.at[8])

    def pair_cps(p, slot):
        cps = []
        for i, (src, dst) in enumerate(((wqh, wq_s), (wkh, wk_s), (wvh, wv_s))):
            for par in range(2):
                cps.append(pltpu.make_async_copy(
                    src.at[:, par * 16 + p], dst.at[slot, par], sem_pair.at[slot * 6 + 2 * i + par]))
        return cps

    if do_b:
        bx_cp(0, 0).start()
        bx_cp(0, 1).start()
        fc_cp.start()
        for p in range(1, 8):
            bx_cp(p, 0).start()
            bx_cp(p, 1).start()
        gf_cp.start()
        wnr_cp.start()
        wni_cp.start()
        for j in range(16):
            w_cp(j, 0).start()
            w_cp(j, 1).start()
        ic_cp.start()
    if do_a:
        x_cp.start()
        c_cp.start()
        for cp in pair_cps(0, 0):
            cp.start()
        wo_cp.start()

    fence = flag_ref[0] > 0

    if do_b:
        lane0 = jax.lax.broadcasted_iota(jnp.int32, (1, 128), 1) == 0
        row0 = jax.lax.broadcasted_iota(jnp.int32, (8, 128), 0) == 0

        fc_cp.wait()

        def b1_body(p, carry):
            bx_cp(p, 0).wait()
            bx_cp(p, 1).wait()
            for h in range(2):
                halves = []
                for par in range(2):
                    xf = pltpu.unpack_elementwise(bx_s[p, par], index=h, packed_dtype=_BF16,
                                                  unpacked_dtype=_F32)
                    xs = [xf[:, 128 * n:128 * (n + 1)] for n in range(8)]
                    a_, b_ = xs[0] + xs[4], xs[0] - xs[4]
                    c_, d_ = xs[2] + xs[6], xs[2] - xs[6]
                    e_, f_ = xs[1] + xs[5], xs[1] - xs[5]
                    g_, h_ = xs[3] + xs[7], xs[3] - xs[7]
                    u_ = (f_ - h_) * _R2
                    v_ = (f_ + h_) * _R2
                    ac, eg = a_ + c_, e_ + g_
                    halves.append([ac + eg, ac - eg, b_ + u_, d_ + v_, a_ - c_, e_ - g_, b_ - u_, d_ - v_])
                pln = [_bf(pltpu.pack_elementwise([halves[0][i], halves[1][i]], packed_dtype=_BF16))
                       for i in range(8)]
                ap = 2 * p + h
                f0 = _bf(fc_s[0, pl.ds(0, 64), :])
                o0 = jax.lax.dot_general(f0[:, 0:128], pln[0], _NT, preferred_element_type=_F32)
                o4 = jax.lax.dot_general(f0[:, 128:256], pln[1], _NT, preferred_element_type=_F32)
                nq = jnp.where(row0, o0[64:72], 0.0)
                im = jnp.concatenate([jnp.where(row0, 0.0, o0[64:72]), o0[72:128], o4[64:128]], axis=0)
                re = jnp.concatenate([o0[0:64], o4[0:64]], axis=0)
                nq_s[ap] = _pk(jnp.concatenate([nq, jnp.zeros_like(nq)], axis=0))
                x1_s[ap, 0] = jnp.concatenate([_pk(re), _pk(im)], axis=1)
                for j in (1, 2, 3):
                    rhs = jnp.concatenate([pln[2 * j], pln[2 * j + 1]], axis=1)
                    o = jax.lax.dot_general(_bf(fc_s[j]), rhs, _NT, preferred_element_type=_F32)
                    x1_s[ap, j] = jnp.concatenate([_pk(o[0:128]), _pk(o[128:256])], axis=1)
            return carry

        jax.lax.fori_loop(0, 8, b1_body, 0)

        gf_cp.wait()

        def spectral(us, w_of):
            xs = _fft16(us, -1)
            qs = []
            for j in range(16):
                (sr, xr), (si, xi) = xs[j]
                wr, wi = w_of(j)
                qs.append((_sub((sr, xr * wr), (si, xi * wi)), _add((sr, xr * wi), (si, xi * wr))))
            res = _fft16(qs, +1)
            assert all(r[0][0] == 1 and r[1][0] == 1 for r in res)
            return [(r[0][1], r[1][1]) for r in res]

        u_s, q_s = (u0_s, u1_s, u2_s, u3_s), (q0_s, q1_s)

        def s_fwd(t, ap):
            u_s[t][ap] = _dot(_bf(x1_s[ap, t]), _bf(gf_s[ap]))

        def filt(t, half, ii):
            cls = _CLS[t][half]
            r0 = pl.multiple_of(64 * half + 16 * ii, 16)
            rows = pl.ds(r0, 16)
            wbase = pl.ds(pl.multiple_of(64 * ii, 64), 64)

            def w_of(j):
                return tuple(pltpu.unpack_elementwise(
                    ws.at[j, wbase][pl.ds(cls // 2, 16, stride=4), :], index=cls % 2,
                    packed_dtype=_BF16, unpacked_dtype=_F32) for ws in (wr_s, wi_s))

            res = spectral([((1, u_s[t][ap, rows, pl.ds(0, 128)]), (1, u_s[t][ap, rows, pl.ds(128, 128)]))
                            for ap in range(16)], w_of)
            qrows = pl.ds(pl.multiple_of(32 * half + 8 * ii, 8), 8)
            for ap in range(16):
                q_s[t % 2][ap, qrows, :] = jnp.concatenate([_pk(res[ap][0]), _pk(res[ap][1])], axis=1)

        def s_inv(t, ap):
            o = jax.lax.dot_general(_bf(gf_s[ap]), _bf(q_s[t % 2][ap]), _NT, preferred_element_type=_F32)
            vi = o[128:256]
            if t == 0:
                vi = jnp.where(lane0, vc_s[ap], vi)
            v_s[ap, t] = jnp.concatenate([_pk(o[0:128]), _pk(vi)], axis=1)

        def nyquist():
            un = [_dot(_bf(nq_s[ap]), _bf(gf_s[ap, pl.ds(0, 64), :])) for ap in range(16)]
            wnr = wnr_s[...].astype(_F32)
            wni = wni_s[...].astype(_F32)
            qn = spectral([((1, u[:, 0:128]), (1, u[:, 128:256])) for u in un],
                          lambda j: (wnr[:, 128 * j:128 * (j + 1)], wni[:, 128 * j:128 * (j + 1)]))
            for ap in range(16):
                lhs = jnp.concatenate([qn[ap][0], qn[ap][1]], axis=1).astype(_BF16)
                vn = jax.lax.dot_general(lhs, _bf(gf_s[ap, pl.ds(0, 64), :]), _NT,
                                         preferred_element_type=_F32)
                vn = jnp.concatenate([vn, jnp.zeros((112, 128), _F32)], axis=0)
                vc_s[ap] = vn.T

        def b2_head():
            for t in range(4):
                for ap in range(16):
                    s_fwd(t, ap)

        pl.when(fence)(b2_head)
        wnr_cp.wait()
        wni_cp.wait()
        pl.when(fence)(nyquist)
        for j in range(16):
            w_cp(j, 0).wait()
            w_cp(j, 1).wait()
        for t in range(4):
            for half in range(2):
                def body(ii, carry, t=t, half=half):
                    filt(t, half, ii)
                    if t > 0:
                        for k in range(2):
                            s_inv(t - 1, 8 * half + 2 * ii + k)
                    return carry

                jax.lax.fori_loop(0, 4, body, 0)

        def b2_tail():
            for ap in range(16):
                s_inv(3, ap)

        pl.when(fence)(b2_tail)

        ic_cp.wait()

        def ob_cp(p):
            return pltpu.make_async_copy(ob_s.at[p], outh.at[:, p, pl.ds(1024, 1024)], sem_ob.at[p])

        for p in range(8):
            ys = []
            for h in range(2):
                ap = 2 * p + h
                cc = [_dot(_bf(v_s[ap, t]), _bf(ic_s[t])) for t in range(4)]
                c0, c4 = cc[0][:, 0:128], cc[0][:, 128:256]
                c1r, c1i = cc[1][:, 0:128], cc[1][:, 128:256]
                c2r, c2i = cc[2][:, 0:128], cc[2][:, 128:256]
                c3r, c3i = cc[3][:, 0:128], cc[3][:, 128:256]
                pp, mm = c0 + c4, c0 - c4
                u1, u2, u3, u4 = c1r + c3r, c1i - c3i, c1r - c3r, c1i + c3i
                t1, t2 = (u3 - u4) * _R2, (u3 + u4) * _R2
                e0, e1, e2, e3 = pp + c2r, pp - c2r, mm - c2i, mm + c2i
                ys.append([e0 + u1, e2 + t1, e1 - u2, e3 - t2, e0 - u1, e2 - t1, e1 + u2, e3 + t2])
            ob_s[p] = jnp.concatenate([pltpu.pack_elementwise([ys[0][n], ys[1][n]], packed_dtype=_BF16)
                                       for n in range(8)], axis=1)
            ob_cp(p).start()

    if do_a:
        x_cp.wait()
        c_cp.wait()

        def a_body(p, carry):
            slot = p % 2
            for cp in pair_cps(p, slot):
                cp.wait()

            @pl.when(p + 1 < H // 2)
            def _():
                for cp in pair_cps(p + 1, 1 - slot):
                    cp.start()

            def split(ref):
                a = ref[slot, 0]
                b = ref[slot, 1]
                lo = pltpu.pack_elementwise([a, b], packed_dtype=jnp.uint16)
                hi = pltpu.pack_elementwise([a >> 16, b >> 16], packed_dtype=jnp.uint16)
                return _bf(lo), _bf(hi)

            wq0, wq1 = split(wq_s)
            wk0, wk1 = split(wk_s)
            wv0, wv1 = split(wv_s)
            x = _bf(x_s[...])
            cc = _bf(c_s[...])
            q2 = _dot(x, jnp.concatenate([wq0, wq1], axis=1)) * _QSCALE
            kv = _dot(cc, jnp.concatenate([wk0, wk1, wv0, wv1], axis=1))
            ctxs = []
            for t in range(2):
                q = q2[:, t * 128:(t + 1) * 128].astype(_BF16)
                k = kv[:, t * 128:(t + 1) * 128].astype(_BF16)
                v = kv[:, 256 + t * 128:256 + (t + 1) * 128].astype(_BF16)
                outs = _attention(q, k, v, bq)
                ctxs.append(_pk(jnp.concatenate(outs, axis=0)))
            ctx_s[p] = jnp.concatenate(ctxs, axis=1)
            return carry

        jax.lax.fori_loop(0, H // 2, a_body, 0)

        wo_cp.wait()

        def oa_cp(i):
            return pltpu.make_async_copy(oa_s.at[i % 2], outh.at[pl.ds(16 * i, 16), :, pl.ds(0, 1024)],
                                         sem_oa.at[i % 2])

        def o_body(i, carry):
            r0 = pl.multiple_of(i * 128, 128)
            lhs = _bf(jnp.concatenate([ctx_s[p, pl.ds(r0, 128), :] for p in range(H // 2)], axis=1))
            res = _pk(_dot(lhs, _bf(wo_s[...])))

            @pl.when(i >= 2)
            def _():
                oa_cp(i - 2).wait()

            oa_s[i % 2] = res.reshape(16, 8, M)
            oa_cp(i).start()
            return carry

        jax.lax.fori_loop(0, 8, o_body, 0)
        oa_cp(6).wait()
        oa_cp(7).wait()

    if do_b:
        for p in range(8):
            ob_cp(p).wait()


def _run(A_x, A_c_kv, A_w_q, A_w_uk, A_w_uv, A_w_o, B_x, B_w_r, B_w_i, *, bq=512, do_a=True, do_b=True, rg_rows=16, n_pre=1, flags=None):
    any_spec = pl.BlockSpec(memory_space=pltpu.HBM)
    vm = pltpu.VMEM
    dma = pltpu.SemaphoreType.DMA
    scratch = [
        vm((1024, 1024), _U32),
        vm((1024, 512), _U32),
        vm((2048, 1024), _U32),
        vm((2, 2, 512, 128), _U32),
        vm((2, 2, 256, 128), _U32),
        vm((2, 2, 256, 128), _U32),
        vm((16, 1024, 256), _U32),
        vm((2, 16, 8, 1024), _U32),
        vm((8, 2, 64, 1024), _U32),
        vm((16, 256, 128), _U32),
        vm((16, 256, 128), _U32),
        vm((1, 2048), _BF16),
        vm((1, 2048), _BF16),
        vm((4, 128, 256), _U32),
        vm((4, 128, 256), _U32),
        vm((16, 128, 256), _U32),
        vm((16, 4, 64, 256), _U32),
        vm((16, 8, 128), _U32),
        vm((16, 4, 64, 256), _U32),
        vm((8, 128, 1024), _U32),
        vm((16, 128, 256), _F32), vm((16, 128, 256), _F32), vm((16, 128, 256), _F32), vm((16, 128, 256), _F32),
        vm((16, 64, 256), _U32), vm((16, 64, 256), _U32),
        vm((16, 128, 128), _F32),
        dma((16,)), dma((9,)), dma((32,)), dma((12,)), dma((8,)), dma((2,)),
    ]
    out = pl.pallas_call(
        functools.partial(_kernel, bq=bq, do_a=do_a, do_b=do_b, rg_rows=rg_rows, n_pre=n_pre),
        out_shape=jax.ShapeDtypeStruct((128, 16, 2048), _BF16),
        in_specs=[pl.BlockSpec(memory_space=pltpu.SMEM)] + [any_spec] * 12,
        out_specs=any_spec,
        scratch_shapes=scratch,
        compiler_params=pltpu.CompilerParams(vmem_limit_bytes=112 * 1024 * 1024, flags=flags),
    )(jnp.asarray(np.ones((1,), np.int32)), *[pltpu.with_memory_space_constraint(a, pltpu.HBM) for a in (
        A_x.reshape(S, M), A_c_kv.reshape(S, DC),
        A_w_q.reshape(512, 64, HD), A_w_uk.reshape(256, 64, HD), A_w_uv.reshape(256, 64, HD),
        A_w_o.reshape(H * HD, M),
        B_x.reshape(64, 32, BD), B_w_r.T, B_w_i.T,
        jnp.asarray(_FC), jnp.asarray(_IC), jnp.asarray(_GF),
    )])
    return out.reshape(1, S, 2048)


@jax.jit
def pallas_concat_heads__compressed_kv_cla__spectral_gfnet__prompt_kernel(
    A_x: jax.Array,
    A_c_kv: jax.Array,
    A_w_q: jax.Array,
    A_w_uk: jax.Array,
    A_w_uv: jax.Array,
    A_w_o: jax.Array,
    B_x: jax.Array,
    B_w_r: jax.Array,
    B_w_i: jax.Array,
):
    return _run(A_x, A_c_kv, A_w_q, A_w_uk, A_w_uv, A_w_o, B_x, B_w_r, B_w_i)
```

```python
import functools

import numpy as np
import jax
import jax.numpy as jnp
import jax.experimental.pallas as pl
import jax.experimental.pallas.tpu as pltpu

S = 2048
M = 1024
H = 32
HD = 128
DC = 512
BD = 1024
NG = 8

_U32 = jnp.uint32
_BF16 = jnp.bfloat16
_F32 = jnp.float32
_NT = (((1,), (1,)), ((), ()))
_QSCALE = float(HD ** -0.5 * np.log2(np.e))
_MASKED = -1e9


def _to_bf16_bits(a):
    u = np.ascontiguousarray(a, dtype=np.float32).view(np.uint32).astype(np.uint64)
    r = (u + 0x7FFF + ((u >> 16) & 1)) >> 16
    return r.astype(np.uint32) & 0xFFFF


def _pack_rows(a):
    b = _to_bf16_bits(a)
    return (b[0::2] | (b[1::2] << 16)).astype(np.uint32)


def _neg(p):
    return None if p is None else (-p[0], p[1])


def _add(p, q):
    if p is None:
        return q
    if q is None:
        return p
    if p[0] == q[0]:
        return (p[0], p[1] + q[1])
    if p[0] > 0:
        return (1, p[1] - q[1])
    return (1, q[1] - p[1])


def _sub(p, q):
    return _add(p, _neg(q))


def _scale(p, f):
    if p is None:
        return None
    return (p[0] * (1 if f > 0 else -1), p[1] * abs(f))


def _cadd(x, y):
    return (_add(x[0], y[0]), _add(x[1], y[1]))


def _csub(x, y):
    return (_sub(x[0], y[0]), _sub(x[1], y[1]))


def _cmul_i(x, s):
    return (_neg(x[1]), x[0]) if s > 0 else (x[1], _neg(x[0]))


def _cmul_w(x, n, sgn):
    n = n % 16
    if n == 0:
        return x
    if n == 4:
        return _cmul_i(x, sgn)
    if n == 8:
        return (_neg(x[0]), _neg(x[1]))
    if n == 12:
        return _cmul_i(x, -sgn)
    wr = float(np.cos(2 * np.pi * n / 16))
    wi = float(sgn * np.sin(2 * np.pi * n / 16))
    re, im = x
    if n % 2 == 0:
        r = abs(wr)
        sr = 1 if wr > 0 else -1
        si = 1 if wi > 0 else -1
        a = _sub(re if sr > 0 else _neg(re), im if si > 0 else _neg(im))
        b = _add(re if si > 0 else _neg(re), im if sr > 0 else _neg(im))
        return (_scale(a, r), _scale(b, r))
    return (_sub(_scale(re, wr), _scale(im, wi)), _add(_scale(re, wi), _scale(im, wr)))


def _dft4(x0, x1, x2, x3, sgn):
    s02, d02 = _cadd(x0, x2), _csub(x0, x2)
    s13, d13 = _cadd(x1, x3), _csub(x1, x3)
    r = _cmul_i(d13, sgn)
    return [_cadd(s02, s13), _cadd(d02, r), _csub(s02, s13), _csub(d02, r)]


def _fft16(xs, sgn):
    t = [_dft4(xs[a0], xs[4 + a0], xs[8 + a0], xs[12 + a0], sgn) for a0 in range(4)]
    t = [[_cmul_w(t[a0][j0], a0 * j0, sgn) for j0 in range(4)] for a0 in range(4)]
    out = [None] * 16
    for j0 in range(4):
        r = _dft4(t[0][j0], t[1][j0], t[2][j0], t[3][j0], sgn)
        for j1 in range(4):
            out[j0 + 4 * j1] = r[j1]
    return out


def _net_signs(sgn):
    out = _fft16([((1, 1.0), (1, 1.0)) for _ in range(16)], sgn)
    return [(o[0][0], o[1][0]) for o in out]


_INV_SIGNS = _net_signs(+1)
_CLS = ((0, 4), (1, 7), (2, 6), (3, 5))
_R2 = float(np.sqrt(0.5))


def _build_consts():
    n2 = np.arange(128)
    kap = np.arange(64)

    def wl(l):
        return np.exp(-2j * np.pi * np.outer(l, n2) / 1024)

    fc = np.zeros((4, 256, 256))
    w = wl(8 * kap)
    fc[0, 0:64, 0:128] = w.real
    fc[0, 64:128, 0:128] = w.imag
    fc[0, 64, 0:128] = (-1.0) ** n2
    w = wl(4 + 8 * kap)
    fc[0, 0:64, 128:256] = w.real
    fc[0, 64:128, 128:256] = w.imag
    for j in (1, 2, 3):
        si = 1.0 if j == 3 else -1.0
        w1, w2 = wl(j + 8 * kap), wl(8 - j + 8 * kap)
        fc[j, 0:64, 0:128], fc[j, 0:64, 128:] = w1.real, -w1.imag * si
        fc[j, 64:128, 0:128], fc[j, 64:128, 128:] = w2.real, w2.imag * si
        fc[j, 128:192, 0:128], fc[j, 128:192, 128:] = w1.imag, w1.real * si
        fc[j, 192:256, 0:128], fc[j, 192:256, 128:] = w2.imag, -w2.real * si

    def cs(l, c):
        ph = 2 * np.pi * np.outer(l, n2) / 1024
        return c[:, None] * np.cos(ph) / 1024, c[:, None] * np.sin(ph) / 1024

    ic = np.zeros((4, 256, 256))
    two = np.full(64, 2.0)
    co, si = cs(8 * kap, np.where(kap == 0, 1.0, 2.0))
    ic[0, 0:64, 0:128], ic[0, 128:192, 0:128] = co, -si
    ic[0, 128, 0:128] = (-1.0) ** n2 / 1024
    co, si = cs(4 + 8 * kap, two)
    ic[0, 64:128, 128:], ic[0, 192:256, 128:] = co, -si
    for j in (1, 2, 3):
        co, si = cs(j + 8 * kap, two)
        ic[j, 0:64, 0:128], ic[j, 128:192, 0:128] = co, -si
        ic[j, 0:64, 128:], ic[j, 128:192, 128:] = si, co
        co, si = cs(8 - j + 8 * kap, two)
        ic[j, 64:128, 0:128], ic[j, 192:256, 0:128] = co, -si
        ic[j, 64:128, 128:], ic[j, 192:256, 128:] = -si, -co

    gf = np.zeros((16, 256, 256))
    for ap in range(16):
        g = np.exp(-2j * np.pi * (16 * np.outer(n2, n2) + ap * n2[None, :]) / 2048)
        gf[ap] = np.block([[g.real, g.imag], [-g.imag, g.real]])

    def pk(m):
        return np.stack([_pack_rows(x) for x in m])

    return pk(fc), pk(ic / 2048), pk(gf)


_FC, _IC, _GF = _build_consts()
assert all(sg == (1, 1) for sg in _INV_SIGNS)


def _bf(x_u32):
    return pltpu.bitcast(x_u32, _BF16)


def _pk(x_f32):
    return pltpu.bitcast(x_f32.astype(_BF16), _U32)


def _dot(a, b):
    return jnp.dot(a, b, preferred_element_type=_F32)


def _val(p, like):
    if p is None:
        return jnp.zeros_like(like)
    return p[1] if p[0] > 0 else -p[1]


class _Head:
    def __init__(self, q, k, v, bq):
        self.q, self.k, self.v, self.bq = q, k, v, bq
        self.state = {}
        row = jax.lax.broadcasted_iota(jnp.int32, (128, 128), 0)
        col = jax.lax.broadcasted_iota(jnp.int32, (128, 128), 1)
        self.causal = col <= row

    def qk(self, i):
        bq = self.bq
        q0 = i * bq
        qq = self.q[q0:q0 + bq]
        nt = (q0 + bq) // 128
        mx = None
        ss = []
        for j in range(nt):
            r0 = max(0, j * 128 - q0)
            s = jax.lax.dot_general(qq[r0:], self.k[j * 128:(j + 1) * 128], _NT,
                                    preferred_element_type=_F32)
            if j * 128 >= q0:
                sd = jnp.where(self.causal, s[:128], _MASKED)
                s = jnp.concatenate([sd, s[128:]], axis=0) if s.shape[0] > 128 else sd
            ss.append(s)
            if mx is None:
                mx = s
            elif r0 == 0:
                mx = jnp.maximum(mx, s)
            else:
                mx = jnp.concatenate([mx[:r0], jnp.maximum(mx[r0:], s)], axis=0)
        self.state[i] = (ss, jnp.max(mx, axis=1, keepdims=True))

    def pv(self, i):
        bq = self.bq
        q0 = i * bq
        ss, m = self.state.pop(i)
        acc = None
        lsum = None
        for j, s in enumerate(ss):
            r0 = max(0, j * 128 - q0)
            p = jnp.exp2(s - m[r0:])
            pv = _dot(p.astype(_BF16), self.v[j * 128:(j + 1) * 128])
            if acc is None:
                acc, lsum = pv, p
            elif r0 == 0:
                acc, lsum = acc + pv, lsum + p
            else:
                acc = jnp.concatenate([acc[:r0], acc[r0:] + pv], axis=0)
                lsum = jnp.concatenate([lsum[:r0], lsum[r0:] + p], axis=0)
        l = jnp.sum(lsum, axis=1, keepdims=True)
        r = pl.reciprocal(l, approx=True)
        r = r * (2.0 - l * r)
        return acc * r


class _HeadWide(_Head):
    def qk(self, i):
        bq = self.bq
        q0 = i * bq
        parts = []
        for r in range(bq // 128):
            c0, c1 = (0, q0 + 128) if r == 0 else (q0 + 128 * r, q0 + 128 * (r + 1))
            s = jax.lax.dot_general(self.q[q0 + 128 * r:q0 + bq], self.k[c0:c1], _NT,
                                    preferred_element_type=_F32)
            w = c1 - c0
            top = jnp.where(self.causal, s[:128, w - 128:], _MASKED)
            if w > 128:
                top = jnp.concatenate([s[:128, :w - 128], top], axis=1)
            s = jnp.concatenate([top, s[128:]], axis=0) if s.shape[0] > 128 else top
            parts.append(s)
        mx = jnp.max(parts[0], axis=1, keepdims=True)
        for r in range(1, bq // 128):
            mr = jnp.max(parts[r], axis=1, keepdims=True)
            mx = jnp.concatenate([mx[:128 * r], jnp.maximum(mx[128 * r:], mr)], axis=0)
        self.state[i] = (parts, mx)

    def pv(self, i):
        bq = self.bq
        q0 = i * bq
        parts, m = self.state.pop(i)
        acc = l = None
        for r, s in enumerate(parts):
            c0, c1 = (0, q0 + 128) if r == 0 else (q0 + 128 * r, q0 + 128 * (r + 1))
            p = jnp.exp2(s - m[128 * r:])
            lr = jnp.sum(p, axis=1, keepdims=True)
            o = _dot(p.astype(_BF16), self.v[c0:c1])
            if r == 0:
                acc, l = o, lr
            else:
                acc = jnp.concatenate([acc[:128 * r], acc[128 * r:] + o], axis=0)
                l = jnp.concatenate([l[:128 * r], l[128 * r:] + lr], axis=0)
        rc = pl.reciprocal(l, approx=True)
        rc = rc * (2.0 - l * rc)
        return acc * rc


def _kernel(flag_ref, x_hbm, c_hbm, wq_hbm, wk_hbm, wv_hbm, wo_hbm, bx_hbm, wr_hbm, wi_hbm,
            fc_hbm, ic_hbm, gf_hbm,
            out_hbm,
            x_s, c_s, wo_s, wq_s, wk_s, wv_s, qkv0_s, qkv1_s, ctx_s, oa_s,
            bx_s, wr_s, wi_s, wnr_s, wni_s, fc_s, ic_s, gf_s, x1_s, nq_s, v_s, ob_s, u0_s, u1_s, u2_s, u3_s, q0_s, q1_s, vc_s,
            sem_bx, sem_misc, sem_w, sem_pair, sem_ob, sem_oa, *, bq, do_a, do_b, rg_rows, n_pre, frows, fill_slots, lookahead, dbg, wide):
    xh = x_hbm.bitcast(_U32)
    ch = c_hbm.bitcast(_U32)
    wqh = wq_hbm.bitcast(_U32)
    wkh = wk_hbm.bitcast(_U32)
    wvh = wv_hbm.bitcast(_U32)
    woh = wo_hbm.bitcast(_U32)
    bxh = bx_hbm.bitcast(_U32)
    wrh = wr_hbm.at[pl.ds(0, 512)].bitcast(_U32)
    wih = wi_hbm.at[pl.ds(0, 512)].bitcast(_U32)
    outh = out_hbm.bitcast(_U32)

    def bx_cp(p, par):
        return pltpu.make_async_copy(bxh.at[:, par * 8 + p], bx_s.at[p, par], sem_bx.at[2 * p + par])

    def w_cp(j, which):
        src, dst = (wrh, wr_s) if which == 0 else (wih, wi_s)
        return pltpu.make_async_copy(src.at[:, pl.ds(128 * j, 128)], dst.at[j], sem_w.at[2 * j + which])

    fc_cp = pltpu.make_async_copy(fc_hbm, fc_s, sem_misc.at[0])
    ic_cp = pltpu.make_async_copy(ic_hbm, ic_s, sem_misc.at[1])
    wnr_cp = pltpu.make_async_copy(wr_hbm.at[pl.ds(512, 1)], wnr_s, sem_misc.at[2])
    gf_cp = pltpu.make_async_copy(gf_hbm, gf_s, sem_misc.at[3])
    x_cp = pltpu.make_async_copy(xh, x_s, sem_misc.at[5])
    c_cp = pltpu.make_async_copy(ch, c_s, sem_misc.at[6])
    wo_cp = pltpu.make_async_copy(woh, wo_s, sem_misc.at[7])
    wni_cp = pltpu.make_async_copy(wi_hbm.at[pl.ds(512, 1)], wni_s, sem_misc.at[8])

    def pair_cps(p, slot):
        cps = []
        for i, (src, dst) in enumerate(((wqh, wq_s), (wkh, wk_s), (wvh, wv_s))):
            for par in range(2):
                cps.append(pltpu.make_async_copy(
                    src.at[:, par * 16 + p], dst.at[slot, par], sem_pair.at[slot * 6 + 2 * i + par]))
        return cps

    if do_b:
        bx_cp(0, 0).start()
        bx_cp(0, 1).start()
        fc_cp.start()
        for p in range(1, 8):
            bx_cp(p, 0).start()
            bx_cp(p, 1).start()
        gf_cp.start()
        wnr_cp.start()
        wni_cp.start()
        for j in range(16):
            w_cp(j, 0).start()
            w_cp(j, 1).start()
        ic_cp.start()
    if do_a:
        x_cp.start()
        c_cp.start()
        for cp in pair_cps(0, 0) + pair_cps(1, 1):
            cp.start()
        wo_cp.start()

    fence = flag_ref[0] > 0

    if do_b:
        lane0 = jax.lax.broadcasted_iota(jnp.int32, (1, 128), 1) == 0
        row0 = jax.lax.broadcasted_iota(jnp.int32, (8, 128), 0) == 0

        fc_cp.wait()

        def b1_body(p, carry):
            bx_cp(p, 0).wait()
            bx_cp(p, 1).wait()
            for h in range(2):
                halves = []
                for par in range(2):
                    xf = pltpu.unpack_elementwise(bx_s[p, par], index=h, packed_dtype=_BF16,
                                                  unpacked_dtype=_F32)
                    xs = [xf[:, 128 * n:128 * (n + 1)] for n in range(8)]
                    a_, b_ = xs[0] + xs[4], xs[0] - xs[4]
                    c_, d_ = xs[2] + xs[6], xs[2] - xs[6]
                    e_, f_ = xs[1] + xs[5], xs[1] - xs[5]
                    g_, h_ = xs[3] + xs[7], xs[3] - xs[7]
                    u_ = (f_ - h_) * _R2
                    v_ = (f_ + h_) * _R2
                    ac, eg = a_ + c_, e_ + g_
                    halves.append([ac + eg, ac - eg, b_ + u_, d_ + v_, a_ - c_, e_ - g_, b_ - u_, d_ - v_])
                pln = [_bf(pltpu.pack_elementwise([halves[0][i], halves[1][i]], packed_dtype=_BF16))
                       for i in range(8)]
                ap = 2 * p + h
                f0 = _bf(fc_s[0, pl.ds(0, 64), :])
                o0 = jax.lax.dot_general(f0[:, 0:128], pln[0], _NT, preferred_element_type=_F32)
                o4 = jax.lax.dot_general(f0[:, 128:256], pln[1], _NT, preferred_element_type=_F32)
                nq = jnp.where(row0, o0[64:72], 0.0)
                im = jnp.concatenate([jnp.where(row0, 0.0, o0[64:72]), o0[72:128], o4[64:128]], axis=0)
                re = jnp.concatenate([o0[0:64], o4[0:64]], axis=0)
                nq_s[ap] = _pk(jnp.concatenate([nq, jnp.zeros_like(nq)], axis=0))
                x1_s[ap, 0] = jnp.concatenate([_pk(re), _pk(im)], axis=1)
                for j in (1, 2, 3):
                    rhs = jnp.concatenate([pln[2 * j], pln[2 * j + 1]], axis=1)
                    o = jax.lax.dot_general(_bf(fc_s[j]), rhs, _NT, preferred_element_type=_F32)
                    x1_s[ap, j] = jnp.concatenate([_pk(o[0:128]), _pk(o[128:256])], axis=1)
            return carry

        jax.lax.fori_loop(0, 8, b1_body, 0)

        gf_cp.wait()

        def spectral(us, w_of):
            xs = _fft16(us, -1)
            qs = []
            for j in range(16):
                (sr, xr), (si, xi) = xs[j]
                wr, wi = w_of(j)
                qs.append((_sub((sr, xr * wr), (si, xi * wi)), _add((sr, xr * wi), (si, xi * wr))))
            res = _fft16(qs, +1)
            assert all(r[0][0] == 1 and r[1][0] == 1 for r in res)
            return [(r[0][1], r[1][1]) for r in res]

        u_s, q_s = (u0_s, u1_s, u2_s, u3_s), (q0_s, q1_s)

        def s_fwd(t, ap):
            u_s[t][ap] = _dot(_bf(x1_s[ap, t]), _bf(gf_s[ap]))

        def filt(t, half, ii):
            cls = _CLS[t][half]
            r0 = pl.multiple_of(64 * half + 16 * ii, 16)
            rows = pl.ds(r0, 16)
            wbase = pl.ds(pl.multiple_of(64 * ii, 64), 64)

            def w_of(j):
                return tuple(pltpu.unpack_elementwise(
                    ws.at[j, wbase][pl.ds(cls // 2, 16, stride=4), :], index=cls % 2,
                    packed_dtype=_BF16, unpacked_dtype=_F32) for ws in (wr_s, wi_s))

            res = spectral([((1, u_s[t][ap, rows, pl.ds(0, 128)]), (1, u_s[t][ap, rows, pl.ds(128, 128)]))
                            for ap in range(16)], w_of)
            qrows = pl.ds(pl.multiple_of(32 * half + 8 * ii, 8), 8)
            for ap in range(16):
                q_s[t % 2][ap, qrows, :] = jnp.concatenate([_pk(res[ap][0]), _pk(res[ap][1])], axis=1)

        def s_inv(t, ap):
            o = jax.lax.dot_general(_bf(gf_s[ap]), _bf(q_s[t % 2][ap]), _NT, preferred_element_type=_F32)
            vi = o[128:256]
            if t == 0:
                vi = jnp.where(lane0, vc_s[ap], vi)
            v_s[ap, t] = jnp.concatenate([_pk(o[0:128]), _pk(vi)], axis=1)

        def nyquist():
            un = [_dot(_bf(nq_s[ap]), _bf(gf_s[ap, pl.ds(0, 64), :])) for ap in range(16)]
            wnr = wnr_s[...].astype(_F32)
            wni = wni_s[...].astype(_F32)
            qn = spectral([((1, u[:, 0:128]), (1, u[:, 128:256])) for u in un],
                          lambda j: (wnr[:, 128 * j:128 * (j + 1)], wni[:, 128 * j:128 * (j + 1)]))
            for ap in range(16):
                lhs = jnp.concatenate([qn[ap][0], qn[ap][1]], axis=1).astype(_BF16)
                vn = jax.lax.dot_general(lhs, _bf(gf_s[ap, pl.ds(0, 64), :]), _NT,
                                         preferred_element_type=_F32)
                vn = jnp.concatenate([vn, jnp.zeros((112, 128), _F32)], axis=0)
                vc_s[ap] = vn.T

        def b2_head():
            for t in range(4):
                for ap in range(16):
                    s_fwd(t, ap)

        pl.when(fence)(b2_head)
        wnr_cp.wait()
        wni_cp.wait()
        pl.when(fence)(nyquist)
        for j in range(16):
            w_cp(j, 0).wait()
            w_cp(j, 1).wait()
        for t in range(4):
            for half in range(2):
                def body(ii, carry, t=t, half=half):
                    filt(t, half, ii)
                    if t > 0:
                        for k in range(2):
                            s_inv(t - 1, 8 * half + 2 * ii + k)
                    return carry

                jax.lax.fori_loop(0, 4, body, 0)

        def b2_tail():
            for ap in range(16):
                s_inv(3, ap)

        pl.when(fence)(b2_tail)

        ic_cp.wait()

        def ob_cp(p):
            return pltpu.make_async_copy(ob_s.at[p], outh.at[:, p, pl.ds(1024, 1024)], sem_ob.at[p])

        for p in range(8):
            ys = []
            for h in range(2):
                ap = 2 * p + h
                cc = [_dot(_bf(v_s[ap, t]), _bf(ic_s[t])) for t in range(4)]
                c0, c4 = cc[0][:, 0:128], cc[0][:, 128:256]
                c1r, c1i = cc[1][:, 0:128], cc[1][:, 128:256]
                c2r, c2i = cc[2][:, 0:128], cc[2][:, 128:256]
                c3r, c3i = cc[3][:, 0:128], cc[3][:, 128:256]
                pp, mm = c0 + c4, c0 - c4
                u1, u2, u3, u4 = c1r + c3r, c1i - c3i, c1r - c3r, c1i + c3i
                t1, t2 = (u3 - u4) * _R2, (u3 + u4) * _R2
                e0, e1, e2, e3 = pp + c2r, pp - c2r, mm - c2i, mm + c2i
                ys.append([e0 + u1, e2 + t1, e1 - u2, e3 - t2, e0 - u1, e2 - t1, e1 + u2, e3 + t2])
            ob_s[p] = jnp.concatenate([pltpu.pack_elementwise([ys[0][n], ys[1][n]], packed_dtype=_BF16)
                                       for n in range(8)], axis=1)
            ob_cp(p).start()

    if do_a:
        x_cp.wait()
        c_cp.wait()

        def project_units(slot, half, dst, rows):
            def split(ref):
                a = ref[slot, 0]
                b = ref[slot, 1]
                if half == 1:
                    a, b = a >> 16, b >> 16
                return _bf(pltpu.pack_elementwise([a, b], packed_dtype=jnp.uint16))

            wq = split(wq_s)
            wkv = jnp.concatenate([split(wk_s), split(wv_s)], axis=1)

            def q_unit(r0):
                q = _dot(_bf(x_s[pl.ds(r0 // 2, rows // 2), :]), wq) * _QSCALE
                dst[0, pl.ds(r0 // 2, rows // 2), :] = _pk(q)

            def kv_unit(r0):
                kv = _dot(_bf(c_s[pl.ds(r0 // 2, rows // 2), :]), wkv)
                dst[1, pl.ds(r0 // 2, rows // 2), :] = _pk(kv[:, 0:128])
                dst[2, pl.ds(r0 // 2, rows // 2), :] = _pk(kv[:, 128:256])

            units = []
            for r0 in range(0, S, rows):
                units.append(functools.partial(kv_unit, r0))
                units.append(functools.partial(q_unit, r0))
            return units

        def attend(p, t, src, fillers):
            head = (_HeadWide if wide else _Head)(_bf(src[0]), _bf(src[1]), _bf(src[2]), bq)
            ns = S // bq
            fillers = list(fillers)
            nslots = ns * fill_slots
            total = len(fillers)
            slot = [0]

            def fill():
                slot[0] += 1
                while fillers and (total - len(fillers)) * nslots < total * slot[0]:
                    fillers.pop(0)()

            outs = []
            head.qk(0)
            for i in range(ns):
                if i + 1 < ns:
                    head.qk(i + 1)
                if fill_slots == 2:
                    fill()
                outs.append(head.pv(i))
                fill()
            ctx_s[p, :, pl.ds(t * 128, 128)] = _pk(jnp.concatenate(outs, axis=0))
            while fillers:
                fillers.pop(0)()

        npair = H // 2
        for cp in pair_cps(0, 0):
            cp.wait()
        for u in project_units(0, 0, qkv0_s, 2048):
            u()

        def pair_step(p, last):
            s0 = p % 3
            attend(p, 0, qkv0_s, project_units(s0, 1, qkv1_s, frows))
            if last:
                attend(p, 1, qkv1_s, [])
            else:
                attend(p, 1, qkv1_s, project_units((p + 1) % 3, 0, qkv0_s, frows))

        def a_body(p, carry):
            for cp in pair_cps(p + 1, (p + 1) % 3):
                cp.wait()

            @pl.when(p + 2 < npair)
            def _():
                for cp in pair_cps(p + 2, (p + 2) % 3):
                    cp.start()

            pair_step(p, False)
            return carry

        jax.lax.fori_loop(0, npair - 1, a_body, 0)
        pair_step(npair - 1, True)

        wo_cp.wait()

        def oa_cp(i):
            return pltpu.make_async_copy(oa_s.at[i % 2], outh.at[pl.ds(16 * i, 16), :, pl.ds(0, 1024)],
                                         sem_oa.at[i % 2])

        def o_body(i, carry):
            r0 = pl.multiple_of(i * 128, 128)
            lhs = _bf(jnp.concatenate([ctx_s[p, pl.ds(r0, 128), :] for p in range(H // 2)], axis=1))
            res = _pk(_dot(lhs, _bf(wo_s[...])))

            @pl.when(i >= 2)
            def _():
                oa_cp(i - 2).wait()

            oa_s[i % 2] = res.reshape(16, 8, M)
            oa_cp(i).start()
            return carry

        jax.lax.fori_loop(0, 8, o_body, 0)
        oa_cp(6).wait()
        oa_cp(7).wait()

    if do_b:
        for p in range(8):
            ob_cp(p).wait()


def _run(A_x, A_c_kv, A_w_q, A_w_uk, A_w_uv, A_w_o, B_x, B_w_r, B_w_i, *, bq=256, do_a=True, do_b=True, rg_rows=16, n_pre=1, frows=128, fill_slots=2, lookahead=1, dbg=0, wide=True, flags=None):
    any_spec = pl.BlockSpec(memory_space=pltpu.HBM)
    vm = pltpu.VMEM
    dma = pltpu.SemaphoreType.DMA
    scratch = [
        vm((1024, 1024), _U32),
        vm((1024, 512), _U32),
        vm((2048, 1024), _U32),
        vm((3, 2, 512, 128), _U32),
        vm((3, 2, 256, 128), _U32),
        vm((3, 2, 256, 128), _U32),
        vm((3, 1024, 128), _U32), vm((3, 1024, 128), _U32),
        vm((16, 1024, 256), _U32),
        vm((2, 16, 8, 1024), _U32),
        vm((8, 2, 64, 1024), _U32),
        vm((16, 256, 128), _U32),
        vm((16, 256, 128), _U32),
        vm((1, 2048), _BF16),
        vm((1, 2048), _BF16),
        vm((4, 128, 256), _U32),
        vm((4, 128, 256), _U32),
        vm((16, 128, 256), _U32),
        vm((16, 4, 64, 256), _U32),
        vm((16, 8, 128), _U32),
        vm((16, 4, 64, 256), _U32),
        vm((8, 128, 1024), _U32),
        vm((16, 128, 256), _F32), vm((16, 128, 256), _F32), vm((16, 128, 256), _F32), vm((16, 128, 256), _F32),
        vm((16, 64, 256), _U32), vm((16, 64, 256), _U32),
        vm((16, 128, 128), _F32),
        dma((16,)), dma((9,)), dma((32,)), dma((18,)), dma((8,)), dma((2,)),
    ]
    out = pl.pallas_call(
        functools.partial(_kernel, bq=bq, do_a=do_a, do_b=do_b, rg_rows=rg_rows, n_pre=n_pre, frows=frows, fill_slots=fill_slots, lookahead=lookahead, dbg=dbg, wide=wide),
        out_shape=jax.ShapeDtypeStruct((128, 16, 2048), _BF16),
        in_specs=[pl.BlockSpec(memory_space=pltpu.SMEM)] + [any_spec] * 12,
        out_specs=any_spec,
        scratch_shapes=scratch,
        compiler_params=pltpu.CompilerParams(vmem_limit_bytes=112 * 1024 * 1024, flags=flags),
    )(jnp.asarray(np.ones((1,), np.int32)), *[pltpu.with_memory_space_constraint(a, pltpu.HBM) for a in (
        A_x.reshape(S, M), A_c_kv.reshape(S, DC),
        A_w_q.reshape(512, 64, HD), A_w_uk.reshape(256, 64, HD), A_w_uv.reshape(256, 64, HD),
        A_w_o.reshape(H * HD, M),
        B_x.reshape(64, 32, BD), B_w_r.T, B_w_i.T,
        jnp.asarray(_FC), jnp.asarray(_IC), jnp.asarray(_GF),
    )])
    return out.reshape(1, S, 2048)


@jax.jit
def pallas_concat_heads__compressed_kv_cla__spectral_gfnet__prompt_kernel(
    A_x: jax.Array,
    A_c_kv: jax.Array,
    A_w_q: jax.Array,
    A_w_uk: jax.Array,
    A_w_uv: jax.Array,
    A_w_o: jax.Array,
    B_x: jax.Array,
    B_w_r: jax.Array,
    B_w_i: jax.Array,
):
    return _run(A_x, A_c_kv, A_w_q, A_w_uk, A_w_uv, A_w_o, B_x, B_w_r, B_w_i)
```

```python
import functools

import numpy as np
import jax
import jax.numpy as jnp
import jax.experimental.pallas as pl
import jax.experimental.pallas.tpu as pltpu

S = 2048
M = 1024
H = 32
HD = 128
DC = 512
BD = 1024
NG = 8

_U32 = jnp.uint32
_BF16 = jnp.bfloat16
_F32 = jnp.float32
_NT = (((1,), (1,)), ((), ()))
_QSCALE = float(HD ** -0.5 * np.log2(np.e))
_MASKED = -1e9


def _to_bf16_bits(a):
    u = np.ascontiguousarray(a, dtype=np.float32).view(np.uint32).astype(np.uint64)
    r = (u + 0x7FFF + ((u >> 16) & 1)) >> 16
    return r.astype(np.uint32) & 0xFFFF


def _pack_rows(a):
    b = _to_bf16_bits(a)
    return (b[0::2] | (b[1::2] << 16)).astype(np.uint32)


def _neg(p):
    return None if p is None else (-p[0], p[1])


def _add(p, q):
    if p is None:
        return q
    if q is None:
        return p
    if p[0] == q[0]:
        return (p[0], p[1] + q[1])
    if p[0] > 0:
        return (1, p[1] - q[1])
    return (1, q[1] - p[1])


def _sub(p, q):
    return _add(p, _neg(q))


def _scale(p, f):
    if p is None:
        return None
    return (p[0] * (1 if f > 0 else -1), p[1] * abs(f))


def _cadd(x, y):
    return (_add(x[0], y[0]), _add(x[1], y[1]))


def _csub(x, y):
    return (_sub(x[0], y[0]), _sub(x[1], y[1]))


def _cmul_i(x, s):
    return (_neg(x[1]), x[0]) if s > 0 else (x[1], _neg(x[0]))


def _cmul_w(x, n, sgn):
    n = n % 16
    if n == 0:
        return x
    if n == 4:
        return _cmul_i(x, sgn)
    if n == 8:
        return (_neg(x[0]), _neg(x[1]))
    if n == 12:
        return _cmul_i(x, -sgn)
    wr = float(np.cos(2 * np.pi * n / 16))
    wi = float(sgn * np.sin(2 * np.pi * n / 16))
    re, im = x
    if n % 2 == 0:
        r = abs(wr)
        sr = 1 if wr > 0 else -1
        si = 1 if wi > 0 else -1
        a = _sub(re if sr > 0 else _neg(re), im if si > 0 else _neg(im))
        b = _add(re if si > 0 else _neg(re), im if sr > 0 else _neg(im))
        return (_scale(a, r), _scale(b, r))
    return (_sub(_scale(re, wr), _scale(im, wi)), _add(_scale(re, wi), _scale(im, wr)))


def _dft4(x0, x1, x2, x3, sgn):
    s02, d02 = _cadd(x0, x2), _csub(x0, x2)
    s13, d13 = _cadd(x1, x3), _csub(x1, x3)
    r = _cmul_i(d13, sgn)
    return [_cadd(s02, s13), _cadd(d02, r), _csub(s02, s13), _csub(d02, r)]


def _fft16(xs, sgn):
    t = [_dft4(xs[a0], xs[4 + a0], xs[8 + a0], xs[12 + a0], sgn) for a0 in range(4)]
    t = [[_cmul_w(t[a0][j0], a0 * j0, sgn) for j0 in range(4)] for a0 in range(4)]
    out = [None] * 16
    for j0 in range(4):
        r = _dft4(t[0][j0], t[1][j0], t[2][j0], t[3][j0], sgn)
        for j1 in range(4):
            out[j0 + 4 * j1] = r[j1]
    return out


def _net_signs(sgn):
    out = _fft16([((1, 1.0), (1, 1.0)) for _ in range(16)], sgn)
    return [(o[0][0], o[1][0]) for o in out]


_INV_SIGNS = _net_signs(+1)
_CLS = ((0, 4), (1, 7), (2, 6), (3, 5))
_R2 = float(np.sqrt(0.5))


def _build_consts():
    n2 = np.arange(128)
    kap = np.arange(64)

    def wl(l):
        return np.exp(-2j * np.pi * np.outer(l, n2) / 1024)

    fc = np.zeros((4, 256, 256))
    w = wl(8 * kap)
    fc[0, 0:64, 0:128] = w.real
    fc[0, 64:128, 0:128] = w.imag
    fc[0, 64, 0:128] = (-1.0) ** n2
    w = wl(4 + 8 * kap)
    fc[0, 0:64, 128:256] = w.real
    fc[0, 64:128, 128:256] = w.imag
    for j in (1, 2, 3):
        si = 1.0 if j == 3 else -1.0
        w1, w2 = wl(j + 8 * kap), wl(8 - j + 8 * kap)
        fc[j, 0:64, 0:128], fc[j, 0:64, 128:] = w1.real, -w1.imag * si
        fc[j, 64:128, 0:128], fc[j, 64:128, 128:] = w2.real, w2.imag * si
        fc[j, 128:192, 0:128], fc[j, 128:192, 128:] = w1.imag, w1.real * si
        fc[j, 192:256, 0:128], fc[j, 192:256, 128:] = w2.imag, -w2.real * si

    def cs(l, c):
        ph = 2 * np.pi * np.outer(l, n2) / 1024
        return c[:, None] * np.cos(ph) / 1024, c[:, None] * np.sin(ph) / 1024

    ic = np.zeros((4, 256, 256))
    two = np.full(64, 2.0)
    co, si = cs(8 * kap, np.where(kap == 0, 1.0, 2.0))
    ic[0, 0:64, 0:128], ic[0, 128:192, 0:128] = co, -si
    ic[0, 128, 0:128] = (-1.0) ** n2 / 1024
    co, si = cs(4 + 8 * kap, two)
    ic[0, 64:128, 128:], ic[0, 192:256, 128:] = co, -si
    for j in (1, 2, 3):
        co, si = cs(j + 8 * kap, two)
        ic[j, 0:64, 0:128], ic[j, 128:192, 0:128] = co, -si
        ic[j, 0:64, 128:], ic[j, 128:192, 128:] = si, co
        co, si = cs(8 - j + 8 * kap, two)
        ic[j, 64:128, 0:128], ic[j, 192:256, 0:128] = co, -si
        ic[j, 64:128, 128:], ic[j, 192:256, 128:] = -si, -co

    f128 = np.exp(-2j * np.pi * np.outer(n2, n2) / 128)
    tw = np.exp(-2j * np.pi * np.outer(np.arange(16), n2) / 2048)
    gt = np.concatenate([f128.real, f128.imag, tw.real, tw.imag], axis=0).astype(np.float32)

    def pk(m):
        return np.stack([_pack_rows(x) for x in m])

    return pk(fc), pk(ic / 2048), gt


_FC, _IC, _GT = _build_consts()
assert all(sg == (1, 1) for sg in _INV_SIGNS)


def _bf(x_u32):
    return pltpu.bitcast(x_u32, _BF16)


def _pk(x_f32):
    return pltpu.bitcast(x_f32.astype(_BF16), _U32)


def _dot(a, b):
    return jnp.dot(a, b, preferred_element_type=_F32)


def _val(p, like):
    if p is None:
        return jnp.zeros_like(like)
    return p[1] if p[0] > 0 else -p[1]


class _Head:
    def __init__(self, q, k, v, bq):
        self.q, self.k, self.v, self.bq = q, k, v, bq
        self.state = {}
        row = jax.lax.broadcasted_iota(jnp.int32, (128, 128), 0)
        col = jax.lax.broadcasted_iota(jnp.int32, (128, 128), 1)
        self.causal = col <= row

    def qk(self, i):
        bq = self.bq
        q0 = i * bq
        qq = self.q[q0:q0 + bq]
        nt = (q0 + bq) // 128
        mx = None
        ss = []
        for j in range(nt):
            r0 = max(0, j * 128 - q0)
            s = jax.lax.dot_general(qq[r0:], self.k[j * 128:(j + 1) * 128], _NT,
                                    preferred_element_type=_F32)
            if j * 128 >= q0:
                sd = jnp.where(self.causal, s[:128], _MASKED)
                s = jnp.concatenate([sd, s[128:]], axis=0) if s.shape[0] > 128 else sd
            ss.append(s)
            if mx is None:
                mx = s
            elif r0 == 0:
                mx = jnp.maximum(mx, s)
            else:
                mx = jnp.concatenate([mx[:r0], jnp.maximum(mx[r0:], s)], axis=0)
        self.state[i] = (ss, jnp.max(mx, axis=1, keepdims=True))

    def pv(self, i):
        bq = self.bq
        q0 = i * bq
        ss, m = self.state.pop(i)
        acc = None
        lsum = None
        for j, s in enumerate(ss):
            r0 = max(0, j * 128 - q0)
            p = jnp.exp2(s - m[r0:])
            pv = _dot(p.astype(_BF16), self.v[j * 128:(j + 1) * 128])
            if acc is None:
                acc, lsum = pv, p
            elif r0 == 0:
                acc, lsum = acc + pv, lsum + p
            else:
                acc = jnp.concatenate([acc[:r0], acc[r0:] + pv], axis=0)
                lsum = jnp.concatenate([lsum[:r0], lsum[r0:] + p], axis=0)
        l = jnp.sum(lsum, axis=1, keepdims=True)
        r = pl.reciprocal(l, approx=True)
        r = r * (2.0 - l * r)
        return acc * r


class _HeadWide(_Head):
    def qk(self, i):
        bq = self.bq
        q0 = i * bq
        parts = []
        for r in range(bq // 128):
            c0, c1 = (0, q0 + 128) if r == 0 else (q0 + 128 * r, q0 + 128 * (r + 1))
            s = jax.lax.dot_general(self.q[q0 + 128 * r:q0 + bq], self.k[c0:c1], _NT,
                                    preferred_element_type=_F32)
            w = c1 - c0
            top = jnp.where(self.causal, s[:128, w - 128:], _MASKED)
            if w > 128:
                top = jnp.concatenate([s[:128, :w - 128], top], axis=1)
            s = jnp.concatenate([top, s[128:]], axis=0) if s.shape[0] > 128 else top
            parts.append(s)
        mx = jnp.max(parts[0], axis=1, keepdims=True)
        for r in range(1, bq // 128):
            mr = jnp.max(parts[r], axis=1, keepdims=True)
            mx = jnp.concatenate([mx[:128 * r], jnp.maximum(mx[128 * r:], mr)], axis=0)
        self.state[i] = (parts, mx)

    def pv(self, i):
        bq = self.bq
        q0 = i * bq
        parts, m = self.state.pop(i)
        acc = l = None
        for r, s in enumerate(parts):
            c0, c1 = (0, q0 + 128) if r == 0 else (q0 + 128 * r, q0 + 128 * (r + 1))
            p = jnp.exp2(s - m[128 * r:])
            lr = jnp.sum(p, axis=1, keepdims=True)
            o = _dot(p.astype(_BF16), self.v[c0:c1])
            if r == 0:
                acc, l = o, lr
            else:
                acc = jnp.concatenate([acc[:128 * r], acc[128 * r:] + o], axis=0)
                l = jnp.concatenate([l[:128 * r], l[128 * r:] + lr], axis=0)
        rc = pl.reciprocal(l, approx=True)
        rc = rc * (2.0 - l * rc)
        return acc * rc


def _kernel(flag_ref, x_hbm, c_hbm, wq_hbm, wk_hbm, wv_hbm, wo_hbm, bx_hbm, wr_hbm, wi_hbm,
            fc_hbm, ic_hbm, gt_hbm,
            out_hbm,
            x_s, c_s, wo_s, wq_s, wk_s, wv_s, qkv0_s, qkv1_s, ctx_s, oa_s,
            bx_s, wr_s, wi_s, wnr_s, wni_s, fc_s, ic_s, gt_s, gf_s, x1_s, nq_s, v_s, ob_s, u0_s, u1_s, u2_s, u3_s, q0_s, q1_s, vc_s,
            sem_bx, sem_misc, sem_w, sem_pair, sem_ob, sem_oa, *, bq, do_a, do_b, rg_rows, n_pre, frows, fill_slots, lookahead, dbg, wide, bx_win, w_at):
    xh = x_hbm.bitcast(_U32)
    ch = c_hbm.bitcast(_U32)
    wqh = wq_hbm.bitcast(_U32)
    wkh = wk_hbm.bitcast(_U32)
    wvh = wv_hbm.bitcast(_U32)
    woh = wo_hbm.bitcast(_U32)
    bxh = bx_hbm.bitcast(_U32)
    wrh = wr_hbm.at[pl.ds(0, 512)].bitcast(_U32)
    wih = wi_hbm.at[pl.ds(0, 512)].bitcast(_U32)
    outh = out_hbm.bitcast(_U32)

    def bx_cp(p, par):
        return pltpu.make_async_copy(bxh.at[:, par * 8 + p], bx_s.at[p, par], sem_bx.at[2 * p + par])

    def w_cp(j, which):
        src, dst = (wrh, wr_s) if which == 0 else (wih, wi_s)
        return pltpu.make_async_copy(src.at[:, pl.ds(128 * j, 128)], dst.at[j], sem_w.at[2 * j + which])

    fc_cp = pltpu.make_async_copy(fc_hbm, fc_s, sem_misc.at[0])
    ic_cp = pltpu.make_async_copy(ic_hbm, ic_s, sem_misc.at[1])
    wnr_cp = pltpu.make_async_copy(wr_hbm.at[pl.ds(512, 1)], wnr_s, sem_misc.at[2])
    x_cp = pltpu.make_async_copy(xh, x_s, sem_misc.at[5])
    c_cp = pltpu.make_async_copy(ch, c_s, sem_misc.at[6])
    wo_cp = pltpu.make_async_copy(woh, wo_s, sem_misc.at[7])
    wni_cp = pltpu.make_async_copy(wi_hbm.at[pl.ds(512, 1)], wni_s, sem_misc.at[8])

    def pair_cps(p, slot):
        cps = []
        for i, (src, dst) in enumerate(((wqh, wq_s), (wkh, wk_s), (wvh, wv_s))):
            for par in range(2):
                cps.append(pltpu.make_async_copy(
                    src.at[:, par * 16 + p], dst.at[slot, par], sem_pair.at[slot * 6 + 2 * i + par]))
        return cps

    gt_cp = pltpu.make_async_copy(gt_hbm, gt_s, sem_misc.at[3])

    def start_a_inputs():
        x_cp.start()
        c_cp.start()
        for cp in pair_cps(0, 0) + pair_cps(1, 1):
            cp.start()

    if do_b:
        gt_cp.start()
        bx_cp(0, 0).start()
        bx_cp(0, 1).start()
        fc_cp.start()
        for p in range(1, bx_win):
            bx_cp(p, 0).start()
            bx_cp(p, 1).start()
        wnr_cp.start()
        wni_cp.start()
    if do_a and not do_b:
        start_a_inputs()
        wo_cp.start()

    fence = flag_ref[0] > 0

    if do_b:
        lane0 = jax.lax.broadcasted_iota(jnp.int32, (1, 128), 1) == 0
        row0 = jax.lax.broadcasted_iota(jnp.int32, (8, 128), 0) == 0

        gt_cp.wait()
        f_r, f_i = gt_s[pl.ds(0, 128), :], gt_s[pl.ds(128, 128), :]
        for ap in range(16):
            t_r, t_i = gt_s[pl.ds(256 + ap, 1), :], gt_s[pl.ds(272 + ap, 1), :]
            g_r = _pk(f_r * t_r - f_i * t_i)
            g_i = _pk(f_r * t_i + f_i * t_r)
            gf_s[ap] = jnp.concatenate([jnp.concatenate([g_r, g_i], axis=1),
                                        jnp.concatenate([g_i ^ jnp.uint32(0x80008000), g_r], axis=1)], axis=0)
        fc_cp.wait()

        def b1_step(p):
            bx_cp(p, 0).wait()
            bx_cp(p, 1).wait()
            if p + bx_win < 8:
                bx_cp(p + bx_win, 0).start()
                bx_cp(p + bx_win, 1).start()
            if p == w_at:
                for j in range(16):
                    w_cp(j, 0).start()
                    w_cp(j, 1).start()
            for h in range(2):
                halves = []
                for par in range(2):
                    xf = pltpu.unpack_elementwise(bx_s[p, par], index=h, packed_dtype=_BF16,
                                                  unpacked_dtype=_F32)
                    xs = [xf[:, 128 * n:128 * (n + 1)] for n in range(8)]
                    a_, b_ = xs[0] + xs[4], xs[0] - xs[4]
                    c_, d_ = xs[2] + xs[6], xs[2] - xs[6]
                    e_, f_ = xs[1] + xs[5], xs[1] - xs[5]
                    g_, h_ = xs[3] + xs[7], xs[3] - xs[7]
                    u_ = (f_ - h_) * _R2
                    v_ = (f_ + h_) * _R2
                    ac, eg = a_ + c_, e_ + g_
                    halves.append([ac + eg, ac - eg, b_ + u_, d_ + v_, a_ - c_, e_ - g_, b_ - u_, d_ - v_])
                pln = [_bf(pltpu.pack_elementwise([halves[0][i], halves[1][i]], packed_dtype=_BF16))
                       for i in range(8)]
                ap = 2 * p + h
                f0 = _bf(fc_s[0, pl.ds(0, 64), :])
                o0 = jax.lax.dot_general(f0[:, 0:128], pln[0], _NT, preferred_element_type=_F32)
                o4 = jax.lax.dot_general(f0[:, 128:256], pln[1], _NT, preferred_element_type=_F32)
                nq = jnp.where(row0, o0[64:72], 0.0)
                im = jnp.concatenate([jnp.where(row0, 0.0, o0[64:72]), o0[72:128], o4[64:128]], axis=0)
                re = jnp.concatenate([o0[0:64], o4[0:64]], axis=0)
                nq_s[ap] = _pk(jnp.concatenate([nq, jnp.zeros_like(nq)], axis=0))
                x1_s[ap, 0] = jnp.concatenate([_pk(re), _pk(im)], axis=1)
                for j in (1, 2, 3):
                    rhs = jnp.concatenate([pln[2 * j], pln[2 * j + 1]], axis=1)
                    o = jax.lax.dot_general(_bf(fc_s[j]), rhs, _NT, preferred_element_type=_F32)
                    x1_s[ap, j] = jnp.concatenate([_pk(o[0:128]), _pk(o[128:256])], axis=1)

        for p in range(8):
            b1_step(p)

        def spectral(us, w_of):
            xs = _fft16(us, -1)
            qs = []
            for j in range(16):
                (sr, xr), (si, xi) = xs[j]
                wr, wi = w_of(j)
                qs.append((_sub((sr, xr * wr), (si, xi * wi)), _add((sr, xr * wi), (si, xi * wr))))
            res = _fft16(qs, +1)
            assert all(r[0][0] == 1 and r[1][0] == 1 for r in res)
            return [(r[0][1], r[1][1]) for r in res]

        u_s, q_s = (u0_s, u1_s, u2_s, u3_s), (q0_s, q1_s)

        def s_fwd(t, ap):
            u_s[t][ap] = _dot(_bf(x1_s[ap, t]), _bf(gf_s[ap]))

        def filt(t, half, ii):
            cls = _CLS[t][half]
            r0 = pl.multiple_of(64 * half + rg_rows * ii, rg_rows)
            rows = pl.ds(r0, rg_rows)
            wbase = pl.ds(pl.multiple_of(4 * rg_rows * ii, 4 * rg_rows), 4 * rg_rows)

            def w_of(j):
                return tuple(pltpu.unpack_elementwise(
                    ws.at[j, wbase][pl.ds(cls // 2, rg_rows, stride=4), :], index=cls % 2,
                    packed_dtype=_BF16, unpacked_dtype=_F32) for ws in (wr_s, wi_s))

            res = spectral([((1, u_s[t][ap, rows, pl.ds(0, 128)]), (1, u_s[t][ap, rows, pl.ds(128, 128)]))
                            for ap in range(16)], w_of)
            for ap in range(16):
                if rg_rows == 8:
                    q_s[t % 2][ap, rows, pl.ds(0, 128)] = res[ap][0]
                    q_s[t % 2][ap, rows, pl.ds(128, 128)] = res[ap][1]
                else:
                    qrows = pl.ds(pl.multiple_of(32 * half + (rg_rows // 2) * ii, rg_rows // 2), rg_rows // 2)
                    q_s[t % 2][ap, qrows, :] = jnp.concatenate([_pk(res[ap][0]), _pk(res[ap][1])], axis=1)

        def s_inv(t, ap):
            q = q_s[t % 2][ap].astype(_BF16) if rg_rows == 8 else _bf(q_s[t % 2][ap])
            o = jax.lax.dot_general(_bf(gf_s[ap]), q, _NT, preferred_element_type=_F32)
            vi = o[128:256]
            if t == 0:
                vi = jnp.where(lane0, vc_s[ap], vi)
            v_s[ap, t] = jnp.concatenate([_pk(o[0:128]), _pk(vi)], axis=1)

        def nyquist(un):
            wnr = wnr_s[...].astype(_F32)
            wni = wni_s[...].astype(_F32)
            qn = spectral([((1, u[:, 0:128]), (1, u[:, 128:256])) for u in un],
                          lambda j: (wnr[:, 128 * j:128 * (j + 1)], wni[:, 128 * j:128 * (j + 1)]))
            for ap in range(16):
                lhs = jnp.concatenate([qn[ap][0], qn[ap][1]], axis=1).astype(_BF16)
                vn = jax.lax.dot_general(lhs, _bf(gf_s[ap, pl.ds(0, 64), :]), _NT,
                                         preferred_element_type=_F32)
                vn = jnp.concatenate([vn, jnp.zeros((112, 128), _F32)], axis=0)
                vc_s[ap] = vn.T

        def b2_head():
            un = [_dot(_bf(nq_s[ap]), _bf(gf_s[ap, pl.ds(0, 64), :])) for ap in range(16)]
            for t in range(4):
                for ap in range(16):
                    s_fwd(t, ap)
                if t == 1:
                    nyquist(un)

        wnr_cp.wait()
        wni_cp.wait()
        pl.when(fence)(b2_head)
        ic_cp.start()
        if do_a:
            start_a_inputs()
        for j in range(16):
            w_cp(j, 0).wait()
            w_cp(j, 1).wait()
        nit = 64 // rg_rows
        for t in range(4):
            for half in range(2):
                def body(ii, carry, t=t, half=half):
                    filt(t, half, ii)
                    if t > 0:
                        for k in range(8 // nit):
                            s_inv(t - 1, 8 * half + (8 // nit) * ii + k)
                    return carry

                jax.lax.fori_loop(0, nit, body, 0)

        def b2_tail():
            for ap in range(16):
                s_inv(3, ap)

        pl.when(fence)(b2_tail)

        if do_a:
            wo_cp.start()
        ic_cp.wait()

        def ob_cp(p):
            return pltpu.make_async_copy(ob_s.at[p], outh.at[:, p, pl.ds(1024, 1024)], sem_ob.at[p])

        for p in range(8):
            ys = []
            for h in range(2):
                ap = 2 * p + h
                cc = [_dot(_bf(v_s[ap, t]), _bf(ic_s[t])) for t in range(4)]
                c0, c4 = cc[0][:, 0:128], cc[0][:, 128:256]
                c1r, c1i = cc[1][:, 0:128], cc[1][:, 128:256]
                c2r, c2i = cc[2][:, 0:128], cc[2][:, 128:256]
                c3r, c3i = cc[3][:, 0:128], cc[3][:, 128:256]
                pp, mm = c0 + c4, c0 - c4
                u1, u2, u3, u4 = c1r + c3r, c1i - c3i, c1r - c3r, c1i + c3i
                t1, t2 = (u3 - u4) * _R2, (u3 + u4) * _R2
                e0, e1, e2, e3 = pp + c2r, pp - c2r, mm - c2i, mm + c2i
                ys.append([e0 + u1, e2 + t1, e1 - u2, e3 - t2, e0 - u1, e2 - t1, e1 + u2, e3 + t2])
            ob_s[p] = jnp.concatenate([pltpu.pack_elementwise([ys[0][n], ys[1][n]], packed_dtype=_BF16)
                                       for n in range(8)], axis=1)
            ob_cp(p).start()

    if do_a:
        x_cp.wait()
        c_cp.wait()

        def project_units(slot, half, dst, rows):
            def split(ref):
                a = ref[slot, 0]
                b = ref[slot, 1]
                if half == 1:
                    a, b = a >> 16, b >> 16
                return _bf(pltpu.pack_elementwise([a, b], packed_dtype=jnp.uint16))

            wq = split(wq_s)
            wkv = jnp.concatenate([split(wk_s), split(wv_s)], axis=1)

            def q_unit(r0):
                q = _dot(_bf(x_s[pl.ds(r0 // 2, rows // 2), :]), wq) * _QSCALE
                dst[0, pl.ds(r0 // 2, rows // 2), :] = _pk(q)

            def kv_unit(r0):
                kv = _dot(_bf(c_s[pl.ds(r0 // 2, rows // 2), :]), wkv)
                dst[1, pl.ds(r0 // 2, rows // 2), :] = _pk(kv[:, 0:128])
                dst[2, pl.ds(r0 // 2, rows // 2), :] = _pk(kv[:, 128:256])

            units = []
            for r0 in range(0, S, rows):
                units.append(functools.partial(kv_unit, r0))
                units.append(functools.partial(q_unit, r0))
            return units

        def attend(p, t, src, fillers):
            head = (_HeadWide if wide else _Head)(_bf(src[0]), _bf(src[1]), _bf(src[2]), bq)
            ns = S // bq
            fillers = list(fillers)
            nslots = ns * fill_slots
            total = len(fillers)
            slot = [0]

            def fill():
                slot[0] += 1
                while fillers and (total - len(fillers)) * nslots < total * slot[0]:
                    fillers.pop(0)()

            outs = []
            head.qk(0)
            for i in range(ns):
                if i + 1 < ns:
                    head.qk(i + 1)
                if fill_slots == 2:
                    fill()
                outs.append(head.pv(i))
                fill()
            ctx_s[p, :, pl.ds(t * 128, 128)] = _pk(jnp.concatenate(outs, axis=0))
            while fillers:
                fillers.pop(0)()

        npair = H // 2
        for cp in pair_cps(0, 0):
            cp.wait()
        for u in project_units(0, 0, qkv0_s, 2048):
            u()

        def pair_step(p, last):
            s0 = p % 3
            attend(p, 0, qkv0_s, project_units(s0, 1, qkv1_s, frows))
            if last:
                attend(p, 1, qkv1_s, [])
            else:
                attend(p, 1, qkv1_s, project_units((p + 1) % 3, 0, qkv0_s, frows))

        def a_body(p, carry):
            for cp in pair_cps(p + 1, (p + 1) % 3):
                cp.wait()

            @pl.when(p + 2 < npair)
            def _():
                for cp in pair_cps(p + 2, (p + 2) % 3):
                    cp.start()

            pair_step(p, False)
            return carry

        jax.lax.fori_loop(0, npair - 1, a_body, 0)
        pair_step(npair - 1, True)

        wo_cp.wait()

        def oa_cp(i):
            return pltpu.make_async_copy(oa_s.at[i % 2], outh.at[pl.ds(16 * i, 16), :, pl.ds(0, 1024)],
                                         sem_oa.at[i % 2])

        def o_body(i, carry):
            r0 = pl.multiple_of(i * 128, 128)
            lhs = _bf(jnp.concatenate([ctx_s[p, pl.ds(r0, 128), :] for p in range(H // 2)], axis=1))
            res = _pk(_dot(lhs, _bf(wo_s[...])))

            @pl.when(i >= 2)
            def _():
                oa_cp(i - 2).wait()

            oa_s[i % 2] = res.reshape(16, 8, M)
            oa_cp(i).start()
            return carry

        jax.lax.fori_loop(0, 8, o_body, 0)
        oa_cp(6).wait()
        oa_cp(7).wait()

    if do_b:
        for p in range(8):
            ob_cp(p).wait()


def _run(A_x, A_c_kv, A_w_q, A_w_uk, A_w_uv, A_w_o, B_x, B_w_r, B_w_i, *, bq=256, do_a=True, do_b=True, rg_rows=16, n_pre=1, frows=128, fill_slots=2, lookahead=1, dbg=0, wide=True, bx_win=3, w_at=7, flags=None):
    any_spec = pl.BlockSpec(memory_space=pltpu.HBM)
    vm = pltpu.VMEM
    dma = pltpu.SemaphoreType.DMA
    scratch = [
        vm((1024, 1024), _U32),
        vm((1024, 512), _U32),
        vm((2048, 1024), _U32),
        vm((3, 2, 512, 128), _U32),
        vm((3, 2, 256, 128), _U32),
        vm((3, 2, 256, 128), _U32),
        vm((3, 1024, 128), _U32), vm((3, 1024, 128), _U32),
        vm((16, 1024, 256), _U32),
        vm((2, 16, 8, 1024), _U32),
        vm((8, 2, 64, 1024), _U32),
        vm((16, 256, 128), _U32),
        vm((16, 256, 128), _U32),
        vm((1, 2048), _BF16),
        vm((1, 2048), _BF16),
        vm((4, 128, 256), _U32),
        vm((4, 128, 256), _U32),
        vm((288, 128), _F32),
        vm((16, 128, 256), _U32),
        vm((16, 4, 64, 256), _U32),
        vm((16, 8, 128), _U32),
        vm((16, 4, 64, 256), _U32),
        vm((8, 128, 1024), _U32),
        vm((16, 128, 256), _F32), vm((16, 128, 256), _F32), vm((16, 128, 256), _F32), vm((16, 128, 256), _F32),
        *([vm((16, 128, 256), _F32)] * 2 if rg_rows == 8 else [vm((16, 64, 256), _U32)] * 2),
        vm((16, 128, 128), _F32),
        dma((16,)), dma((9,)), dma((32,)), dma((18,)), dma((8,)), dma((2,)),
    ]
    out = pl.pallas_call(
        functools.partial(_kernel, bq=bq, do_a=do_a, do_b=do_b, rg_rows=rg_rows, n_pre=n_pre, frows=frows, fill_slots=fill_slots, lookahead=lookahead, dbg=dbg, wide=wide, bx_win=bx_win, w_at=w_at),
        out_shape=jax.ShapeDtypeStruct((128, 16, 2048), _BF16),
        in_specs=[pl.BlockSpec(memory_space=pltpu.SMEM)] + [any_spec] * 12,
        out_specs=any_spec,
        scratch_shapes=scratch,
        compiler_params=pltpu.CompilerParams(vmem_limit_bytes=112 * 1024 * 1024, flags=flags),
    )(jnp.asarray(np.ones((1,), np.int32)), *[pltpu.with_memory_space_constraint(a, pltpu.HBM) for a in (
        A_x.reshape(S, M), A_c_kv.reshape(S, DC),
        A_w_q.reshape(512, 64, HD), A_w_uk.reshape(256, 64, HD), A_w_uv.reshape(256, 64, HD),
        A_w_o.reshape(H * HD, M),
        B_x.reshape(64, 32, BD), B_w_r.T, B_w_i.T,
        jnp.asarray(_FC), jnp.asarray(_IC), jnp.asarray(_GT),
    )])
    return out.reshape(1, S, 2048)


@jax.jit
def pallas_concat_heads__compressed_kv_cla__spectral_gfnet__prompt_kernel(
    A_x: jax.Array,
    A_c_kv: jax.Array,
    A_w_q: jax.Array,
    A_w_uk: jax.Array,
    A_w_uv: jax.Array,
    A_w_o: jax.Array,
    B_x: jax.Array,
    B_w_r: jax.Array,
    B_w_i: jax.Array,
):
    return _run(A_x, A_c_kv, A_w_q, A_w_uk, A_w_uv, A_w_o, B_x, B_w_r, B_w_i)
```

```python
import functools

import numpy as np
import jax
import jax.numpy as jnp
import jax.experimental.pallas as pl
import jax.experimental.pallas.tpu as pltpu

S = 2048
M = 1024
H = 32
HD = 128
DC = 512
BD = 1024
NG = 8

_U32 = jnp.uint32
_BF16 = jnp.bfloat16
_F32 = jnp.float32
_NT = (((1,), (1,)), ((), ()))
_QSCALE = float(HD ** -0.5 * np.log2(np.e))
_MASKED = -1e9


def _to_bf16_bits(a):
    u = np.ascontiguousarray(a, dtype=np.float32).view(np.uint32).astype(np.uint64)
    r = (u + 0x7FFF + ((u >> 16) & 1)) >> 16
    return r.astype(np.uint32) & 0xFFFF


def _pack_rows(a):
    b = _to_bf16_bits(a)
    return (b[0::2] | (b[1::2] << 16)).astype(np.uint32)


def _neg(p):
    return None if p is None else (-p[0], p[1])


def _add(p, q):
    if p is None:
        return q
    if q is None:
        return p
    if p[0] == q[0]:
        return (p[0], p[1] + q[1])
    if p[0] > 0:
        return (1, p[1] - q[1])
    return (1, q[1] - p[1])


def _sub(p, q):
    return _add(p, _neg(q))


def _scale(p, f):
    if p is None:
        return None
    return (p[0] * (1 if f > 0 else -1), p[1] * abs(f))


def _cadd(x, y):
    return (_add(x[0], y[0]), _add(x[1], y[1]))


def _csub(x, y):
    return (_sub(x[0], y[0]), _sub(x[1], y[1]))


def _cmul_i(x, s):
    return (_neg(x[1]), x[0]) if s > 0 else (x[1], _neg(x[0]))


def _cmul_w(x, n, sgn):
    n = n % 16
    if n == 0:
        return x
    if n == 4:
        return _cmul_i(x, sgn)
    if n == 8:
        return (_neg(x[0]), _neg(x[1]))
    if n == 12:
        return _cmul_i(x, -sgn)
    wr = float(np.cos(2 * np.pi * n / 16))
    wi = float(sgn * np.sin(2 * np.pi * n / 16))
    re, im = x
    if n % 2 == 0:
        r = abs(wr)
        sr = 1 if wr > 0 else -1
        si = 1 if wi > 0 else -1
        a = _sub(re if sr > 0 else _neg(re), im if si > 0 else _neg(im))
        b = _add(re if si > 0 else _neg(re), im if sr > 0 else _neg(im))
        return (_scale(a, r), _scale(b, r))
    return (_sub(_scale(re, wr), _scale(im, wi)), _add(_scale(re, wi), _scale(im, wr)))


def _dft4(x0, x1, x2, x3, sgn):
    s02, d02 = _cadd(x0, x2), _csub(x0, x2)
    s13, d13 = _cadd(x1, x3), _csub(x1, x3)
    r = _cmul_i(d13, sgn)
    return [_cadd(s02, s13), _cadd(d02, r), _csub(s02, s13), _csub(d02, r)]


def _fft16(xs, sgn):
    t = [_dft4(xs[a0], xs[4 + a0], xs[8 + a0], xs[12 + a0], sgn) for a0 in range(4)]
    t = [[_cmul_w(t[a0][j0], a0 * j0, sgn) for j0 in range(4)] for a0 in range(4)]
    out = [None] * 16
    for j0 in range(4):
        r = _dft4(t[0][j0], t[1][j0], t[2][j0], t[3][j0], sgn)
        for j1 in range(4):
            out[j0 + 4 * j1] = r[j1]
    return out


def _net_signs(sgn):
    out = _fft16([((1, 1.0), (1, 1.0)) for _ in range(16)], sgn)
    return [(o[0][0], o[1][0]) for o in out]


_INV_SIGNS = _net_signs(+1)
_CLS = ((0, 4), (1, 7), (2, 6), (3, 5))
_R2 = float(np.sqrt(0.5))


def _build_consts():
    n2 = np.arange(128)
    kap = np.arange(64)

    def wl(l):
        return np.exp(-2j * np.pi * np.outer(l, n2) / 1024)

    fc = np.zeros((4, 256, 256))
    w = wl(8 * kap)
    fc[0, 0:64, 0:128] = w.real
    fc[0, 64:128, 0:128] = w.imag
    fc[0, 64, 0:128] = (-1.0) ** n2
    w = wl(4 + 8 * kap)
    fc[0, 0:64, 128:256] = w.real
    fc[0, 64:128, 128:256] = w.imag
    for j in (1, 2, 3):
        si = 1.0 if j == 3 else -1.0
        w1, w2 = wl(j + 8 * kap), wl(8 - j + 8 * kap)
        fc[j, 0:64, 0:128], fc[j, 0:64, 128:] = w1.real, -w1.imag * si
        fc[j, 64:128, 0:128], fc[j, 64:128, 128:] = w2.real, w2.imag * si
        fc[j, 128:192, 0:128], fc[j, 128:192, 128:] = w1.imag, w1.real * si
        fc[j, 192:256, 0:128], fc[j, 192:256, 128:] = w2.imag, -w2.real * si

    def cs(l, c):
        ph = 2 * np.pi * np.outer(l, n2) / 1024
        return c[:, None] * np.cos(ph) / 1024, c[:, None] * np.sin(ph) / 1024

    ic = np.zeros((4, 256, 256))
    two = np.full(64, 2.0)
    co, si = cs(8 * kap, np.where(kap == 0, 1.0, 2.0))
    ic[0, 0:64, 0:128], ic[0, 128:192, 0:128] = co, -si
    ic[0, 128, 0:128] = (-1.0) ** n2 / 1024
    co, si = cs(4 + 8 * kap, two)
    ic[0, 64:128, 128:], ic[0, 192:256, 128:] = co, -si
    for j in (1, 2, 3):
        co, si = cs(j + 8 * kap, two)
        ic[j, 0:64, 0:128], ic[j, 128:192, 0:128] = co, -si
        ic[j, 0:64, 128:], ic[j, 128:192, 128:] = si, co
        co, si = cs(8 - j + 8 * kap, two)
        ic[j, 64:128, 0:128], ic[j, 192:256, 0:128] = co, -si
        ic[j, 64:128, 128:], ic[j, 192:256, 128:] = -si, -co

    f128 = np.exp(-2j * np.pi * np.outer(n2, n2) / 128)
    tw = np.exp(-2j * np.pi * np.outer(np.arange(16), n2) / 2048)

    def even_odd(m, blk):
        r = m.reshape(-1, blk // 2, 2, m.shape[-1])
        return np.concatenate([r[:, :, 0], r[:, :, 1]], axis=1).reshape(m.shape)

    fc[0] = even_odd(fc[0], 64)
    for j in (1, 2, 3):
        fc[j] = even_odd(fc[j], 128)
    il = np.arange(256).reshape(16, 2, 8).transpose(0, 2, 1).reshape(-1)
    ic = ic[:, il, :]
    sigma = np.concatenate([np.arange(0, 128, 2), np.arange(1, 128, 2)])
    fpos = f128[sigma]
    gt = np.concatenate([fpos[0::2].real, fpos[1::2].real, fpos[0::2].imag, fpos[1::2].imag,
                         tw.real, tw.imag], axis=0).astype(np.float32)

    def pk(m):
        return np.stack([_pack_rows(x) for x in m])

    return pk(fc), pk(ic / 2048), gt


_FC, _IC, _GT = _build_consts()
assert all(sg == (1, 1) for sg in _INV_SIGNS)


def _bf(x_u32):
    return pltpu.bitcast(x_u32, _BF16)


def _pk(x_f32):
    return pltpu.bitcast(x_f32.astype(_BF16), _U32)


_STMODE = {"a": 1, "b": 1}


def _st(ref, x_f32, part="b"):
    if _STMODE[part]:
        ref.bitcast(_BF16)[...] = x_f32.astype(_BF16)
    else:
        ref[...] = _pk(x_f32)


def _pk2(x_f32):
    r = x_f32.shape[0] // 2
    return pltpu.pack_elementwise([x_f32[:r], x_f32[r:]], packed_dtype=_BF16)


def _dot(a, b):
    return jnp.dot(a, b, preferred_element_type=_F32)


def _val(p, like):
    if p is None:
        return jnp.zeros_like(like)
    return p[1] if p[0] > 0 else -p[1]


class _Head:
    def __init__(self, q, k, v, bq):
        self.q, self.k, self.v, self.bq = q, k, v, bq
        self.state = {}
        row = jax.lax.broadcasted_iota(jnp.int32, (128, 128), 0)
        col = jax.lax.broadcasted_iota(jnp.int32, (128, 128), 1)
        self.causal = col <= row

    def qk(self, i):
        bq = self.bq
        q0 = i * bq
        qq = self.q[q0:q0 + bq]
        nt = (q0 + bq) // 128
        mx = None
        ss = []
        for j in range(nt):
            r0 = max(0, j * 128 - q0)
            s = jax.lax.dot_general(qq[r0:], self.k[j * 128:(j + 1) * 128], _NT,
                                    preferred_element_type=_F32)
            if j * 128 >= q0:
                sd = jnp.where(self.causal, s[:128], _MASKED)
                s = jnp.concatenate([sd, s[128:]], axis=0) if s.shape[0] > 128 else sd
            ss.append(s)
            if mx is None:
                mx = s
            elif r0 == 0:
                mx = jnp.maximum(mx, s)
            else:
                mx = jnp.concatenate([mx[:r0], jnp.maximum(mx[r0:], s)], axis=0)
        self.state[i] = (ss, jnp.max(mx, axis=1, keepdims=True))

    def pv(self, i):
        bq = self.bq
        q0 = i * bq
        ss, m = self.state.pop(i)
        acc = None
        lsum = None
        for j, s in enumerate(ss):
            r0 = max(0, j * 128 - q0)
            p = jnp.exp2(s - m[r0:])
            pv = _dot(p.astype(_BF16), self.v[j * 128:(j + 1) * 128])
            if acc is None:
                acc, lsum = pv, p
            elif r0 == 0:
                acc, lsum = acc + pv, lsum + p
            else:
                acc = jnp.concatenate([acc[:r0], acc[r0:] + pv], axis=0)
                lsum = jnp.concatenate([lsum[:r0], lsum[r0:] + p], axis=0)
        l = jnp.sum(lsum, axis=1, keepdims=True)
        r = pl.reciprocal(l, approx=True)
        r = r * (2.0 - l * r)
        return acc * r


class _HeadWide(_Head):
    def qk(self, i):
        bq = self.bq
        q0 = i * bq
        parts = []
        for r in range(bq // 128):
            c0, c1 = (0, q0 + 128) if r == 0 else (q0 + 128 * r, q0 + 128 * (r + 1))
            s = jax.lax.dot_general(self.q[q0 + 128 * r:q0 + bq], self.k[c0:c1], _NT,
                                    preferred_element_type=_F32)
            w = c1 - c0
            top = jnp.where(self.causal, s[:128, w - 128:], _MASKED)
            if w > 128:
                top = jnp.concatenate([s[:128, :w - 128], top], axis=1)
            s = jnp.concatenate([top, s[128:]], axis=0) if s.shape[0] > 128 else top
            parts.append(s)
        mx = jnp.max(parts[0], axis=1, keepdims=True)
        for r in range(1, bq // 128):
            mr = jnp.max(parts[r], axis=1, keepdims=True)
            mx = jnp.concatenate([mx[:128 * r], jnp.maximum(mx[128 * r:], mr)], axis=0)
        self.state[i] = (parts, mx)

    def pv(self, i):
        bq = self.bq
        q0 = i * bq
        parts, m = self.state.pop(i)
        acc = l = None
        for r, s in enumerate(parts):
            c0, c1 = (0, q0 + 128) if r == 0 else (q0 + 128 * r, q0 + 128 * (r + 1))
            p = jnp.exp2(s - m[128 * r:])
            lr = jnp.sum(p, axis=1, keepdims=True)
            o = _dot(p.astype(_BF16), self.v[c0:c1])
            if r == 0:
                acc, l = o, lr
            else:
                acc = jnp.concatenate([acc[:128 * r], acc[128 * r:] + o], axis=0)
                l = jnp.concatenate([l[:128 * r], l[128 * r:] + lr], axis=0)
        rc = pl.reciprocal(l, approx=True)
        rc = rc * (2.0 - l * rc)
        return acc * rc


def _kernel(flag_ref, x_hbm, c_hbm, wq_hbm, wk_hbm, wv_hbm, wo_hbm, bx_hbm, wr_hbm, wi_hbm,
            fc_hbm, ic_hbm, gt_hbm,
            out_hbm,
            pad_s, x_s, c_s, wo_s, wq_s, wk_s, wv_s, qkv0_s, qkv1_s, ctx_s, oa_s,
            bx_s, wr_s, wi_s, wnr_s, wni_s, fc_s, ic_s, gt_s, gf_s, x1_s, nq_s, v_s, ob_s, u0_s, u1_s, u2_s, u3_s, q0_s, q1_s, vc_s,
            sem_bx, sem_misc, sem_w, sem_pair, sem_ob, sem_oa, *, bq, do_a, do_b, rg_rows, n_pre, frows, fill_slots, lookahead, dbg, wide, bx_win, w_at, b3_at):
    xh = x_hbm.bitcast(_U32)
    ch = c_hbm.bitcast(_U32)
    wqh = wq_hbm.bitcast(_U32)
    wkh = wk_hbm.bitcast(_U32)
    wvh = wv_hbm.bitcast(_U32)
    woh = wo_hbm.bitcast(_U32)
    bxh = bx_hbm.bitcast(_U32)
    wrh = wr_hbm.at[pl.ds(0, 512)].bitcast(_U32)
    wih = wi_hbm.at[pl.ds(0, 512)].bitcast(_U32)
    outh = out_hbm.bitcast(_U32)

    def bx_cp(p, par):
        return pltpu.make_async_copy(bxh.at[:, par * 8 + p], bx_s.at[p, par], sem_bx.at[2 * p + par])

    def w_cp(j, which):
        src, dst = (wrh, wr_s) if which == 0 else (wih, wi_s)
        return pltpu.make_async_copy(src.at[:, pl.ds(128 * j, 128)], dst.at[j], sem_w.at[2 * j + which])

    fc_cp = pltpu.make_async_copy(fc_hbm, fc_s, sem_misc.at[0])
    ic_cp = pltpu.make_async_copy(ic_hbm, ic_s, sem_misc.at[1])
    wnr_cp = pltpu.make_async_copy(wr_hbm.at[pl.ds(512, 1)], wnr_s, sem_misc.at[2])
    x_cp = pltpu.make_async_copy(xh, x_s, sem_misc.at[5])
    c_cp = pltpu.make_async_copy(ch, c_s, sem_misc.at[6])
    wo_cp = pltpu.make_async_copy(woh, wo_s, sem_misc.at[7])
    wni_cp = pltpu.make_async_copy(wi_hbm.at[pl.ds(512, 1)], wni_s, sem_misc.at[8])

    def pair_cps(p, slot):
        cps = []
        for i, (src, dst) in enumerate(((wqh, wq_s), (wkh, wk_s), (wvh, wv_s))):
            for par in range(2):
                cps.append(pltpu.make_async_copy(
                    src.at[:, par * 16 + p], dst.at[slot, par], sem_pair.at[slot * 6 + 2 * i + par]))
        return cps

    gt_cp = pltpu.make_async_copy(gt_hbm, gt_s, sem_misc.at[3])

    def start_a_inputs():
        x_cp.start()
        c_cp.start()
        for cp in pair_cps(0, 0) + pair_cps(1, 1):
            cp.start()

    if do_b:
        gt_cp.start()
        bx_cp(0, 0).start()
        bx_cp(0, 1).start()
        fc_cp.start()
        for p in range(1, bx_win):
            bx_cp(p, 0).start()
            bx_cp(p, 1).start()
        wnr_cp.start()
        wni_cp.start()
    if do_a and not do_b:
        start_a_inputs()

    fence = flag_ref[0] > 0

    if do_b:
        lane0 = jax.lax.broadcasted_iota(jnp.int32, (1, 128), 1) == 0
        row0 = jax.lax.broadcasted_iota(jnp.int32, (8, 128), 0) == 0

        gt_cp.wait()
        f_r, f_i = gt_s[pl.ds(0, 128), :], gt_s[pl.ds(128, 128), :]
        for ap in range(16):
            t_r, t_i = gt_s[pl.ds(256 + ap, 1), :], gt_s[pl.ds(272 + ap, 1), :]
            g_r = _pk2(f_r * t_r - f_i * t_i)
            g_i = _pk2(f_r * t_i + f_i * t_r)
            gf_s[ap] = jnp.concatenate([jnp.concatenate([g_r, g_i], axis=1),
                                        jnp.concatenate([g_i ^ jnp.uint32(0x80008000), g_r], axis=1)], axis=0)
        fc_cp.wait()

        def b1_step(p):
            bx_cp(p, 0).wait()
            bx_cp(p, 1).wait()
            if p + bx_win < 8:
                bx_cp(p + bx_win, 0).start()
                bx_cp(p + bx_win, 1).start()
            if p == w_at:
                for j in range(16):
                    w_cp(j, 0).start()
                    w_cp(j, 1).start()
            for h in range(2):
                halves = []
                for par in range(2):
                    xf = pltpu.unpack_elementwise(bx_s[p, par], index=h, packed_dtype=_BF16,
                                                  unpacked_dtype=_F32)
                    xs = [xf[:, 128 * n:128 * (n + 1)] for n in range(8)]
                    a_, b_ = xs[0] + xs[4], xs[0] - xs[4]
                    c_, d_ = xs[2] + xs[6], xs[2] - xs[6]
                    e_, f_ = xs[1] + xs[5], xs[1] - xs[5]
                    g_, h_ = xs[3] + xs[7], xs[3] - xs[7]
                    u_ = (f_ - h_) * _R2
                    v_ = (f_ + h_) * _R2
                    ac, eg = a_ + c_, e_ + g_
                    halves.append([ac + eg, ac - eg, b_ + u_, d_ + v_, a_ - c_, e_ - g_, b_ - u_, d_ - v_])
                pln = [jnp.concatenate([halves[0][i], halves[1][i]], axis=0).astype(_BF16)
                       for i in range(8)]
                ap = 2 * p + h
                f0 = _bf(fc_s[0, pl.ds(0, 64), :])
                o0 = jax.lax.dot_general(f0[:, 0:128], pln[0], _NT, preferred_element_type=_F32)
                o4 = jax.lax.dot_general(f0[:, 128:256], pln[1], _NT, preferred_element_type=_F32)
                nq = jnp.where(row0, o0[64:72], 0.0)
                im0 = jnp.concatenate([jnp.where(row0, 0.0, o0[64:72]), o0[72:128]], axis=0)
                nq_s[:, pl.ds(128 * ap, 128)] = _pk2(jnp.concatenate([nq, jnp.zeros_like(nq)], axis=0))
                x1_s[ap, 0] = jnp.concatenate(
                    [jnp.concatenate([_pk2(o0[0:64]), _pk2(o4[0:64])], axis=0),
                     jnp.concatenate([_pk2(im0), _pk2(o4[64:128])], axis=0)], axis=1)
                for j in (1, 2, 3):
                    rhs = jnp.concatenate([pln[2 * j], pln[2 * j + 1]], axis=1)
                    o = jax.lax.dot_general(_bf(fc_s[j]), rhs, _NT, preferred_element_type=_F32)
                    pk = _pk if dbg == 5 else _pk2
                    x1_s[ap, j] = jnp.concatenate([pk(o[0:128]), pk(o[128:256])], axis=1)

        for p in range(8):
            b1_step(p)

        def spectral(us, w_of):
            xs = _fft16(us, -1)
            qs = []
            for j in range(16):
                (sr, xr), (si, xi) = xs[j]
                wr, wi = w_of(j)
                qs.append((_sub((sr, xr * wr), (si, xi * wi)), _add((sr, xr * wi), (si, xi * wr))))
            res = _fft16(qs, +1)
            assert all(r[0][0] == 1 and r[1][0] == 1 for r in res)
            return [(r[0][1], r[1][1]) for r in res]

        u_s, q_s = (u0_s, u1_s, u2_s, u3_s), (q0_s, q1_s)

        def s_fwd(t, ap):
            u_s[t][ap] = _dot(_bf(x1_s[ap, t]), _bf(gf_s[ap]))

        def filt(t, half, ii):
            cls = _CLS[t][half]
            r0 = pl.multiple_of(64 * half + rg_rows * ii, rg_rows)
            rows = pl.ds(r0, rg_rows)
            wbase = pl.ds(pl.multiple_of(4 * rg_rows * ii, 4 * rg_rows), 4 * rg_rows)

            def w_of(j):
                return tuple(pltpu.unpack_elementwise(
                    ws.at[j, wbase][pl.ds(cls // 2, rg_rows, stride=4), :], index=cls % 2,
                    packed_dtype=_BF16, unpacked_dtype=_F32) for ws in (wr_s, wi_s))

            res = spectral([((1, u_s[t][ap, rows, pl.ds(0, 128)]), (1, u_s[t][ap, rows, pl.ds(128, 128)]))
                            for ap in range(16)], w_of)
            for ap in range(16):
                if rg_rows == 8:
                    q_s[t % 2][ap, rows, pl.ds(0, 128)] = res[ap][0]
                    q_s[t % 2][ap, rows, pl.ds(128, 128)] = res[ap][1]
                else:
                    qrows = pl.ds(pl.multiple_of(32 * half + (rg_rows // 2) * ii, rg_rows // 2), rg_rows // 2)
                    pk = _pk if dbg == 4 else _pk2
                    q_s[t % 2][ap, qrows, :] = jnp.concatenate([pk(res[ap][0]), pk(res[ap][1])], axis=1)

        def s_inv(t, ap):
            q = q_s[t % 2][ap].astype(_BF16) if rg_rows == 8 else _bf(q_s[t % 2][ap])
            o = jax.lax.dot_general(_bf(gf_s[ap]), q, _NT, preferred_element_type=_F32)
            vi = o[128:256]
            if t == 0:
                vi = jnp.where(lane0, vc_s[ap], vi)
            pk = _pk if dbg == 3 else _pk2
            v_s[ap, t] = jnp.concatenate([pk(o[0:128]), pk(vi)], axis=1)

        def nyquist(un):
            wnr = wnr_s[...].astype(_F32)
            wni = wni_s[...].astype(_F32)
            qn = spectral([((1, u[:, 0:128]), (1, u[:, 128:256])) for u in un],
                          lambda j: (wnr[:, 128 * j:128 * (j + 1)], wni[:, 128 * j:128 * (j + 1)]))
            for ap in range(16):
                lhs = jnp.concatenate([qn[ap][0], qn[ap][1]], axis=1).astype(_BF16)
                vn = jax.lax.dot_general(lhs, _bf(gf_s[ap, pl.ds(0, 64), :]), _NT,
                                         preferred_element_type=_F32)
                vn = jnp.concatenate([vn, jnp.zeros((112, 128), _F32)], axis=0)
                vc_s[ap] = vn.T

        def b2_head():
            un = [_dot(_bf(nq_s[:, pl.ds(128 * ap, 128)]), _bf(gf_s[ap, pl.ds(0, 64), :])) for ap in range(16)]
            for t in range(4):
                for ap in range(16):
                    s_fwd(t, ap)
                if t == 1:
                    nyquist(un)

        wnr_cp.wait()
        wni_cp.wait()
        pl.when(fence)(b2_head)
        for j in range(16):
            w_cp(j, 0).wait()
            w_cp(j, 1).wait()
        ic_cp.start()
        if do_a:
            start_a_inputs()
        nit = 64 // rg_rows
        for t in range(4):
            for half in range(2):
                def body(ii, carry, t=t, half=half):
                    filt(t, half, ii)
                    if t > 0:
                        for k in range(8 // nit):
                            s_inv(t - 1, 8 * half + (8 // nit) * ii + k)
                    return carry

                jax.lax.fori_loop(0, nit, body, 0)

        def b2_tail():
            for ap in range(16):
                s_inv(3, ap)

        pl.when(fence)(b2_tail)

        def ob_cp(p):
            return pltpu.make_async_copy(ob_s.at[p], outh.at[:, p, pl.ds(1024, 1024)], sem_ob.at[p])

        def b3():
            ic_cp.wait()

            for p in range(8):
                ys = []
                for h in range(2):
                    ap = 2 * p + h
                    cc = [_dot(_bf(v_s[ap, t]), _bf(ic_s[t])) for t in range(4)]
                    c0, c4 = cc[0][:, 0:128], cc[0][:, 128:256]
                    c1r, c1i = cc[1][:, 0:128], cc[1][:, 128:256]
                    c2r, c2i = cc[2][:, 0:128], cc[2][:, 128:256]
                    c3r, c3i = cc[3][:, 0:128], cc[3][:, 128:256]
                    pp, mm = c0 + c4, c0 - c4
                    u1, u2, u3, u4 = c1r + c3r, c1i - c3i, c1r - c3r, c1i + c3i
                    t1, t2 = (u3 - u4) * _R2, (u3 + u4) * _R2
                    e0, e1, e2, e3 = pp + c2r, pp - c2r, mm - c2i, mm + c2i
                    ys.append([e0 + u1, e2 + t1, e1 - u2, e3 - t2, e0 - u1, e2 - t1, e1 + u2, e3 + t2])
                ob_s[p] = jnp.concatenate([pltpu.pack_elementwise([ys[0][n], ys[1][n]], packed_dtype=_BF16)
                                           for n in range(8)], axis=1)
                ob_cp(p).start()

        if b3_at == 0 or not do_a:
            b3()

    if do_a:
        x_cp.wait()
        c_cp.wait()

        def project_units(slot, half, dst, rows):
            def split(ref):
                a = ref[slot, 0]
                b = ref[slot, 1]
                if half == 1:
                    a, b = a >> 16, b >> 16
                return _bf(pltpu.pack_elementwise([a, b], packed_dtype=jnp.uint16))

            wq = split(wq_s)
            wkv = jnp.concatenate([split(wk_s), split(wv_s)], axis=1)

            def q_unit(r0):
                q = _dot(_bf(x_s[pl.ds(r0 // 2, rows // 2), :]), wq) * _QSCALE
                _st(dst.at[pl.ds(r0 // 2, rows // 2), pl.ds(0, 128)], q, 'a')

            def kv_unit(r0):
                kv = _dot(_bf(c_s[pl.ds(r0 // 2, rows // 2), :]), wkv)
                _st(dst.at[pl.ds(r0 // 2, rows // 2), pl.ds(128, 256)], kv, 'a')

            units = []
            for r0 in range(0, S, rows):
                units.append(functools.partial(kv_unit, r0))
                units.append(functools.partial(q_unit, r0))
            return units

        def attend(p, t, src, fillers):
            head = (_HeadWide if wide else _Head)(*[_bf(src[:, pl.ds(128 * i, 128)]) for i in range(3)], bq)
            ns = S // bq
            fillers = list(fillers)
            nslots = ns * fill_slots
            total = len(fillers)
            slot = [0]

            def fill():
                slot[0] += 1
                while fillers and (total - len(fillers)) * nslots < total * slot[0]:
                    fillers.pop(0)()

            outs = []
            head.qk(0)
            for i in range(ns):
                if i + 1 < ns:
                    head.qk(i + 1)
                if fill_slots == 2:
                    fill()
                outs.append(head.pv(i))
                fill()
            _st(ctx_s.at[p, :, pl.ds(t * 128, 128)], jnp.concatenate(outs, axis=0), 'a')
            while fillers:
                fillers.pop(0)()

        npair = H // 2
        for cp in pair_cps(0, 0):
            cp.wait()
        for u in project_units(0, 0, qkv0_s, 2048):
            u()

        def pair_step(p, last):
            s0 = p % 3
            attend(p, 0, qkv0_s, project_units(s0, 1, qkv1_s, frows))
            if last:
                attend(p, 1, qkv1_s, [])
            else:
                attend(p, 1, qkv1_s, project_units((p + 1) % 3, 0, qkv0_s, frows))

        def a_body(p, carry):
            for cp in pair_cps(p + 1, (p + 1) % 3):
                cp.wait()

            @pl.when(p + 2 < npair)
            def _():
                for cp in pair_cps(p + 2, (p + 2) % 3):
                    cp.start()

            @pl.when(p == 2)
            def _():
                wo_cp.start()

            pl.when(fence)(lambda: pair_step(p, False))
            return carry

        jax.lax.fori_loop(0, npair - 1, a_body, 0)
        if b3_at == 1 and do_b:
            b3()
        pair_step(npair - 1, True)
        if b3_at == 2 and do_b:
            b3()

        wo_cp.wait()

        def oa_cp(i):
            return pltpu.make_async_copy(oa_s.at[i % 2], outh.at[pl.ds(16 * i, 16), :, pl.ds(0, 1024)],
                                         sem_oa.at[i % 2])

        def o_body(i, carry):
            r0 = pl.multiple_of(i * 128, 128)
            lhs = _bf(jnp.concatenate([ctx_s[p, pl.ds(r0, 128), :] for p in range(H // 2)], axis=1))
            res = _dot(lhs, _bf(wo_s[...]))

            @pl.when(i >= 2)
            def _():
                oa_cp(i - 2).wait()

            _st(oa_s.at[i % 2], res.reshape(16, 16, M))
            oa_cp(i).start()
            return carry

        jax.lax.fori_loop(0, 8, o_body, 0)
        oa_cp(6).wait()
        oa_cp(7).wait()

    if do_b:
        for p in range(8):
            ob_cp(p).wait()


def _run(A_x, A_c_kv, A_w_q, A_w_uk, A_w_uv, A_w_o, B_x, B_w_r, B_w_i, *, bq=256, do_a=True, do_b=True, rg_rows=16, n_pre=1, frows=128, fill_slots=2, lookahead=1, dbg=0, wide=True, bx_win=3, w_at=7, b3_at=0, pad=8, sta=0, stb=0, flags=None):
    _STMODE['a'], _STMODE['b'] = sta, stb
    any_spec = pl.BlockSpec(memory_space=pltpu.HBM)
    vm = pltpu.VMEM
    dma = pltpu.SemaphoreType.DMA
    scratch = [
        vm((pad, 128), _U32),
        vm((1024, 1024), _U32),
        vm((1024, 512), _U32),
        vm((2048, 1024), _U32),
        vm((3, 2, 512, 128), _U32),
        vm((3, 2, 256, 128), _U32),
        vm((3, 2, 256, 128), _U32),
        vm((1024, 384), _U32), vm((1024, 384), _U32),
        vm((16, 1024, 256), _U32),
        vm((2, 16, 8, 1024), _U32),
        vm((8, 2, 64, 1024), _U32),
        vm((16, 256, 128), _U32),
        vm((16, 256, 128), _U32),
        vm((1, 2048), _BF16),
        vm((1, 2048), _BF16),
        vm((4, 128, 256), _U32),
        vm((4, 128, 256), _U32),
        vm((288, 128), _F32),
        vm((16, 128, 256), _U32),
        vm((16, 4, 64, 256), _U32),
        vm((8, 2048), _U32),
        vm((16, 4, 64, 256), _U32),
        vm((8, 128, 1024), _U32),
        vm((16, 128, 256), _F32), vm((16, 128, 256), _F32), vm((16, 128, 256), _F32), vm((16, 128, 256), _F32),
        *([vm((16, 128, 256), _F32)] * 2 if rg_rows == 8 else [vm((16, 64, 256), _U32)] * 2),
        vm((16, 128, 128), _F32),
        dma((16,)), dma((9,)), dma((32,)), dma((18,)), dma((8,)), dma((2,)),
    ]
    out = pl.pallas_call(
        functools.partial(_kernel, bq=bq, do_a=do_a, do_b=do_b, rg_rows=rg_rows, n_pre=n_pre, frows=frows, fill_slots=fill_slots, lookahead=lookahead, dbg=dbg, wide=wide, bx_win=bx_win, w_at=w_at, b3_at=b3_at),
        out_shape=jax.ShapeDtypeStruct((128, 16, 2048), _BF16),
        in_specs=[pl.BlockSpec(memory_space=pltpu.SMEM)] + [any_spec] * 12,
        out_specs=any_spec,
        scratch_shapes=scratch,
        compiler_params=pltpu.CompilerParams(vmem_limit_bytes=112 * 1024 * 1024, flags=flags),
    )(jnp.asarray(np.ones((1,), np.int32)), *[pltpu.with_memory_space_constraint(a, pltpu.HBM) for a in (
        A_x.reshape(S, M), A_c_kv.reshape(S, DC),
        A_w_q.reshape(512, 64, HD), A_w_uk.reshape(256, 64, HD), A_w_uv.reshape(256, 64, HD),
        A_w_o.reshape(H * HD, M),
        B_x.reshape(64, 32, BD), B_w_r.T, B_w_i.T,
        jnp.asarray(_FC), jnp.asarray(_IC), jnp.asarray(_GT),
    )])
    return out.reshape(1, S, 2048)


@jax.jit
def pallas_concat_heads__compressed_kv_cla__spectral_gfnet__prompt_kernel(
    A_x: jax.Array,
    A_c_kv: jax.Array,
    A_w_q: jax.Array,
    A_w_uk: jax.Array,
    A_w_uv: jax.Array,
    A_w_o: jax.Array,
    B_x: jax.Array,
    B_w_r: jax.Array,
    B_w_i: jax.Array,
):
    return _run(A_x, A_c_kv, A_w_q, A_w_uk, A_w_uv, A_w_o, B_x, B_w_r, B_w_i)
```

```python
import functools

import numpy as np
import jax
import jax.numpy as jnp
import jax.experimental.pallas as pl
import jax.experimental.pallas.tpu as pltpu

S = 2048
M = 1024
H = 32
HD = 128
DC = 512
BD = 1024
NG = 8

_U32 = jnp.uint32
_BF16 = jnp.bfloat16
_F32 = jnp.float32
_NT = (((1,), (1,)), ((), ()))
_QSCALE = float(HD ** -0.5 * np.log2(np.e))
_MASKED = -1e9


def _to_bf16_bits(a):
    u = np.ascontiguousarray(a, dtype=np.float32).view(np.uint32).astype(np.uint64)
    r = (u + 0x7FFF + ((u >> 16) & 1)) >> 16
    return r.astype(np.uint32) & 0xFFFF


def _pack_rows(a):
    b = _to_bf16_bits(a)
    return (b[0::2] | (b[1::2] << 16)).astype(np.uint32)


def _neg(p):
    return None if p is None else (-p[0], p[1])


def _add(p, q):
    if p is None:
        return q
    if q is None:
        return p
    if p[0] == q[0]:
        return (p[0], p[1] + q[1])
    if p[0] > 0:
        return (1, p[1] - q[1])
    return (1, q[1] - p[1])


def _sub(p, q):
    return _add(p, _neg(q))


def _scale(p, f):
    if p is None:
        return None
    return (p[0] * (1 if f > 0 else -1), p[1] * abs(f))


def _cadd(x, y):
    return (_add(x[0], y[0]), _add(x[1], y[1]))


def _csub(x, y):
    return (_sub(x[0], y[0]), _sub(x[1], y[1]))


def _cmul_i(x, s):
    return (_neg(x[1]), x[0]) if s > 0 else (x[1], _neg(x[0]))


def _cmul_w(x, n, sgn):
    n = n % 16
    if n == 0:
        return x
    if n == 4:
        return _cmul_i(x, sgn)
    if n == 8:
        return (_neg(x[0]), _neg(x[1]))
    if n == 12:
        return _cmul_i(x, -sgn)
    wr = float(np.cos(2 * np.pi * n / 16))
    wi = float(sgn * np.sin(2 * np.pi * n / 16))
    re, im = x
    if n % 2 == 0:
        r = abs(wr)
        sr = 1 if wr > 0 else -1
        si = 1 if wi > 0 else -1
        a = _sub(re if sr > 0 else _neg(re), im if si > 0 else _neg(im))
        b = _add(re if si > 0 else _neg(re), im if sr > 0 else _neg(im))
        return (_scale(a, r), _scale(b, r))
    return (_sub(_scale(re, wr), _scale(im, wi)), _add(_scale(re, wi), _scale(im, wr)))


def _dft4(x0, x1, x2, x3, sgn):
    s02, d02 = _cadd(x0, x2), _csub(x0, x2)
    s13, d13 = _cadd(x1, x3), _csub(x1, x3)
    r = _cmul_i(d13, sgn)
    return [_cadd(s02, s13), _cadd(d02, r), _csub(s02, s13), _csub(d02, r)]


def _fft16(xs, sgn):
    t = [_dft4(xs[a0], xs[4 + a0], xs[8 + a0], xs[12 + a0], sgn) for a0 in range(4)]
    t = [[_cmul_w(t[a0][j0], a0 * j0, sgn) for j0 in range(4)] for a0 in range(4)]
    out = [None] * 16
    for j0 in range(4):
        r = _dft4(t[0][j0], t[1][j0], t[2][j0], t[3][j0], sgn)
        for j1 in range(4):
            out[j0 + 4 * j1] = r[j1]
    return out


def _net_signs(sgn):
    out = _fft16([((1, 1.0), (1, 1.0)) for _ in range(16)], sgn)
    return [(o[0][0], o[1][0]) for o in out]


_INV_SIGNS = _net_signs(+1)
_CLS = ((0, 4), (1, 7), (2, 6), (3, 5))
_R2 = float(np.sqrt(0.5))


def _build_consts():
    n2 = np.arange(128)
    kap = np.arange(64)

    def wl(l):
        return np.exp(-2j * np.pi * np.outer(l, n2) / 1024)

    fc = np.zeros((4, 256, 256))
    w = wl(8 * kap)
    fc[0, 0:64, 0:128] = w.real
    fc[0, 64:128, 0:128] = w.imag
    fc[0, 64, 0:128] = (-1.0) ** n2
    w = wl(4 + 8 * kap)
    fc[0, 0:64, 128:256] = w.real
    fc[0, 64:128, 128:256] = w.imag
    for j in (1, 2, 3):
        si = 1.0 if j == 3 else -1.0
        w1, w2 = wl(j + 8 * kap), wl(8 - j + 8 * kap)
        fc[j, 0:64, 0:128], fc[j, 0:64, 128:] = w1.real, -w1.imag * si
        fc[j, 64:128, 0:128], fc[j, 64:128, 128:] = w2.real, w2.imag * si
        fc[j, 128:192, 0:128], fc[j, 128:192, 128:] = w1.imag, w1.real * si
        fc[j, 192:256, 0:128], fc[j, 192:256, 128:] = w2.imag, -w2.real * si

    def cs(l, c):
        ph = 2 * np.pi * np.outer(l, n2) / 1024
        return c[:, None] * np.cos(ph) / 1024, c[:, None] * np.sin(ph) / 1024

    ic = np.zeros((4, 256, 256))
    two = np.full(64, 2.0)
    co, si = cs(8 * kap, np.where(kap == 0, 1.0, 2.0))
    ic[0, 0:64, 0:128], ic[0, 128:192, 0:128] = co, -si
    ic[0, 128, 0:128] = (-1.0) ** n2 / 1024
    co, si = cs(4 + 8 * kap, two)
    ic[0, 64:128, 128:], ic[0, 192:256, 128:] = co, -si
    for j in (1, 2, 3):
        co, si = cs(j + 8 * kap, two)
        ic[j, 0:64, 0:128], ic[j, 128:192, 0:128] = co, -si
        ic[j, 0:64, 128:], ic[j, 128:192, 128:] = si, co
        co, si = cs(8 - j + 8 * kap, two)
        ic[j, 64:128, 0:128], ic[j, 192:256, 0:128] = co, -si
        ic[j, 64:128, 128:], ic[j, 192:256, 128:] = -si, -co

    f128 = np.exp(-2j * np.pi * np.outer(n2, n2) / 128)
    tw = np.exp(-2j * np.pi * np.outer(np.arange(16), n2) / 2048)

    def even_odd(m, blk):
        r = m.reshape(-1, blk // 2, 2, m.shape[-1])
        return np.concatenate([r[:, :, 0], r[:, :, 1]], axis=1).reshape(m.shape)

    fc[0] = even_odd(fc[0], 64)
    for j in (1, 2, 3):
        fc[j] = even_odd(fc[j], 128)
    il = np.arange(256).reshape(16, 2, 8).transpose(0, 2, 1).reshape(-1)
    ic = ic[:, il, :]
    sigma = np.concatenate([np.arange(0, 128, 2), np.arange(1, 128, 2)])
    fpos = f128[sigma]
    gt = np.concatenate([fpos[0::2].real, fpos[1::2].real, fpos[0::2].imag, fpos[1::2].imag,
                         tw.real, tw.imag], axis=0).astype(np.float32)

    def pk(m):
        return np.stack([_pack_rows(x) for x in m])

    return pk(fc), pk(ic / 2048), gt


_FC, _IC, _GT = _build_consts()
assert all(sg == (1, 1) for sg in _INV_SIGNS)


def _bf(x_u32):
    return pltpu.bitcast(x_u32, _BF16)


def _pk(x_f32):
    return pltpu.bitcast(x_f32.astype(_BF16), _U32)


_STMODE = {"a": 1, "b": 1}


def _st(ref, x_f32, part="b"):
    if _STMODE[part]:
        ref.bitcast(_BF16)[...] = x_f32.astype(_BF16)
    else:
        ref[...] = _pk(x_f32)


def _pk2(x_f32):
    r = x_f32.shape[0] // 2
    return pltpu.pack_elementwise([x_f32[:r], x_f32[r:]], packed_dtype=_BF16)


def _dot(a, b):
    return jnp.dot(a, b, preferred_element_type=_F32)


def _val(p, like):
    if p is None:
        return jnp.zeros_like(like)
    return p[1] if p[0] > 0 else -p[1]


class _Head:
    def __init__(self, q, k, v, bq):
        self.q, self.k, self.v, self.bq = q, k, v, bq
        self.state = {}
        row = jax.lax.broadcasted_iota(jnp.int32, (128, 128), 0)
        col = jax.lax.broadcasted_iota(jnp.int32, (128, 128), 1)
        self.causal = col <= row

    def qk(self, i):
        bq = self.bq
        q0 = i * bq
        qq = self.q[q0:q0 + bq]
        nt = (q0 + bq) // 128
        mx = None
        ss = []
        for j in range(nt):
            r0 = max(0, j * 128 - q0)
            s = jax.lax.dot_general(qq[r0:], self.k[j * 128:(j + 1) * 128], _NT,
                                    preferred_element_type=_F32)
            if j * 128 >= q0:
                sd = jnp.where(self.causal, s[:128], _MASKED)
                s = jnp.concatenate([sd, s[128:]], axis=0) if s.shape[0] > 128 else sd
            ss.append(s)
            if mx is None:
                mx = s
            elif r0 == 0:
                mx = jnp.maximum(mx, s)
            else:
                mx = jnp.concatenate([mx[:r0], jnp.maximum(mx[r0:], s)], axis=0)
        self.state[i] = (ss, jnp.max(mx, axis=1, keepdims=True))

    def pv(self, i):
        bq = self.bq
        q0 = i * bq
        ss, m = self.state.pop(i)
        acc = None
        lsum = None
        for j, s in enumerate(ss):
            r0 = max(0, j * 128 - q0)
            p = jnp.exp2(s - m[r0:])
            pv = _dot(p.astype(_BF16), self.v[j * 128:(j + 1) * 128])
            if acc is None:
                acc, lsum = pv, p
            elif r0 == 0:
                acc, lsum = acc + pv, lsum + p
            else:
                acc = jnp.concatenate([acc[:r0], acc[r0:] + pv], axis=0)
                lsum = jnp.concatenate([lsum[:r0], lsum[r0:] + p], axis=0)
        l = jnp.sum(lsum, axis=1, keepdims=True)
        r = pl.reciprocal(l, approx=True)
        r = r * (2.0 - l * r)
        return acc * r


class _HeadWide(_Head):
    def qk(self, i):
        bq = self.bq
        q0 = i * bq
        parts = []
        for r in range(bq // 128):
            c0, c1 = (0, q0 + 128) if r == 0 else (q0 + 128 * r, q0 + 128 * (r + 1))
            s = jax.lax.dot_general(self.q[q0 + 128 * r:q0 + bq], self.k[c0:c1], _NT,
                                    preferred_element_type=_F32)
            w = c1 - c0
            top = jnp.where(self.causal, s[:128, w - 128:], _MASKED)
            if w > 128:
                top = jnp.concatenate([s[:128, :w - 128], top], axis=1)
            s = jnp.concatenate([top, s[128:]], axis=0) if s.shape[0] > 128 else top
            parts.append(s)
        mx = jnp.max(parts[0], axis=1, keepdims=True)
        for r in range(1, bq // 128):
            mr = jnp.max(parts[r], axis=1, keepdims=True)
            mx = jnp.concatenate([mx[:128 * r], jnp.maximum(mx[128 * r:], mr)], axis=0)
        self.state[i] = (parts, mx)

    def pv(self, i):
        bq = self.bq
        q0 = i * bq
        parts, m = self.state.pop(i)
        acc = l = None
        for r, s in enumerate(parts):
            c0, c1 = (0, q0 + 128) if r == 0 else (q0 + 128 * r, q0 + 128 * (r + 1))
            p = jnp.exp2(s - m[128 * r:])
            lr = jnp.sum(p, axis=1, keepdims=True)
            o = _dot(p.astype(_BF16), self.v[c0:c1])
            if r == 0:
                acc, l = o, lr
            else:
                acc = jnp.concatenate([acc[:128 * r], acc[128 * r:] + o], axis=0)
                l = jnp.concatenate([l[:128 * r], l[128 * r:] + lr], axis=0)
        rc = pl.reciprocal(l, approx=True)
        rc = rc * (2.0 - l * rc)
        return acc * rc


def _kernel(flag_ref, x_hbm, c_hbm, wq_hbm, wk_hbm, wv_hbm, wo_hbm, bx_hbm, wr_hbm, wi_hbm,
            fc_hbm, ic_hbm, gt_hbm,
            out_hbm,
            pad_s, x_s, c_s, wo_s, wq_s, wk_s, wv_s, qkv0_s, qkv1_s, ctx_s, oa_s,
            bx_s, wr_s, wi_s, wnr_s, wni_s, fc_s, ic_s, gt_s, gf_s, x1_s, nq_s, v_s, ob_s, u0_s, u1_s, u2_s, u3_s, q0_s, q1_s, vc_s,
            sem_bx, sem_misc, sem_w, sem_pair, sem_ob, sem_oa, *, bq, do_a, do_b, rg_rows, n_pre, frows, fill_slots, lookahead, dbg, wide, bx_win, w_at, b3_at, b3_p, sorder, last_cfg):
    xh = x_hbm.bitcast(_U32)
    ch = c_hbm.bitcast(_U32)
    wqh = wq_hbm.bitcast(_U32)
    wkh = wk_hbm.bitcast(_U32)
    wvh = wv_hbm.bitcast(_U32)
    woh = wo_hbm.bitcast(_U32)
    bxh = bx_hbm.bitcast(_U32)
    wrh = wr_hbm.at[pl.ds(0, 512)].bitcast(_U32)
    wih = wi_hbm.at[pl.ds(0, 512)].bitcast(_U32)
    outh = out_hbm.bitcast(_U32)

    def bx_cp(p, par):
        return pltpu.make_async_copy(bxh.at[:, par * 8 + p], bx_s.at[p, par], sem_bx.at[2 * p + par])

    def w_cp(j, which):
        src, dst = (wrh, wr_s) if which == 0 else (wih, wi_s)
        return pltpu.make_async_copy(src.at[:, pl.ds(128 * j, 128)], dst.at[j], sem_w.at[2 * j + which])

    fc_cp = pltpu.make_async_copy(fc_hbm, fc_s, sem_misc.at[0])
    ic_cp = pltpu.make_async_copy(ic_hbm, ic_s, sem_misc.at[1])
    wnr_cp = pltpu.make_async_copy(wr_hbm.at[pl.ds(512, 1)], wnr_s, sem_misc.at[2])
    x_cp = pltpu.make_async_copy(xh, x_s, sem_misc.at[5])
    c_cp = pltpu.make_async_copy(ch, c_s, sem_misc.at[6])
    wo_cp = pltpu.make_async_copy(woh, wo_s, sem_misc.at[7])
    wni_cp = pltpu.make_async_copy(wi_hbm.at[pl.ds(512, 1)], wni_s, sem_misc.at[8])

    def pair_cps(p, slot):
        cps = []
        for i, (src, dst) in enumerate(((wqh, wq_s), (wkh, wk_s), (wvh, wv_s))):
            for par in range(2):
                cps.append(pltpu.make_async_copy(
                    src.at[:, par * 16 + p], dst.at[slot, par], sem_pair.at[slot * 6 + 2 * i + par]))
        return cps

    gt_cp = pltpu.make_async_copy(gt_hbm, gt_s, sem_misc.at[3])

    def start_a_inputs():
        x_cp.start()
        c_cp.start()
        for cp in pair_cps(0, 0) + pair_cps(1, 1):
            cp.start()

    if do_b:
        gt_cp.start()
        fc_cp.start()
        bx_cp(0, 0).start()
        bx_cp(0, 1).start()
        for p in range(1, bx_win):
            bx_cp(p, 0).start()
            bx_cp(p, 1).start()
        wnr_cp.start()
        wni_cp.start()
    if do_a and not do_b:
        start_a_inputs()

    fence = flag_ref[0] > 0

    if do_b:
        lane0 = jax.lax.broadcasted_iota(jnp.int32, (1, 128), 1) == 0
        row0 = jax.lax.broadcasted_iota(jnp.int32, (8, 128), 0) == 0

        gt_cp.wait()
        f_r, f_i = gt_s[pl.ds(0, 128), :], gt_s[pl.ds(128, 128), :]
        for ap in range(16):
            t_r, t_i = gt_s[pl.ds(256 + ap, 1), :], gt_s[pl.ds(272 + ap, 1), :]
            g_r = _pk2(f_r * t_r - f_i * t_i)
            g_i = _pk2(f_r * t_i + f_i * t_r)
            gf_s[ap] = jnp.concatenate([jnp.concatenate([g_r, g_i], axis=1),
                                        jnp.concatenate([g_i ^ jnp.uint32(0x80008000), g_r], axis=1)], axis=0)
        fc_cp.wait()

        def b1_step(p):
            bx_cp(p, 0).wait()
            bx_cp(p, 1).wait()
            if p + bx_win < 8:
                bx_cp(p + bx_win, 0).start()
                bx_cp(p + bx_win, 1).start()
            if p == w_at:
                for j in range(16):
                    w_cp(j, 0).start()
                    w_cp(j, 1).start()
            for h in range(2):
                halves = []
                for par in range(2):
                    xf = pltpu.unpack_elementwise(bx_s[p, par], index=h, packed_dtype=_BF16,
                                                  unpacked_dtype=_F32)
                    xs = [xf[:, 128 * n:128 * (n + 1)] for n in range(8)]
                    a_, b_ = xs[0] + xs[4], xs[0] - xs[4]
                    c_, d_ = xs[2] + xs[6], xs[2] - xs[6]
                    e_, f_ = xs[1] + xs[5], xs[1] - xs[5]
                    g_, h_ = xs[3] + xs[7], xs[3] - xs[7]
                    u_ = (f_ - h_) * _R2
                    v_ = (f_ + h_) * _R2
                    ac, eg = a_ + c_, e_ + g_
                    halves.append([ac + eg, ac - eg, b_ + u_, d_ + v_, a_ - c_, e_ - g_, b_ - u_, d_ - v_])
                pln = [jnp.concatenate([halves[0][i], halves[1][i]], axis=0).astype(_BF16)
                       for i in range(8)]
                ap = 2 * p + h
                f0 = _bf(fc_s[0, pl.ds(0, 64), :])
                o0 = jax.lax.dot_general(f0[:, 0:128], pln[0], _NT, preferred_element_type=_F32)
                o4 = jax.lax.dot_general(f0[:, 128:256], pln[1], _NT, preferred_element_type=_F32)
                nq = jnp.where(row0, o0[64:72], 0.0)
                im0 = jnp.concatenate([jnp.where(row0, 0.0, o0[64:72]), o0[72:128]], axis=0)
                nq_s[:, pl.ds(128 * ap, 128)] = _pk2(jnp.concatenate([nq, jnp.zeros_like(nq)], axis=0))
                x1_s[ap, 0] = jnp.concatenate(
                    [jnp.concatenate([_pk2(o0[0:64]), _pk2(o4[0:64])], axis=0),
                     jnp.concatenate([_pk2(im0), _pk2(o4[64:128])], axis=0)], axis=1)
                for j in (1, 2, 3):
                    rhs = jnp.concatenate([pln[2 * j], pln[2 * j + 1]], axis=1)
                    o = jax.lax.dot_general(_bf(fc_s[j]), rhs, _NT, preferred_element_type=_F32)
                    pk = _pk if dbg == 5 else _pk2
                    x1_s[ap, j] = jnp.concatenate([pk(o[0:128]), pk(o[128:256])], axis=1)

        for p in range(8):
            b1_step(p)

        def spectral(us, w_of):
            xs = _fft16(us, -1)
            qs = []
            for j in range(16):
                (sr, xr), (si, xi) = xs[j]
                wr, wi = w_of(j)
                qs.append((_sub((sr, xr * wr), (si, xi * wi)), _add((sr, xr * wi), (si, xi * wr))))
            res = _fft16(qs, +1)
            assert all(r[0][0] == 1 and r[1][0] == 1 for r in res)
            return [(r[0][1], r[1][1]) for r in res]

        u_s, q_s = (u0_s, u1_s, u2_s, u3_s), (q0_s, q1_s)

        def s_fwd(t, ap):
            u_s[t][ap] = _dot(_bf(x1_s[ap, t]), _bf(gf_s[ap]))

        def filt(t, half, ii):
            cls = _CLS[t][half]
            r0 = pl.multiple_of(64 * half + rg_rows * ii, rg_rows)
            rows = pl.ds(r0, rg_rows)
            wbase = pl.ds(pl.multiple_of(4 * rg_rows * ii, 4 * rg_rows), 4 * rg_rows)

            def w_of(j):
                return tuple(pltpu.unpack_elementwise(
                    ws.at[j, wbase][pl.ds(cls // 2, rg_rows, stride=4), :], index=cls % 2,
                    packed_dtype=_BF16, unpacked_dtype=_F32) for ws in (wr_s, wi_s))

            res = spectral([((1, u_s[t][ap, rows, pl.ds(0, 128)]), (1, u_s[t][ap, rows, pl.ds(128, 128)]))
                            for ap in range(16)], w_of)
            for ap in range(16):
                if rg_rows == 8:
                    q_s[t % 2][ap, rows, pl.ds(0, 128)] = res[ap][0]
                    q_s[t % 2][ap, rows, pl.ds(128, 128)] = res[ap][1]
                else:
                    qrows = pl.ds(pl.multiple_of(32 * half + (rg_rows // 2) * ii, rg_rows // 2), rg_rows // 2)
                    pk = _pk if dbg == 4 else _pk2
                    q_s[t % 2][ap, qrows, :] = jnp.concatenate([pk(res[ap][0]), pk(res[ap][1])], axis=1)

        def s_inv(t, ap):
            q = q_s[t % 2][ap].astype(_BF16) if rg_rows == 8 else _bf(q_s[t % 2][ap])
            o = jax.lax.dot_general(_bf(gf_s[ap]), q, _NT, preferred_element_type=_F32)
            vi = o[128:256]
            if t == 0:
                vi = jnp.where(lane0, vc_s[ap], vi)
            pk = _pk if dbg == 3 else _pk2
            v_s[ap, t] = jnp.concatenate([pk(o[0:128]), pk(vi)], axis=1)

        def nyquist(un):
            wnr = wnr_s[...].astype(_F32)
            wni = wni_s[...].astype(_F32)
            qn = spectral([((1, u[:, 0:128]), (1, u[:, 128:256])) for u in un],
                          lambda j: (wnr[:, 128 * j:128 * (j + 1)], wni[:, 128 * j:128 * (j + 1)]))
            for ap in range(16):
                lhs = jnp.concatenate([qn[ap][0], qn[ap][1]], axis=1).astype(_BF16)
                vn = jax.lax.dot_general(lhs, _bf(gf_s[ap, pl.ds(0, 64), :]), _NT,
                                         preferred_element_type=_F32)
                vn = jnp.concatenate([vn, jnp.zeros((112, 128), _F32)], axis=0)
                vc_s[ap] = vn.T

        def b2_head():
            un = [_dot(_bf(nq_s[:, pl.ds(128 * ap, 128)]), _bf(gf_s[ap, pl.ds(0, 64), :])) for ap in range(16)]
            for ap in range(16):
                u = _dot(_bf(x1_s[ap, 0:n_pre].reshape(64 * n_pre, 256)), _bf(gf_s[ap]))
                for t in range(n_pre):
                    u_s[t][ap] = u[128 * t:128 * (t + 1)]
                if ap == 7:
                    nyquist(un)

        wnr_cp.wait()
        wni_cp.wait()
        pl.when(fence)(b2_head)
        for j in range(16):
            w_cp(j, 0).wait()
            w_cp(j, 1).wait()
        ic_cp.start()
        if do_a:
            start_a_inputs()
        nit = 64 // rg_rows
        for t in range(4):
            for half in range(2):
                def body(ii, carry, t=t, half=half):
                    filt(t, half, ii)
                    for k in range(8 // nit):
                        if t + n_pre < 4:
                            s_fwd(t + n_pre, 8 * half + (8 // nit) * ii + k)
                        if t > 0:
                            s_inv(t - 1, 8 * half + (8 // nit) * ii + k)
                    return carry

                jax.lax.fori_loop(0, nit, body, 0)

        def b2_tail():
            for ap in range(16):
                s_inv(3, ap)

        pl.when(fence)(b2_tail)

        def ob_cp(p):
            return pltpu.make_async_copy(ob_s.at[p], outh.at[:, p, pl.ds(1024, 1024)], sem_ob.at[p])

        def b3():
            ic_cp.wait()

            for pq in range(8 // b3_p):
                aps = range(2 * b3_p * pq, 2 * b3_p * (pq + 1))
                cc = [_dot(_bf(jnp.concatenate([v_s[ap, t] for ap in aps], axis=0)), _bf(ic_s[t]))
                      for t in range(4)]
                c0, c4 = cc[0][:, 0:128], cc[0][:, 128:256]
                c1r, c1i = cc[1][:, 0:128], cc[1][:, 128:256]
                c2r, c2i = cc[2][:, 0:128], cc[2][:, 128:256]
                c3r, c3i = cc[3][:, 0:128], cc[3][:, 128:256]
                pp, mm = c0 + c4, c0 - c4
                u1, u2, u3, u4 = c1r + c3r, c1i - c3i, c1r - c3r, c1i + c3i
                t1, t2 = (u3 - u4) * _R2, (u3 + u4) * _R2
                e0, e1, e2, e3 = pp + c2r, pp - c2r, mm - c2i, mm + c2i
                ys = [e0 + u1, e2 + t1, e1 - u2, e3 - t2, e0 - u1, e2 - t1, e1 + u2, e3 + t2]
                for k in range(b3_p):
                    p = b3_p * pq + k
                    ob_s[p] = jnp.concatenate(
                        [pltpu.pack_elementwise([y[256 * k:256 * k + 128], y[256 * k + 128:256 * k + 256]],
                                                packed_dtype=_BF16) for y in ys], axis=1)
                    ob_cp(p).start()

        if b3_at == 0 or not do_a:
            b3()

    if do_a:
        x_cp.wait()
        c_cp.wait()

        def project_units(slot, half, dst, rows):
            def split(ref):
                a = ref[slot, 0]
                b = ref[slot, 1]
                if half == 1:
                    a, b = a >> 16, b >> 16
                return _bf(pltpu.pack_elementwise([a, b], packed_dtype=jnp.uint16))

            wq = split(wq_s)
            wkv = jnp.concatenate([split(wk_s), split(wv_s)], axis=1)

            def q_unit(r0):
                q = _dot(_bf(x_s[pl.ds(r0 // 2, rows // 2), :]), wq) * _QSCALE
                _st(dst.at[pl.ds(r0 // 2, rows // 2), pl.ds(0, 128)], q, 'a')

            def kv_unit(r0):
                kv = _dot(_bf(c_s[pl.ds(r0 // 2, rows // 2), :]), wkv)
                _st(dst.at[pl.ds(r0 // 2, rows // 2), pl.ds(128, 256)], kv, 'a')

            units = []
            for r0 in range(0, S, rows):
                units.append(functools.partial(kv_unit, r0))
                units.append(functools.partial(q_unit, r0))
            return units

        def attend(p, t, src, fillers, bq=bq, sorder=sorder, last_cfg=last_cfg):
            head = (_HeadWide if wide else _Head)(*[_bf(src[:, pl.ds(128 * i, 128)]) for i in range(3)], bq)
            ns = S // bq
            fillers = list(fillers)
            nslots = ns * fill_slots
            total = len(fillers)
            slot = [0]

            def fill():
                slot[0] += 1
                while fillers and (total - len(fillers)) * nslots < total * slot[0]:
                    fillers.pop(0)()

            order = list(range(ns))
            if sorder == 1:
                order = order[::-1]
            elif sorder == 2:
                order = [order[-1 - n // 2] if n % 2 == 0 else order[n // 2] for n in range(ns)]
            elif sorder == 3:
                order = [order[n // 2] if n % 2 == 0 else order[-1 - n // 2] for n in range(ns)]
            for n in range(min(lookahead, ns)):
                head.qk(order[n])
            for n in range(ns):
                if n + lookahead < ns:
                    head.qk(order[n + lookahead])
                if fill_slots == 2:
                    fill()
                i = order[n]
                _st(ctx_s.at[p, pl.ds(i * bq // 2, bq // 2), pl.ds(t * 128, 128)], head.pv(i), 'a')
                fill()
            while fillers:
                fillers.pop(0)()

        npair = H // 2
        for cp in pair_cps(0, 0):
            cp.wait()
        for u in project_units(0, 0, qkv0_s, 2048):
            u()

        def pair_step(p, last):
            s0 = p % 3
            attend(p, 0, qkv0_s, project_units(s0, 1, qkv1_s, frows))
            if last:
                attend(p, 1, qkv1_s, [], *last_cfg)
            else:
                attend(p, 1, qkv1_s, project_units((p + 1) % 3, 0, qkv0_s, frows))

        def a_body(p, carry):
            for cp in pair_cps(p + 1, (p + 1) % 3):
                cp.wait()

            @pl.when(p + 2 < npair)
            def _():
                for cp in pair_cps(p + 2, (p + 2) % 3):
                    cp.start()

            @pl.when(p == 2)
            def _():
                wo_cp.start()

            pl.when(fence)(lambda: pair_step(p, False))
            return carry

        jax.lax.fori_loop(0, npair - 1, a_body, 0)
        if b3_at == 1 and do_b:
            b3()
        pair_step(npair - 1, True)
        if b3_at == 2 and do_b:
            b3()

        wo_cp.wait()

        def oa_cp(i):
            return pltpu.make_async_copy(oa_s.at[i % 2], outh.at[pl.ds(16 * i, 16), :, pl.ds(0, 1024)],
                                         sem_oa.at[i % 2])

        def o_body(i, carry):
            r0 = pl.multiple_of(i * 128, 128)
            lhs = _bf(jnp.concatenate([ctx_s[p, pl.ds(r0, 128), :] for p in range(H // 2)], axis=1))
            res = _dot(lhs, _bf(wo_s[...]))

            @pl.when(i >= 2)
            def _():
                oa_cp(i - 2).wait()

            _st(oa_s.at[i % 2], res.reshape(16, 16, M))
            oa_cp(i).start()
            return carry

        jax.lax.fori_loop(0, 8, o_body, 0)
        oa_cp(6).wait()
        oa_cp(7).wait()

    if do_b:
        for p in range(8):
            ob_cp(p).wait()


def _run(A_x, A_c_kv, A_w_q, A_w_uk, A_w_uv, A_w_o, B_x, B_w_r, B_w_i, *, bq=256, do_a=True, do_b=True, rg_rows=16, n_pre=3, frows=128, fill_slots=2, lookahead=1, dbg=0, wide=True, bx_win=3, w_at=5, b3_at=0, b3_p=2, sorder=2, last_cfg=(128, 0), pad=8, sta=0, stb=0, flags=None):
    _STMODE['a'], _STMODE['b'] = sta, stb
    any_spec = pl.BlockSpec(memory_space=pltpu.HBM)
    vm = pltpu.VMEM
    dma = pltpu.SemaphoreType.DMA
    scratch = [
        vm((pad, 128), _U32),
        vm((1024, 1024), _U32),
        vm((1024, 512), _U32),
        vm((2048, 1024), _U32),
        vm((3, 2, 512, 128), _U32),
        vm((3, 2, 256, 128), _U32),
        vm((3, 2, 256, 128), _U32),
        vm((1024, 384), _U32), vm((1024, 384), _U32),
        vm((16, 1024, 256), _U32),
        vm((2, 16, 8, 1024), _U32),
        vm((8, 2, 64, 1024), _U32),
        vm((16, 256, 128), _U32),
        vm((16, 256, 128), _U32),
        vm((1, 2048), _BF16),
        vm((1, 2048), _BF16),
        vm((4, 128, 256), _U32),
        vm((4, 128, 256), _U32),
        vm((288, 128), _F32),
        vm((16, 128, 256), _U32),
        vm((16, 4, 64, 256), _U32),
        vm((8, 2048), _U32),
        vm((16, 4, 64, 256), _U32),
        vm((8, 128, 1024), _U32),
        vm((16, 128, 256), _F32), vm((16, 128, 256), _F32), vm((16, 128, 256), _F32), vm((16, 128, 256), _F32),
        *([vm((16, 128, 256), _F32)] * 2 if rg_rows == 8 else [vm((16, 64, 256), _U32)] * 2),
        vm((16, 128, 128), _F32),
        dma((16,)), dma((9,)), dma((32,)), dma((18,)), dma((8,)), dma((2,)),
    ]
    out = pl.pallas_call(
        functools.partial(_kernel, bq=bq, do_a=do_a, do_b=do_b, rg_rows=rg_rows, n_pre=n_pre, frows=frows, fill_slots=fill_slots, lookahead=lookahead, dbg=dbg, wide=wide, bx_win=bx_win, w_at=w_at, b3_at=b3_at, b3_p=b3_p, sorder=sorder, last_cfg=last_cfg),
        out_shape=jax.ShapeDtypeStruct((128, 16, 2048), _BF16),
        in_specs=[pl.BlockSpec(memory_space=pltpu.SMEM)] + [any_spec] * 12,
        out_specs=any_spec,
        scratch_shapes=scratch,
        compiler_params=pltpu.CompilerParams(vmem_limit_bytes=112 * 1024 * 1024, flags=flags),
    )(jnp.asarray(np.ones((1,), np.int32)), *[pltpu.with_memory_space_constraint(a, pltpu.HBM) for a in (
        A_x.reshape(S, M), A_c_kv.reshape(S, DC),
        A_w_q.reshape(512, 64, HD), A_w_uk.reshape(256, 64, HD), A_w_uv.reshape(256, 64, HD),
        A_w_o.reshape(H * HD, M),
        B_x.reshape(64, 32, BD), B_w_r.T, B_w_i.T,
        jnp.asarray(_FC), jnp.asarray(_IC), jnp.asarray(_GT),
    )])
    return out.reshape(1, S, 2048)


@jax.jit
def pallas_concat_heads__compressed_kv_cla__spectral_gfnet__prompt_kernel(
    A_x: jax.Array,
    A_c_kv: jax.Array,
    A_w_q: jax.Array,
    A_w_uk: jax.Array,
    A_w_uv: jax.Array,
    A_w_o: jax.Array,
    B_x: jax.Array,
    B_w_r: jax.Array,
    B_w_i: jax.Array,
):
    return _run(A_x, A_c_kv, A_w_q, A_w_uk, A_w_uv, A_w_o, B_x, B_w_r, B_w_i)
```

```python
import functools

import numpy as np
import jax
import jax.numpy as jnp
import jax.experimental.pallas as pl
import jax.experimental.pallas.tpu as pltpu

S = 2048
M = 1024
H = 32
HD = 128
DC = 512
BD = 1024
NG = 8

_U32 = jnp.uint32
_BF16 = jnp.bfloat16
_F32 = jnp.float32
_NT = (((1,), (1,)), ((), ()))
_QSCALE = float(HD ** -0.5 * np.log2(np.e))
_MASKED = -1e9


def _to_bf16_bits(a):
    u = np.ascontiguousarray(a, dtype=np.float32).view(np.uint32).astype(np.uint64)
    r = (u + 0x7FFF + ((u >> 16) & 1)) >> 16
    return r.astype(np.uint32) & 0xFFFF


def _pack_rows(a):
    b = _to_bf16_bits(a)
    return (b[0::2] | (b[1::2] << 16)).astype(np.uint32)


def _neg(p):
    return None if p is None else (-p[0], p[1])


def _add(p, q):
    if p is None:
        return q
    if q is None:
        return p
    if p[0] == q[0]:
        return (p[0], p[1] + q[1])
    if p[0] > 0:
        return (1, p[1] - q[1])
    return (1, q[1] - p[1])


def _sub(p, q):
    return _add(p, _neg(q))


def _scale(p, f):
    if p is None:
        return None
    return (p[0] * (1 if f > 0 else -1), p[1] * abs(f))


def _cadd(x, y):
    return (_add(x[0], y[0]), _add(x[1], y[1]))


def _csub(x, y):
    return (_sub(x[0], y[0]), _sub(x[1], y[1]))


def _cmul_i(x, s):
    return (_neg(x[1]), x[0]) if s > 0 else (x[1], _neg(x[0]))


def _cmul_w(x, n, sgn):
    n = n % 16
    if n == 0:
        return x
    if n == 4:
        return _cmul_i(x, sgn)
    if n == 8:
        return (_neg(x[0]), _neg(x[1]))
    if n == 12:
        return _cmul_i(x, -sgn)
    wr = float(np.cos(2 * np.pi * n / 16))
    wi = float(sgn * np.sin(2 * np.pi * n / 16))
    re, im = x
    if n % 2 == 0:
        r = abs(wr)
        sr = 1 if wr > 0 else -1
        si = 1 if wi > 0 else -1
        a = _sub(re if sr > 0 else _neg(re), im if si > 0 else _neg(im))
        b = _add(re if si > 0 else _neg(re), im if sr > 0 else _neg(im))
        return (_scale(a, r), _scale(b, r))
    return (_sub(_scale(re, wr), _scale(im, wi)), _add(_scale(re, wi), _scale(im, wr)))


def _dft4(x0, x1, x2, x3, sgn):
    s02, d02 = _cadd(x0, x2), _csub(x0, x2)
    s13, d13 = _cadd(x1, x3), _csub(x1, x3)
    r = _cmul_i(d13, sgn)
    return [_cadd(s02, s13), _cadd(d02, r), _csub(s02, s13), _csub(d02, r)]


def _fft16(xs, sgn):
    t = [_dft4(xs[a0], xs[4 + a0], xs[8 + a0], xs[12 + a0], sgn) for a0 in range(4)]
    t = [[_cmul_w(t[a0][j0], a0 * j0, sgn) for j0 in range(4)] for a0 in range(4)]
    out = [None] * 16
    for j0 in range(4):
        r = _dft4(t[0][j0], t[1][j0], t[2][j0], t[3][j0], sgn)
        for j1 in range(4):
            out[j0 + 4 * j1] = r[j1]
    return out


def _net_signs(sgn):
    out = _fft16([((1, 1.0), (1, 1.0)) for _ in range(16)], sgn)
    return [(o[0][0], o[1][0]) for o in out]


_INV_SIGNS = _net_signs(+1)
_CLS = ((0, 4), (1, 7), (2, 6), (3, 5))
_R2 = float(np.sqrt(0.5))


def _build_consts():
    n2 = np.arange(128)
    kap = np.arange(64)

    def wl(l):
        return np.exp(-2j * np.pi * np.outer(l, n2) / 1024)

    fc = np.zeros((4, 256, 256))
    w = wl(8 * kap)
    fc[0, 0:64, 0:128] = w.real
    fc[0, 64:128, 0:128] = w.imag
    fc[0, 64, 0:128] = (-1.0) ** n2
    w = wl(4 + 8 * kap)
    fc[0, 0:64, 128:256] = w.real
    fc[0, 64:128, 128:256] = w.imag
    for j in (1, 2, 3):
        si = 1.0 if j == 3 else -1.0
        w1, w2 = wl(j + 8 * kap), wl(8 - j + 8 * kap)
        fc[j, 0:64, 0:128], fc[j, 0:64, 128:] = w1.real, -w1.imag * si
        fc[j, 64:128, 0:128], fc[j, 64:128, 128:] = w2.real, w2.imag * si
        fc[j, 128:192, 0:128], fc[j, 128:192, 128:] = w1.imag, w1.real * si
        fc[j, 192:256, 0:128], fc[j, 192:256, 128:] = w2.imag, -w2.real * si

    def cs(l, c):
        ph = 2 * np.pi * np.outer(l, n2) / 1024
        return c[:, None] * np.cos(ph) / 1024, c[:, None] * np.sin(ph) / 1024

    ic = np.zeros((4, 256, 256))
    two = np.full(64, 2.0)
    co, si = cs(8 * kap, np.where(kap == 0, 1.0, 2.0))
    ic[0, 0:64, 0:128], ic[0, 128:192, 0:128] = co, -si
    ic[0, 128, 0:128] = (-1.0) ** n2 / 1024
    co, si = cs(4 + 8 * kap, two)
    ic[0, 64:128, 128:], ic[0, 192:256, 128:] = co, -si
    for j in (1, 2, 3):
        co, si = cs(j + 8 * kap, two)
        ic[j, 0:64, 0:128], ic[j, 128:192, 0:128] = co, -si
        ic[j, 0:64, 128:], ic[j, 128:192, 128:] = si, co
        co, si = cs(8 - j + 8 * kap, two)
        ic[j, 64:128, 0:128], ic[j, 192:256, 0:128] = co, -si
        ic[j, 64:128, 128:], ic[j, 192:256, 128:] = -si, -co

    f128 = np.exp(-2j * np.pi * np.outer(n2, n2) / 128)
    tw = np.exp(-2j * np.pi * np.outer(np.arange(16), n2) / 2048)

    def even_odd(m, blk):
        r = m.reshape(-1, blk // 2, 2, m.shape[-1])
        return np.concatenate([r[:, :, 0], r[:, :, 1]], axis=1).reshape(m.shape)

    fc[0] = even_odd(fc[0], 64)
    for j in (1, 2, 3):
        fc[j] = even_odd(fc[j], 128)
    il = np.arange(256).reshape(16, 2, 8).transpose(0, 2, 1).reshape(-1)
    ic_nat = ic
    ic = ic[:, il, :]
    sigma = np.concatenate([np.arange(0, 128, 2), np.arange(1, 128, 2)])
    fpos = f128[sigma]
    gt = np.concatenate([fpos[0::2].real, fpos[1::2].real, fpos[0::2].imag, fpos[1::2].imag,
                         tw.real, tw.imag], axis=0).astype(np.float32)

    def pk(m):
        return np.stack([_pack_rows(x) for x in m])

    return pk(fc), pk(ic / 2048), pk(ic_nat / 2048), gt


_FC, _IC, _IC_NAT, _GT = _build_consts()
assert all(sg == (1, 1) for sg in _INV_SIGNS)


def _bf(x_u32):
    return pltpu.bitcast(x_u32, _BF16)


def _pk(x_f32):
    return pltpu.bitcast(x_f32.astype(_BF16), _U32)


_STMODE = {"a": 1, "b": 1}


def _st(ref, x_f32, part="b"):
    if _STMODE[part]:
        ref.bitcast(_BF16)[...] = x_f32.astype(_BF16)
    else:
        ref[...] = _pk(x_f32)


def _pk2(x_f32):
    r = x_f32.shape[0] // 2
    return pltpu.pack_elementwise([x_f32[:r], x_f32[r:]], packed_dtype=_BF16)


def _dot(a, b):
    return jnp.dot(a, b, preferred_element_type=_F32)


def _val(p, like):
    if p is None:
        return jnp.zeros_like(like)
    return p[1] if p[0] > 0 else -p[1]


class _Head:
    def __init__(self, q, k, v, bq):
        self.q, self.k, self.v, self.bq = q, k, v, bq
        self.state = {}
        row = jax.lax.broadcasted_iota(jnp.int32, (128, 128), 0)
        col = jax.lax.broadcasted_iota(jnp.int32, (128, 128), 1)
        self.causal = col <= row

    def qk(self, i):
        bq = self.bq
        q0 = i * bq
        qq = self.q[q0:q0 + bq]
        nt = (q0 + bq) // 128
        mx = None
        ss = []
        for j in range(nt):
            r0 = max(0, j * 128 - q0)
            s = jax.lax.dot_general(qq[r0:], self.k[j * 128:(j + 1) * 128], _NT,
                                    preferred_element_type=_F32)
            if j * 128 >= q0:
                sd = jnp.where(self.causal, s[:128], _MASKED)
                s = jnp.concatenate([sd, s[128:]], axis=0) if s.shape[0] > 128 else sd
            ss.append(s)
            if mx is None:
                mx = s
            elif r0 == 0:
                mx = jnp.maximum(mx, s)
            else:
                mx = jnp.concatenate([mx[:r0], jnp.maximum(mx[r0:], s)], axis=0)
        self.state[i] = (ss, jnp.max(mx, axis=1, keepdims=True))

    def pv(self, i):
        bq = self.bq
        q0 = i * bq
        ss, m = self.state.pop(i)
        acc = None
        lsum = None
        for j, s in enumerate(ss):
            r0 = max(0, j * 128 - q0)
            p = jnp.exp2(s - m[r0:])
            pv = _dot(p.astype(_BF16), self.v[j * 128:(j + 1) * 128])
            if acc is None:
                acc, lsum = pv, p
            elif r0 == 0:
                acc, lsum = acc + pv, lsum + p
            else:
                acc = jnp.concatenate([acc[:r0], acc[r0:] + pv], axis=0)
                lsum = jnp.concatenate([lsum[:r0], lsum[r0:] + p], axis=0)
        l = jnp.sum(lsum, axis=1, keepdims=True)
        r = pl.reciprocal(l, approx=True)
        r = r * (2.0 - l * r)
        return acc * r


class _HeadWide(_Head):
    def qk(self, i):
        bq = self.bq
        q0 = i * bq
        parts = []
        for r in range(bq // 128):
            c0, c1 = (0, q0 + 128) if r == 0 else (q0 + 128 * r, q0 + 128 * (r + 1))
            s = jax.lax.dot_general(self.q[q0 + 128 * r:q0 + bq], self.k[c0:c1], _NT,
                                    preferred_element_type=_F32)
            w = c1 - c0
            top = jnp.where(self.causal, s[:128, w - 128:], _MASKED)
            if w > 128:
                top = jnp.concatenate([s[:128, :w - 128], top], axis=1)
            s = jnp.concatenate([top, s[128:]], axis=0) if s.shape[0] > 128 else top
            parts.append(s)
        mx = jnp.max(parts[0], axis=1, keepdims=True)
        for r in range(1, bq // 128):
            mr = jnp.max(parts[r], axis=1, keepdims=True)
            mx = jnp.concatenate([mx[:128 * r], jnp.maximum(mx[128 * r:], mr)], axis=0)
        self.state[i] = (parts, mx)

    def pv(self, i):
        bq = self.bq
        q0 = i * bq
        parts, m = self.state.pop(i)
        acc = l = None
        for r, s in enumerate(parts):
            c0, c1 = (0, q0 + 128) if r == 0 else (q0 + 128 * r, q0 + 128 * (r + 1))
            p = jnp.exp2(s - m[128 * r:])
            lr = jnp.sum(p, axis=1, keepdims=True)
            o = _dot(p.astype(_BF16), self.v[c0:c1])
            if r == 0:
                acc, l = o, lr
            else:
                acc = jnp.concatenate([acc[:128 * r], acc[128 * r:] + o], axis=0)
                l = jnp.concatenate([l[:128 * r], l[128 * r:] + lr], axis=0)
        rc = pl.reciprocal(l, approx=True)
        rc = rc * (2.0 - l * rc)
        return acc * rc


def _kernel(flag_ref, x_hbm, c_hbm, wq_hbm, wk_hbm, wv_hbm, wo_hbm, bx_hbm, wr_hbm, wi_hbm,
            fc_hbm, ic_hbm, gt_hbm,
            out_hbm,
            pad_s, x_s, c_s, wo_s, wq_s, wk_s, wv_s, qkv0_s, qkv1_s, ctx_s, oa_s,
            bx_s, wr_s, wi_s, wnr_s, wni_s, fc_s, ic_s, gt_s, gf_s, x1_s, nq_s, v_s, ob_s, u0_s, u1_s, u2_s, u3_s, q0_s, q1_s, vc_s,
            sem_bx, sem_misc, sem_w, sem_pair, sem_ob, sem_oa, *, bq, do_a, do_b, rg_rows, n_pre, frows, fill_slots, lookahead, dbg, wide, bx_win, w_at, b3_at, b3_p, sorder, last_cfg, afence, chain):
    xh = x_hbm.bitcast(_U32)
    ch = c_hbm.bitcast(_U32)
    wqh = wq_hbm.bitcast(_U32)
    wkh = wk_hbm.bitcast(_U32)
    wvh = wv_hbm.bitcast(_U32)
    woh = wo_hbm.bitcast(_U32)
    bxh = bx_hbm.bitcast(_U32)
    wrh = wr_hbm.at[pl.ds(0, 512)].bitcast(_U32)
    wih = wi_hbm.at[pl.ds(0, 512)].bitcast(_U32)
    outh = out_hbm.bitcast(_U32)

    def bx_cp(p, par):
        return pltpu.make_async_copy(bxh.at[:, par * 8 + p], bx_s.at[p, par], sem_bx.at[2 * p + par])

    def w_cp(j, which):
        src, dst = (wrh, wr_s) if which == 0 else (wih, wi_s)
        return pltpu.make_async_copy(src.at[:, pl.ds(128 * j, 128)], dst.at[j], sem_w.at[2 * j + which])

    fc_cp = pltpu.make_async_copy(fc_hbm, fc_s, sem_misc.at[0])
    ic_cp = pltpu.make_async_copy(ic_hbm, ic_s, sem_misc.at[1])
    wnr_cp = pltpu.make_async_copy(wr_hbm.at[pl.ds(512, 1)], wnr_s, sem_misc.at[2])
    x_cp = pltpu.make_async_copy(xh, x_s, sem_misc.at[5])
    c_cp = pltpu.make_async_copy(ch, c_s, sem_misc.at[6])
    wo_cp = pltpu.make_async_copy(woh, wo_s, sem_misc.at[7])
    wni_cp = pltpu.make_async_copy(wi_hbm.at[pl.ds(512, 1)], wni_s, sem_misc.at[8])

    def pair_cps(p, slot):
        cps = []
        for i, (src, dst) in enumerate(((wqh, wq_s), (wkh, wk_s), (wvh, wv_s))):
            for par in range(2):
                cps.append(pltpu.make_async_copy(
                    src.at[:, par * 16 + p], dst.at[slot, par], sem_pair.at[slot * 6 + 2 * i + par]))
        return cps

    gt_cp = pltpu.make_async_copy(gt_hbm, gt_s, sem_misc.at[3])

    def start_a_inputs():
        x_cp.start()
        c_cp.start()
        for cp in pair_cps(0, 0) + pair_cps(1, 1):
            cp.start()

    if do_b:
        gt_cp.start()
        fc_cp.start()
        bx_cp(0, 0).start()
        bx_cp(0, 1).start()
        for p in range(1, bx_win):
            bx_cp(p, 0).start()
            bx_cp(p, 1).start()
        wnr_cp.start()
        wni_cp.start()
    if do_a and not do_b:
        start_a_inputs()

    zero = flag_ref[0] - 1
    fence = flag_ref[0] > 0

    if do_b:
        lane0 = jax.lax.broadcasted_iota(jnp.int32, (1, 128), 1) == 0
        row0 = jax.lax.broadcasted_iota(jnp.int32, (8, 128), 0) == 0

        gt_cp.wait()
        f_r, f_i = gt_s[pl.ds(0, 128), :], gt_s[pl.ds(128, 128), :]
        for ap in range(16):
            t_r, t_i = gt_s[pl.ds(256 + ap, 1), :], gt_s[pl.ds(272 + ap, 1), :]
            g_r = _pk2(f_r * t_r - f_i * t_i)
            g_i = _pk2(f_r * t_i + f_i * t_r)
            gf_s[ap] = jnp.concatenate([jnp.concatenate([g_r, g_i], axis=1),
                                        jnp.concatenate([g_i ^ jnp.uint32(0x80008000), g_r], axis=1)], axis=0)
        fc_cp.wait()

        def b1_step(p):
            bx_cp(p, 0).wait()
            bx_cp(p, 1).wait()
            if p + bx_win < 8:
                bx_cp(p + bx_win, 0).start()
                bx_cp(p + bx_win, 1).start()
            if p == w_at:
                for j in range(16):
                    w_cp(j, 0).start()
                    w_cp(j, 1).start()
            for h in range(2):
                halves = []
                for par in range(2):
                    xf = pltpu.unpack_elementwise(bx_s[p, par], index=h, packed_dtype=_BF16,
                                                  unpacked_dtype=_F32)
                    xs = [xf[:, 128 * n:128 * (n + 1)] for n in range(8)]
                    a_, b_ = xs[0] + xs[4], xs[0] - xs[4]
                    c_, d_ = xs[2] + xs[6], xs[2] - xs[6]
                    e_, f_ = xs[1] + xs[5], xs[1] - xs[5]
                    g_, h_ = xs[3] + xs[7], xs[3] - xs[7]
                    u_ = (f_ - h_) * _R2
                    v_ = (f_ + h_) * _R2
                    ac, eg = a_ + c_, e_ + g_
                    halves.append([ac + eg, ac - eg, b_ + u_, d_ + v_, a_ - c_, e_ - g_, b_ - u_, d_ - v_])
                pln = [jnp.concatenate([halves[0][i], halves[1][i]], axis=0).astype(_BF16)
                       for i in range(8)]
                ap = 2 * p + h
                f0 = _bf(fc_s[0, pl.ds(0, 64), :])
                o0 = jax.lax.dot_general(f0[:, 0:128], pln[0], _NT, preferred_element_type=_F32)
                o4 = jax.lax.dot_general(f0[:, 128:256], pln[1], _NT, preferred_element_type=_F32)
                nq = jnp.where(row0, o0[64:72], 0.0)
                im0 = jnp.concatenate([jnp.where(row0, 0.0, o0[64:72]), o0[72:128]], axis=0)
                nq_s[:, pl.ds(128 * ap, 128)] = _pk2(jnp.concatenate([nq, jnp.zeros_like(nq)], axis=0))
                x1_s[ap, 0] = jnp.concatenate(
                    [jnp.concatenate([_pk2(o0[0:64]), _pk2(o4[0:64])], axis=0),
                     jnp.concatenate([_pk2(im0), _pk2(o4[64:128])], axis=0)], axis=1)
                for j in (1, 2, 3):
                    rhs = jnp.concatenate([pln[2 * j], pln[2 * j + 1]], axis=1)
                    o = jax.lax.dot_general(_bf(fc_s[j]), rhs, _NT, preferred_element_type=_F32)
                    x1_s[ap, j] = jnp.concatenate([_pk2(o[0:128]), _pk2(o[128:256])], axis=1)

        for p in range(8):
            b1_step(p)

        def spectral(us, w_of):
            xs = _fft16(us, -1)
            qs = []
            for j in range(16):
                (sr, xr), (si, xi) = xs[j]
                wr, wi = w_of(j)
                qs.append((_sub((sr, xr * wr), (si, xi * wi)), _add((sr, xr * wi), (si, xi * wr))))
            res = _fft16(qs, +1)
            assert all(r[0][0] == 1 and r[1][0] == 1 for r in res)
            return [(r[0][1], r[1][1]) for r in res]

        u_s, q_s = (u0_s, u1_s, u2_s, u3_s), (q0_s, q1_s)

        def s_fwd(t, ap):
            u_s[t][ap] = _dot(_bf(x1_s[ap, t]), _bf(gf_s[ap]))

        def filt(t, g):
            R = rg_rows
            r0 = R * g
            cls = _CLS[t][r0 // 64]
            k0 = r0 % 64
            rows = pl.ds(pl.multiple_of(r0 + zero, R), R)

            def w_of(j):
                return tuple(pltpu.unpack_elementwise(
                    ws.at[j, pl.ds(pl.multiple_of(zero, 64), 256)][pl.ds(cls // 2 + 4 * k0, R, stride=4), :],
                    index=cls % 2, packed_dtype=_BF16, unpacked_dtype=_F32) for ws in (wr_s, wi_s))

            res = spectral([((1, u_s[t][ap, rows, pl.ds(0, 128)]), (1, u_s[t][ap, rows, pl.ds(128, 128)]))
                            for ap in range(16)], w_of)
            for ap in range(16):
                if R == 8:
                    q_s[t % 2][ap, pl.ds(r0, 8), :] = jnp.concatenate([res[ap][0], res[ap][1]], axis=1)
                else:
                    q_s[t % 2][ap, pl.ds(r0 // 2, 8), :] = jnp.concatenate([_pk2(res[ap][0]), _pk2(res[ap][1])], axis=1)
            if chain:
                tail = res[15][1][0:8]
                u_s[t][16, pl.ds(pl.multiple_of(zero, 8), 8), pl.ds(0, 128)] = tail
                for ws in (wr_s, wi_s):
                    ws[16, pl.ds(pl.multiple_of(zero, 8), 8), :] = pltpu.bitcast(tail, _U32)

        def s_inv(t, ap):
            q = q_s[t % 2][ap].astype(_BF16) if rg_rows == 8 else _bf(q_s[t % 2][ap])
            o = jax.lax.dot_general(_bf(gf_s[ap]), q, _NT, preferred_element_type=_F32)
            vi = o[128:256]
            if t == 0:
                vi = jnp.where(lane0, vc_s[ap], vi)
            v_s[ap, t] = jnp.concatenate([_pk2(o[0:128]), _pk2(vi)], axis=1)

        def nyquist(un):
            wnr = wnr_s[...].astype(_F32)
            wni = wni_s[...].astype(_F32)
            qn = spectral([((1, u[:, 0:128]), (1, u[:, 128:256])) for u in un],
                          lambda j: (wnr[:, 128 * j:128 * (j + 1)], wni[:, 128 * j:128 * (j + 1)]))
            for ap in range(16):
                lhs = jnp.concatenate([qn[ap][0], qn[ap][1]], axis=1).astype(_BF16)
                vn = jax.lax.dot_general(lhs, _bf(gf_s[ap, pl.ds(0, 64), :]), _NT,
                                         preferred_element_type=_F32)
                vn = jnp.concatenate([vn, jnp.zeros((112, 128), _F32)], axis=0)
                vc_s[ap] = vn.T

        def b2_head():
            un = [_dot(_bf(nq_s[:, pl.ds(128 * ap, 128)]), _bf(gf_s[ap, pl.ds(0, 64), :])) for ap in range(16)]
            for ap in range(16):
                u = _dot(_bf(x1_s[ap, 0:n_pre].reshape(64 * n_pre, 256)), _bf(gf_s[ap]))
                for t in range(n_pre):
                    u_s[t][ap] = u[128 * t:128 * (t + 1)]
                if ap == 7:
                    nyquist(un)

        wnr_cp.wait()
        wni_cp.wait()
        pl.when(fence)(b2_head)
        for j in range(16):
            w_cp(j, 0).wait()
            w_cp(j, 1).wait()
        ic_cp.start()
        if do_a:
            start_a_inputs()
        def b2_slot(t):
            ng = 128 // rg_rows
            for g in range(ng):
                filt(t, g)
                for k in range(16 // ng):
                    if t + n_pre < 4:
                        s_fwd(t + n_pre, (16 // ng) * g + k)
                    if t > 0:
                        s_inv(t - 1, (16 // ng) * g + k)

        for t in range(4):
            pl.when(flag_ref[t + 1] > 0)(functools.partial(b2_slot, t))

        def b2_tail():
            for ap in range(16):
                s_inv(3, ap)

        pl.when(fence)(b2_tail)

        def ob_cp(p):
            return pltpu.make_async_copy(ob_s.at[p], outh.at[:, p, pl.ds(1024, 1024)], sem_ob.at[p])

        def b3():
            ic_cp.wait()

            for pq in range(8 // b3_p):
                aps = range(2 * b3_p * pq, 2 * b3_p * (pq + 1))
                cc = [_dot(_bf(jnp.concatenate([v_s[ap, t] for ap in aps], axis=0)), _bf(ic_s[t]))
                      for t in range(4)]
                c0, c4 = cc[0][:, 0:128], cc[0][:, 128:256]
                c1r, c1i = cc[1][:, 0:128], cc[1][:, 128:256]
                c2r, c2i = cc[2][:, 0:128], cc[2][:, 128:256]
                c3r, c3i = cc[3][:, 0:128], cc[3][:, 128:256]
                pp, mm = c0 + c4, c0 - c4
                u1, u2, u3, u4 = c1r + c3r, c1i - c3i, c1r - c3r, c1i + c3i
                t1, t2 = (u3 - u4) * _R2, (u3 + u4) * _R2
                e0, e1, e2, e3 = pp + c2r, pp - c2r, mm - c2i, mm + c2i
                ys = [e0 + u1, e2 + t1, e1 - u2, e3 - t2, e0 - u1, e2 - t1, e1 + u2, e3 + t2]
                for k in range(b3_p):
                    p = b3_p * pq + k
                    ob_s[p] = jnp.concatenate(
                        [pltpu.pack_elementwise([y[256 * k:256 * k + 128], y[256 * k + 128:256 * k + 256]],
                                                packed_dtype=_BF16) for y in ys], axis=1)
                    ob_cp(p).start()

        if b3_at == 0 or not do_a:
            b3()

    if do_a:
        x_cp.wait()
        c_cp.wait()

        def project_units(slot, half, dst, rows):
            def split(ref):
                a = ref[slot, 0]
                b = ref[slot, 1]
                if half == 1:
                    a, b = a >> 16, b >> 16
                return _bf(pltpu.pack_elementwise([a, b], packed_dtype=jnp.uint16))

            wq = split(wq_s)
            wkv = jnp.concatenate([split(wk_s), split(wv_s)], axis=1)

            def q_unit(r0):
                q = _dot(_bf(x_s[pl.ds(r0 // 2, rows // 2), :]), wq) * _QSCALE
                _st(dst.at[pl.ds(r0 // 2, rows // 2), pl.ds(0, 128)], q, 'a')

            def kv_unit(r0):
                kv = _dot(_bf(c_s[pl.ds(r0 // 2, rows // 2), :]), wkv)
                _st(dst.at[pl.ds(r0 // 2, rows // 2), pl.ds(128, 256)], kv, 'a')

            units = []
            for r0 in range(0, S, rows):
                units.append(functools.partial(kv_unit, r0))
                units.append(functools.partial(q_unit, r0))
            return units

        def attend(p, t, src, fillers, bq=bq, sorder=sorder, last_cfg=last_cfg, afence=afence, chain=chain):
            head = (_HeadWide if wide else _Head)(*[_bf(src[:, pl.ds(128 * i, 128)]) for i in range(3)], bq)
            ns = S // bq
            fillers = list(fillers)
            nslots = ns * fill_slots
            total = len(fillers)
            slot = [0]

            def fill():
                slot[0] += 1
                while fillers and (total - len(fillers)) * nslots < total * slot[0]:
                    fillers.pop(0)()

            order = list(range(ns))
            if sorder == 1:
                order = order[::-1]
            elif sorder == 2:
                order = [order[-1 - n // 2] if n % 2 == 0 else order[n // 2] for n in range(ns)]
            elif sorder == 3:
                order = [order[n // 2] if n % 2 == 0 else order[-1 - n // 2] for n in range(ns)]
            for n in range(min(lookahead, ns)):
                head.qk(order[n])
            for n in range(ns):
                if n + lookahead < ns:
                    head.qk(order[n + lookahead])
                if fill_slots == 2:
                    fill()
                i = order[n]
                _st(ctx_s.at[p, pl.ds(i * bq // 2, bq // 2), pl.ds(t * 128, 128)], head.pv(i), 'a')
                fill()
            while fillers:
                fillers.pop(0)()

        npair = H // 2
        for cp in pair_cps(0, 0):
            cp.wait()
        for u in project_units(0, 0, qkv0_s, 2048):
            u()

        def pair_step(p, last):
            s0 = p % 3
            attend(p, 0, qkv0_s, project_units(s0, 1, qkv1_s, frows))
            if last:
                attend(p, 1, qkv1_s, [], *last_cfg)
            else:
                attend(p, 1, qkv1_s, project_units((p + 1) % 3, 0, qkv0_s, frows))

        def a_body(p, carry):
            for cp in pair_cps(p + 1, (p + 1) % 3):
                cp.wait()

            @pl.when(p + 2 < npair)
            def _():
                for cp in pair_cps(p + 2, (p + 2) % 3):
                    cp.start()

            @pl.when(p == 2)
            def _():
                wo_cp.start()

            if afence:
                pl.when(fence)(lambda: pair_step(p, False))
            else:
                pair_step(p, False)
            return carry

        jax.lax.fori_loop(0, npair - 1, a_body, 0)
        if b3_at == 1 and do_b:
            b3()
        pair_step(npair - 1, True)
        if b3_at == 2 and do_b:
            b3()

        wo_cp.wait()

        def oa_cp(i):
            return pltpu.make_async_copy(oa_s.at[i % 2], outh.at[pl.ds(16 * i, 16), :, pl.ds(0, 1024)],
                                         sem_oa.at[i % 2])

        def o_body(i, carry):
            r0 = pl.multiple_of(i * 128, 128)
            lhs = _bf(jnp.concatenate([ctx_s[p, pl.ds(r0, 128), :] for p in range(H // 2)], axis=1))
            res = _dot(lhs, _bf(wo_s[...]))

            @pl.when(i >= 2)
            def _():
                oa_cp(i - 2).wait()

            _st(oa_s.at[i % 2], res.reshape(16, 16, M))
            oa_cp(i).start()
            return carry

        jax.lax.fori_loop(0, 8, o_body, 0)
        oa_cp(6).wait()
        oa_cp(7).wait()

    if do_b:
        for p in range(8):
            ob_cp(p).wait()


def _run(A_x, A_c_kv, A_w_q, A_w_uk, A_w_uv, A_w_o, B_x, B_w_r, B_w_i, *, bq=256, do_a=True, do_b=True, rg_rows=8, n_pre=3, frows=128, fill_slots=2, lookahead=1, dbg=0, wide=True, bx_win=3, w_at=5, b3_at=0, b3_p=2, sorder=2, last_cfg=(128, 0), pad=8, cp=dict(disable_bounds_checks=True, disable_semaphore_checks=True), afence=0, chain=0, sta=0, stb=0, flags=None):
    _STMODE['a'], _STMODE['b'] = sta, stb
    any_spec = pl.BlockSpec(memory_space=pltpu.HBM)
    vm = pltpu.VMEM
    dma = pltpu.SemaphoreType.DMA
    scratch = [
        vm((pad, 128), _U32),
        vm((1024, 1024), _U32),
        vm((1024, 512), _U32),
        vm((2048, 1024), _U32),
        vm((3, 2, 512, 128), _U32),
        vm((3, 2, 256, 128), _U32),
        vm((3, 2, 256, 128), _U32),
        vm((1024, 384), _U32), vm((1024, 384), _U32),
        vm((16, 1024, 256), _U32),
        vm((2, 16, 8, 1024), _U32),
        vm((8, 2, 64, 1024), _U32),
        vm((17, 256, 128), _U32),
        vm((17, 256, 128), _U32),
        vm((1, 2048), _BF16),
        vm((1, 2048), _BF16),
        vm((4, 128, 256), _U32),
        vm((4, 128, 256), _U32),
        vm((288, 128), _F32),
        vm((16, 128, 256), _U32),
        vm((16, 4, 64, 256), _U32),
        vm((8, 2048), _U32),
        vm((16, 4, 64, 256), _U32),
        vm((8, 128, 1024), _U32),
        vm((17, 128, 256), _F32), vm((17, 128, 256), _F32), vm((17, 128, 256), _F32), vm((17, 128, 256), _F32),
        *([vm((16, 128, 256), _F32)] * 2 if rg_rows == 8 else [vm((16, 64, 256), _U32)] * 2),
        vm((16, 128, 128), _F32),
        dma((16,)), dma((9,)), dma((32,)), dma((18,)), dma((8,)), dma((2,)),
    ]
    out = pl.pallas_call(
        functools.partial(_kernel, bq=bq, do_a=do_a, do_b=do_b, rg_rows=rg_rows, n_pre=n_pre, frows=frows, fill_slots=fill_slots, lookahead=lookahead, dbg=dbg, wide=wide, bx_win=bx_win, w_at=w_at, b3_at=b3_at, b3_p=b3_p, sorder=sorder, last_cfg=last_cfg, afence=afence, chain=chain),
        out_shape=jax.ShapeDtypeStruct((128, 16, 2048), _BF16),
        in_specs=[pl.BlockSpec(memory_space=pltpu.SMEM)] + [any_spec] * 12,
        out_specs=any_spec,
        scratch_shapes=scratch,
        compiler_params=pltpu.CompilerParams(vmem_limit_bytes=112 * 1024 * 1024, flags=flags, **(cp or {})),
    )(jnp.asarray(np.arange(1, 9, dtype=np.int32)), *[pltpu.with_memory_space_constraint(a, pltpu.HBM) for a in (
        A_x.reshape(S, M), A_c_kv.reshape(S, DC),
        A_w_q.reshape(512, 64, HD), A_w_uk.reshape(256, 64, HD), A_w_uv.reshape(256, 64, HD),
        A_w_o.reshape(H * HD, M),
        B_x.reshape(64, 32, BD), B_w_r.T, B_w_i.T,
        jnp.asarray(_FC), jnp.asarray(_IC_NAT if rg_rows == 8 else _IC), jnp.asarray(_GT),
    )])
    return out.reshape(1, S, 2048)


@jax.jit
def pallas_concat_heads__compressed_kv_cla__spectral_gfnet__prompt_kernel(
    A_x: jax.Array,
    A_c_kv: jax.Array,
    A_w_q: jax.Array,
    A_w_uk: jax.Array,
    A_w_uv: jax.Array,
    A_w_o: jax.Array,
    B_x: jax.Array,
    B_w_r: jax.Array,
    B_w_i: jax.Array,
):
    return _run(A_x, A_c_kv, A_w_q, A_w_uk, A_w_uv, A_w_o, B_x, B_w_r, B_w_i)
```

```python
import functools

import numpy as np
import jax
import jax.numpy as jnp
import jax.experimental.pallas as pl
import jax.experimental.pallas.tpu as pltpu

S = 2048
M = 1024
H = 32
HD = 128
DC = 512
BD = 1024
NG = 8

_U32 = jnp.uint32
_BF16 = jnp.bfloat16
_F32 = jnp.float32
_NT = (((1,), (1,)), ((), ()))
_QSCALE = float(HD ** -0.5 * np.log2(np.e))
_MASKED = -1e9


def _to_bf16_bits(a):
    u = np.ascontiguousarray(a, dtype=np.float32).view(np.uint32).astype(np.uint64)
    r = (u + 0x7FFF + ((u >> 16) & 1)) >> 16
    return r.astype(np.uint32) & 0xFFFF


def _pack_rows(a):
    b = _to_bf16_bits(a)
    return (b[0::2] | (b[1::2] << 16)).astype(np.uint32)


def _neg(p):
    return None if p is None else (-p[0], p[1])


def _add(p, q):
    if p is None:
        return q
    if q is None:
        return p
    if p[0] == q[0]:
        return (p[0], p[1] + q[1])
    if p[0] > 0:
        return (1, p[1] - q[1])
    return (1, q[1] - p[1])


def _sub(p, q):
    return _add(p, _neg(q))


def _scale(p, f):
    if p is None:
        return None
    return (p[0] * (1 if f > 0 else -1), p[1] * abs(f))


def _cadd(x, y):
    return (_add(x[0], y[0]), _add(x[1], y[1]))


def _csub(x, y):
    return (_sub(x[0], y[0]), _sub(x[1], y[1]))


def _cmul_i(x, s):
    return (_neg(x[1]), x[0]) if s > 0 else (x[1], _neg(x[0]))


def _cmul_w(x, n, sgn):
    n = n % 16
    if n == 0:
        return x
    if n == 4:
        return _cmul_i(x, sgn)
    if n == 8:
        return (_neg(x[0]), _neg(x[1]))
    if n == 12:
        return _cmul_i(x, -sgn)
    wr = float(np.cos(2 * np.pi * n / 16))
    wi = float(sgn * np.sin(2 * np.pi * n / 16))
    re, im = x
    if n % 2 == 0:
        r = abs(wr)
        sr = 1 if wr > 0 else -1
        si = 1 if wi > 0 else -1
        a = _sub(re if sr > 0 else _neg(re), im if si > 0 else _neg(im))
        b = _add(re if si > 0 else _neg(re), im if sr > 0 else _neg(im))
        return (_scale(a, r), _scale(b, r))
    return (_sub(_scale(re, wr), _scale(im, wi)), _add(_scale(re, wi), _scale(im, wr)))


def _dft4(x0, x1, x2, x3, sgn):
    s02, d02 = _cadd(x0, x2), _csub(x0, x2)
    s13, d13 = _cadd(x1, x3), _csub(x1, x3)
    r = _cmul_i(d13, sgn)
    return [_cadd(s02, s13), _cadd(d02, r), _csub(s02, s13), _csub(d02, r)]


def _fft16(xs, sgn):
    t = [_dft4(xs[a0], xs[4 + a0], xs[8 + a0], xs[12 + a0], sgn) for a0 in range(4)]
    t = [[_cmul_w(t[a0][j0], a0 * j0, sgn) for j0 in range(4)] for a0 in range(4)]
    out = [None] * 16
    for j0 in range(4):
        r = _dft4(t[0][j0], t[1][j0], t[2][j0], t[3][j0], sgn)
        for j1 in range(4):
            out[j0 + 4 * j1] = r[j1]
    return out


def _net_signs(sgn):
    out = _fft16([((1, 1.0), (1, 1.0)) for _ in range(16)], sgn)
    return [(o[0][0], o[1][0]) for o in out]


_INV_SIGNS = _net_signs(+1)
_CLS = ((0, 4), (1, 7), (2, 6), (3, 5))
_R2 = float(np.sqrt(0.5))


def _build_consts():
    n2 = np.arange(128)
    kap = np.arange(64)

    def wl(l):
        return np.exp(-2j * np.pi * np.outer(l, n2) / 1024)

    fc = np.zeros((4, 256, 256))
    w = wl(8 * kap)
    fc[0, 0:64, 0:128] = w.real
    fc[0, 64:128, 0:128] = w.imag
    fc[0, 64, 0:128] = (-1.0) ** n2
    w = wl(4 + 8 * kap)
    fc[0, 0:64, 128:256] = w.real
    fc[0, 64:128, 128:256] = w.imag
    for j in (1, 2, 3):
        si = 1.0 if j == 3 else -1.0
        w1, w2 = wl(j + 8 * kap), wl(8 - j + 8 * kap)
        fc[j, 0:64, 0:128], fc[j, 0:64, 128:] = w1.real, -w1.imag * si
        fc[j, 64:128, 0:128], fc[j, 64:128, 128:] = w2.real, w2.imag * si
        fc[j, 128:192, 0:128], fc[j, 128:192, 128:] = w1.imag, w1.real * si
        fc[j, 192:256, 0:128], fc[j, 192:256, 128:] = w2.imag, -w2.real * si

    def cs(l, c):
        ph = 2 * np.pi * np.outer(l, n2) / 1024
        return c[:, None] * np.cos(ph) / 1024, c[:, None] * np.sin(ph) / 1024

    ic = np.zeros((4, 256, 256))
    two = np.full(64, 2.0)
    co, si = cs(8 * kap, np.where(kap == 0, 1.0, 2.0))
    ic[0, 0:64, 0:128], ic[0, 128:192, 0:128] = co, -si
    ic[0, 128, 0:128] = (-1.0) ** n2 / 1024
    co, si = cs(4 + 8 * kap, two)
    ic[0, 64:128, 128:], ic[0, 192:256, 128:] = co, -si
    for j in (1, 2, 3):
        co, si = cs(j + 8 * kap, two)
        ic[j, 0:64, 0:128], ic[j, 128:192, 0:128] = co, -si
        ic[j, 0:64, 128:], ic[j, 128:192, 128:] = si, co
        co, si = cs(8 - j + 8 * kap, two)
        ic[j, 64:128, 0:128], ic[j, 192:256, 0:128] = co, -si
        ic[j, 64:128, 128:], ic[j, 192:256, 128:] = -si, -co

    f128 = np.exp(-2j * np.pi * np.outer(n2, n2) / 128)
    tw = np.exp(-2j * np.pi * np.outer(np.arange(16), n2) / 2048)

    def even_odd(m, blk):
        r = m.reshape(-1, blk // 2, 2, m.shape[-1])
        return np.concatenate([r[:, :, 0], r[:, :, 1]], axis=1).reshape(m.shape)

    fc[0] = even_odd(fc[0], 64)
    for j in (1, 2, 3):
        fc[j] = even_odd(fc[j], 128)
    il = np.arange(256).reshape(16, 2, 8).transpose(0, 2, 1).reshape(-1)
    ic_nat = ic
    ic = ic[:, il, :]
    sigma = np.concatenate([np.arange(0, 128, 2), np.arange(1, 128, 2)])
    fpos = f128[sigma]
    gt = np.concatenate([fpos[0::2].real, fpos[1::2].real, fpos[0::2].imag, fpos[1::2].imag,
                         tw.real, tw.imag], axis=0).astype(np.float32)

    def pk(m):
        return np.stack([_pack_rows(x) for x in m])

    return pk(fc), pk(ic / 2048), pk(ic_nat / 2048), gt


_FC, _IC, _IC_NAT, _GT = _build_consts()
assert all(sg == (1, 1) for sg in _INV_SIGNS)


def _bf(x_u32):
    return pltpu.bitcast(x_u32, _BF16)


def _pk(x_f32):
    return pltpu.bitcast(x_f32.astype(_BF16), _U32)


_STMODE = {"a": 1, "b": 1}


def _st(ref, x_f32, part="b"):
    if _STMODE[part]:
        ref.bitcast(_BF16)[...] = x_f32.astype(_BF16)
    else:
        ref[...] = _pk(x_f32)


def _pk2(x_f32):
    r = x_f32.shape[0] // 2
    return pltpu.pack_elementwise([x_f32[:r], x_f32[r:]], packed_dtype=_BF16)


def _dot(a, b):
    return jnp.dot(a, b, preferred_element_type=_F32)


def _val(p, like):
    if p is None:
        return jnp.zeros_like(like)
    return p[1] if p[0] > 0 else -p[1]


class _Head:
    def __init__(self, q, k, v, bq):
        self.q, self.k, self.v, self.bq = q, k, v, bq
        self.state = {}
        row = jax.lax.broadcasted_iota(jnp.int32, (128, 128), 0)
        col = jax.lax.broadcasted_iota(jnp.int32, (128, 128), 1)
        self.causal = col <= row

    def qk(self, i):
        bq = self.bq
        q0 = i * bq
        qq = self.q[q0:q0 + bq]
        nt = (q0 + bq) // 128
        mx = None
        ss = []
        for j in range(nt):
            r0 = max(0, j * 128 - q0)
            s = jax.lax.dot_general(qq[r0:], self.k[j * 128:(j + 1) * 128], _NT,
                                    preferred_element_type=_F32)
            if j * 128 >= q0:
                sd = jnp.where(self.causal, s[:128], _MASKED)
                s = jnp.concatenate([sd, s[128:]], axis=0) if s.shape[0] > 128 else sd
            ss.append(s)
            if mx is None:
                mx = s
            elif r0 == 0:
                mx = jnp.maximum(mx, s)
            else:
                mx = jnp.concatenate([mx[:r0], jnp.maximum(mx[r0:], s)], axis=0)
        self.state[i] = (ss, jnp.max(mx, axis=1, keepdims=True))

    def pv(self, i):
        bq = self.bq
        q0 = i * bq
        ss, m = self.state.pop(i)
        acc = None
        lsum = None
        for j, s in enumerate(ss):
            r0 = max(0, j * 128 - q0)
            p = jnp.exp2(s - m[r0:])
            pv = _dot(p.astype(_BF16), self.v[j * 128:(j + 1) * 128])
            if acc is None:
                acc, lsum = pv, p
            elif r0 == 0:
                acc, lsum = acc + pv, lsum + p
            else:
                acc = jnp.concatenate([acc[:r0], acc[r0:] + pv], axis=0)
                lsum = jnp.concatenate([lsum[:r0], lsum[r0:] + p], axis=0)
        l = jnp.sum(lsum, axis=1, keepdims=True)
        r = pl.reciprocal(l, approx=True)
        r = r * (2.0 - l * r)
        return acc * r


class _HeadWide(_Head):
    def qk(self, i):
        bq = self.bq
        q0 = i * bq
        parts = []
        for r in range(bq // 128):
            c0, c1 = (0, q0 + 128) if r == 0 else (q0 + 128 * r, q0 + 128 * (r + 1))
            s = jax.lax.dot_general(self.q[q0 + 128 * r:q0 + bq], self.k[c0:c1], _NT,
                                    preferred_element_type=_F32)
            w = c1 - c0
            top = jnp.where(self.causal, s[:128, w - 128:], _MASKED)
            if w > 128:
                top = jnp.concatenate([s[:128, :w - 128], top], axis=1)
            s = jnp.concatenate([top, s[128:]], axis=0) if s.shape[0] > 128 else top
            parts.append(s)
        mx = jnp.max(parts[0], axis=1, keepdims=True)
        for r in range(1, bq // 128):
            mr = jnp.max(parts[r], axis=1, keepdims=True)
            mx = jnp.concatenate([mx[:128 * r], jnp.maximum(mx[128 * r:], mr)], axis=0)
        self.state[i] = (parts, mx)

    def pv(self, i):
        bq = self.bq
        q0 = i * bq
        parts, m = self.state.pop(i)
        acc = l = None
        for r, s in enumerate(parts):
            c0, c1 = (0, q0 + 128) if r == 0 else (q0 + 128 * r, q0 + 128 * (r + 1))
            p = jnp.exp2(s - m[128 * r:])
            lr = jnp.sum(p, axis=1, keepdims=True)
            o = _dot(p.astype(_BF16), self.v[c0:c1])
            if r == 0:
                acc, l = o, lr
            else:
                acc = jnp.concatenate([acc[:128 * r], acc[128 * r:] + o], axis=0)
                l = jnp.concatenate([l[:128 * r], l[128 * r:] + lr], axis=0)
        rc = pl.reciprocal(l, approx=True)
        rc = rc * (2.0 - l * rc)
        return acc * rc


def _kernel(flag_ref, x_hbm, c_hbm, wq_hbm, wk_hbm, wv_hbm, wo_hbm, bx_hbm, wr_hbm, wi_hbm,
            fc_hbm, ic_hbm, gt_hbm,
            out_hbm,
            pad_s, x_s, c_s, wo_s, wq_s, wk_s, wv_s, qkv0_s, qkv1_s, ctx_s, oa_s,
            bx_s, wr_s, wi_s, wnr_s, wni_s, fc_s, ic_s, gt_s, gf_s, x1_s, nq_s, v_s, ob_s, u0_s, u1_s, u2_s, u3_s, q0_s, q1_s, vc_s,
            sem_bx, sem_misc, sem_w, sem_pair, sem_ob, sem_oa, *, bq, do_a, do_b, rg_rows, n_pre, frows, fill_slots, lookahead, dbg, wide, bx_win, w_at, b3_at, b3_p, sorder, last_cfg, afence, chain, b1_pipe, b1_grp):
    xh = x_hbm.bitcast(_U32)
    ch = c_hbm.bitcast(_U32)
    wqh = wq_hbm.bitcast(_U32)
    wkh = wk_hbm.bitcast(_U32)
    wvh = wv_hbm.bitcast(_U32)
    woh = wo_hbm.bitcast(_U32)
    bxh = bx_hbm.bitcast(_U32)
    wrh = wr_hbm.at[pl.ds(0, 512)].bitcast(_U32)
    wih = wi_hbm.at[pl.ds(0, 512)].bitcast(_U32)
    outh = out_hbm.bitcast(_U32)

    def bx_cp(p, par):
        return pltpu.make_async_copy(bxh.at[:, par * 8 + p], bx_s.at[p, par], sem_bx.at[2 * p + par])

    def w_cp(j, which):
        src, dst = (wrh, wr_s) if which == 0 else (wih, wi_s)
        return pltpu.make_async_copy(src.at[:, pl.ds(128 * j, 128)], dst.at[j], sem_w.at[2 * j + which])

    fc_cp = pltpu.make_async_copy(fc_hbm, fc_s, sem_misc.at[0])
    ic_cp = pltpu.make_async_copy(ic_hbm, ic_s, sem_misc.at[1])
    wnr_cp = pltpu.make_async_copy(wr_hbm.at[pl.ds(512, 1)], wnr_s, sem_misc.at[2])
    x_cp = pltpu.make_async_copy(xh, x_s, sem_misc.at[5])
    c_cp = pltpu.make_async_copy(ch, c_s, sem_misc.at[6])
    wo_cp = pltpu.make_async_copy(woh, wo_s, sem_misc.at[7])
    wni_cp = pltpu.make_async_copy(wi_hbm.at[pl.ds(512, 1)], wni_s, sem_misc.at[8])

    def pair_cps(p, slot):
        cps = []
        for i, (src, dst) in enumerate(((wqh, wq_s), (wkh, wk_s), (wvh, wv_s))):
            for par in range(2):
                cps.append(pltpu.make_async_copy(
                    src.at[:, par * 16 + p], dst.at[slot, par], sem_pair.at[slot * 6 + 2 * i + par]))
        return cps

    gt_cp = pltpu.make_async_copy(gt_hbm, gt_s, sem_misc.at[3])

    def start_a_inputs():
        x_cp.start()
        c_cp.start()
        for cp in pair_cps(0, 0) + pair_cps(1, 1):
            cp.start()

    if do_b:
        gt_cp.start()
        fc_cp.start()
        bx_cp(0, 0).start()
        bx_cp(0, 1).start()
        for p in range(1, bx_win):
            bx_cp(p, 0).start()
            bx_cp(p, 1).start()
        wnr_cp.start()
        wni_cp.start()
    if do_a and not do_b:
        start_a_inputs()

    zero = flag_ref[0] - 1
    fence = flag_ref[0] > 0

    if do_b:
        lane0 = jax.lax.broadcasted_iota(jnp.int32, (1, 128), 1) == 0
        row0 = jax.lax.broadcasted_iota(jnp.int32, (8, 128), 0) == 0

        gt_cp.wait()
        f_r, f_i = gt_s[pl.ds(0, 128), :], gt_s[pl.ds(128, 128), :]
        for ap in range(16):
            t_r, t_i = gt_s[pl.ds(256 + ap, 1), :], gt_s[pl.ds(272 + ap, 1), :]
            g_r = _pk2(f_r * t_r - f_i * t_i)
            g_i = _pk2(f_r * t_i + f_i * t_r)
            gf_s[ap] = jnp.concatenate([jnp.concatenate([g_r, g_i], axis=1),
                                        jnp.concatenate([g_i ^ jnp.uint32(0x80008000), g_r], axis=1)], axis=0)
        fc_cp.wait()

        def b1_prep(p):
            if p % b1_grp == 0:
                for q in range(p, p + b1_grp):
                    bx_cp(q, 0).wait()
                    bx_cp(q, 1).wait()
                for q in range(p, p + b1_grp):
                    if q + bx_win < 8:
                        bx_cp(q + bx_win, 0).start()
                        bx_cp(q + bx_win, 1).start()
                if p <= w_at < p + b1_grp:
                    for j in range(16):
                        w_cp(j, 0).start()
                        w_cp(j, 1).start()
            planes = []
            for h in range(2):
                halves = []
                for par in range(2):
                    xf = pltpu.unpack_elementwise(bx_s[p, par], index=h, packed_dtype=_BF16,
                                                  unpacked_dtype=_F32)
                    xs = [xf[:, 128 * n:128 * (n + 1)] for n in range(8)]
                    a_, b_ = xs[0] + xs[4], xs[0] - xs[4]
                    c_, d_ = xs[2] + xs[6], xs[2] - xs[6]
                    e_, f_ = xs[1] + xs[5], xs[1] - xs[5]
                    g_, h_ = xs[3] + xs[7], xs[3] - xs[7]
                    u_ = (f_ - h_) * _R2
                    v_ = (f_ + h_) * _R2
                    ac, eg = a_ + c_, e_ + g_
                    halves.append([ac + eg, ac - eg, b_ + u_, d_ + v_, a_ - c_, e_ - g_, b_ - u_, d_ - v_])
                planes.append([jnp.concatenate([halves[0][i], halves[1][i]], axis=0).astype(_BF16)
                               for i in range(8)])
            return planes

        def b1_mm(p, planes, hs=(0, 1)):
            for h in hs:
                pln = planes[h]
                ap = 2 * p + h
                f0 = _bf(fc_s[0, pl.ds(0, 64), :])
                o0 = jax.lax.dot_general(f0[:, 0:128], pln[0], _NT, preferred_element_type=_F32)
                o4 = jax.lax.dot_general(f0[:, 128:256], pln[1], _NT, preferred_element_type=_F32)
                nq = jnp.where(row0, o0[64:72], 0.0)
                im0 = jnp.concatenate([jnp.where(row0, 0.0, o0[64:72]), o0[72:128]], axis=0)
                nq_s[:, pl.ds(128 * ap, 128)] = _pk2(jnp.concatenate([nq, jnp.zeros_like(nq)], axis=0))
                x1_s[ap, 0] = jnp.concatenate(
                    [jnp.concatenate([_pk2(o0[0:64]), _pk2(o4[0:64])], axis=0),
                     jnp.concatenate([_pk2(im0), _pk2(o4[64:128])], axis=0)], axis=1)
                for j in (1, 2, 3):
                    rhs = jnp.concatenate([pln[2 * j], pln[2 * j + 1]], axis=1)
                    o = jax.lax.dot_general(_bf(fc_s[j]), rhs, _NT, preferred_element_type=_F32)
                    x1_s[ap, j] = jnp.concatenate([_pk2(o[0:128]), _pk2(o[128:256])], axis=1)

        if b1_pipe == 2:
            cur = b1_prep(0)
            b1_mm(0, cur, (0,))
            for p in range(8):
                if p + 1 < 8:
                    nxt = b1_prep(p + 1)
                b1_mm(p, cur, (1,))
                if p + 1 < 8:
                    b1_mm(p + 1, nxt, (0,))
                    cur = nxt
        elif b1_pipe:
            nxt = b1_prep(0)
            for p in range(8):
                cur = nxt
                if p + 1 < 8:
                    nxt = b1_prep(p + 1)
                b1_mm(p, cur)
        else:
            for p in range(8):
                b1_mm(p, b1_prep(p))

        def spectral(us, w_of):
            xs = _fft16(us, -1)
            qs = []
            for j in range(16):
                (sr, xr), (si, xi) = xs[j]
                wr, wi = w_of(j)
                qs.append((_sub((sr, xr * wr), (si, xi * wi)), _add((sr, xr * wi), (si, xi * wr))))
            res = _fft16(qs, +1)
            assert all(r[0][0] == 1 and r[1][0] == 1 for r in res)
            return [(r[0][1], r[1][1]) for r in res]

        u_s, q_s = (u0_s, u1_s, u2_s, u3_s), (q0_s, q1_s)

        def s_fwd(t, ap):
            u_s[t][ap] = _dot(_bf(x1_s[ap, t]), _bf(gf_s[ap]))

        def filt(t, g):
            R = rg_rows
            r0 = R * g
            cls = _CLS[t][r0 // 64]
            k0 = r0 % 64
            rows = pl.ds(pl.multiple_of(r0 + zero, R), R)

            def w_of(j):
                return tuple(pltpu.unpack_elementwise(
                    ws.at[j, pl.ds(pl.multiple_of(zero, 64), 256)][pl.ds(cls // 2 + 4 * k0, R, stride=4), :],
                    index=cls % 2, packed_dtype=_BF16, unpacked_dtype=_F32) for ws in (wr_s, wi_s))

            res = spectral([((1, u_s[t][ap, rows, pl.ds(0, 128)]), (1, u_s[t][ap, rows, pl.ds(128, 128)]))
                            for ap in range(16)], w_of)
            for ap in range(16):
                if R == 8:
                    q_s[t % 2][ap, pl.ds(r0, 8), :] = jnp.concatenate([res[ap][0], res[ap][1]], axis=1)
                else:
                    q_s[t % 2][ap, pl.ds(r0 // 2, 8), :] = jnp.concatenate([_pk2(res[ap][0]), _pk2(res[ap][1])], axis=1)
            if chain:
                tail = res[15][1][0:8]
                u_s[t][16, pl.ds(pl.multiple_of(zero, 8), 8), pl.ds(0, 128)] = tail
                for ws in (wr_s, wi_s):
                    ws[16, pl.ds(pl.multiple_of(zero, 8), 8), :] = pltpu.bitcast(tail, _U32)

        def s_inv(t, ap):
            q = q_s[t % 2][ap].astype(_BF16) if rg_rows == 8 else _bf(q_s[t % 2][ap])
            o = jax.lax.dot_general(_bf(gf_s[ap]), q, _NT, preferred_element_type=_F32)
            vi = o[128:256]
            if t == 0:
                vi = jnp.where(lane0, vc_s[ap], vi)
            v_s[ap, t] = jnp.concatenate([_pk2(o[0:128]), _pk2(vi)], axis=1)

        def nyquist(un):
            wnr = wnr_s[...].astype(_F32)
            wni = wni_s[...].astype(_F32)
            qn = spectral([((1, u[:, 0:128]), (1, u[:, 128:256])) for u in un],
                          lambda j: (wnr[:, 128 * j:128 * (j + 1)], wni[:, 128 * j:128 * (j + 1)]))
            for ap in range(16):
                lhs = jnp.concatenate([qn[ap][0], qn[ap][1]], axis=1).astype(_BF16)
                vn = jax.lax.dot_general(lhs, _bf(gf_s[ap, pl.ds(0, 64), :]), _NT,
                                         preferred_element_type=_F32)
                vn = jnp.concatenate([vn, jnp.zeros((112, 128), _F32)], axis=0)
                vc_s[ap] = vn.T

        def b2_head():
            un = [_dot(_bf(nq_s[:, pl.ds(128 * ap, 128)]), _bf(gf_s[ap, pl.ds(0, 64), :])) for ap in range(16)]
            for ap in range(16):
                u = _dot(_bf(x1_s[ap, 0:n_pre].reshape(64 * n_pre, 256)), _bf(gf_s[ap]))
                for t in range(n_pre):
                    u_s[t][ap] = u[128 * t:128 * (t + 1)]
                if ap == 7:
                    nyquist(un)

        wnr_cp.wait()
        wni_cp.wait()
        pl.when(fence)(b2_head)
        for j in range(16):
            w_cp(j, 0).wait()
            w_cp(j, 1).wait()
        ic_cp.start()
        if do_a:
            start_a_inputs()
        def b2_slot(t):
            ng = 128 // rg_rows
            for g in range(ng):
                filt(t, g)
                for k in range(16 // ng):
                    if t + n_pre < 4:
                        s_fwd(t + n_pre, (16 // ng) * g + k)
                    if t > 0:
                        s_inv(t - 1, (16 // ng) * g + k)

        for t in range(4):
            pl.when(flag_ref[t + 1] > 0)(functools.partial(b2_slot, t))

        def b2_tail():
            for ap in range(16):
                s_inv(3, ap)

        pl.when(fence)(b2_tail)

        def ob_cp(p):
            return pltpu.make_async_copy(ob_s.at[p], outh.at[:, p, pl.ds(1024, 1024)], sem_ob.at[p])

        def b3():
            ic_cp.wait()

            for pq in range(8 // b3_p):
                aps = range(2 * b3_p * pq, 2 * b3_p * (pq + 1))
                cc = [_dot(_bf(jnp.concatenate([v_s[ap, t] for ap in aps], axis=0)), _bf(ic_s[t]))
                      for t in range(4)]
                c0, c4 = cc[0][:, 0:128], cc[0][:, 128:256]
                c1r, c1i = cc[1][:, 0:128], cc[1][:, 128:256]
                c2r, c2i = cc[2][:, 0:128], cc[2][:, 128:256]
                c3r, c3i = cc[3][:, 0:128], cc[3][:, 128:256]
                pp, mm = c0 + c4, c0 - c4
                u1, u2, u3, u4 = c1r + c3r, c1i - c3i, c1r - c3r, c1i + c3i
                t1, t2 = (u3 - u4) * _R2, (u3 + u4) * _R2
                e0, e1, e2, e3 = pp + c2r, pp - c2r, mm - c2i, mm + c2i
                ys = [e0 + u1, e2 + t1, e1 - u2, e3 - t2, e0 - u1, e2 - t1, e1 + u2, e3 + t2]
                for k in range(b3_p):
                    p = b3_p * pq + k
                    ob_s[p] = jnp.concatenate(
                        [pltpu.pack_elementwise([y[256 * k:256 * k + 128], y[256 * k + 128:256 * k + 256]],
                                                packed_dtype=_BF16) for y in ys], axis=1)
                    ob_cp(p).start()

        if b3_at == 0 or not do_a:
            b3()

    if do_a:
        x_cp.wait()
        c_cp.wait()

        def project_units(slot, half, dst, rows):
            def split(ref):
                a = ref[slot, 0]
                b = ref[slot, 1]
                if half == 1:
                    a, b = a >> 16, b >> 16
                return _bf(pltpu.pack_elementwise([a, b], packed_dtype=jnp.uint16))

            wq = split(wq_s)
            wkv = jnp.concatenate([split(wk_s), split(wv_s)], axis=1)

            def q_unit(r0):
                q = _dot(_bf(x_s[pl.ds(r0 // 2, rows // 2), :]), wq) * _QSCALE
                _st(dst.at[pl.ds(r0 // 2, rows // 2), pl.ds(0, 128)], q, 'a')

            def kv_unit(r0):
                kv = _dot(_bf(c_s[pl.ds(r0 // 2, rows // 2), :]), wkv)
                _st(dst.at[pl.ds(r0 // 2, rows // 2), pl.ds(128, 256)], kv, 'a')

            units = []
            for r0 in range(0, S, rows):
                units.append(functools.partial(kv_unit, r0))
                units.append(functools.partial(q_unit, r0))
            return units

        def attend(p, t, src, fillers, bq=bq, sorder=sorder, last_cfg=last_cfg, afence=afence, chain=chain, b1_pipe=b1_pipe, b1_grp=b1_grp):
            head = (_HeadWide if wide else _Head)(*[_bf(src[:, pl.ds(128 * i, 128)]) for i in range(3)], bq)
            ns = S // bq
            fillers = list(fillers)
            nslots = ns * fill_slots
            total = len(fillers)
            slot = [0]

            def fill():
                slot[0] += 1
                while fillers and (total - len(fillers)) * nslots < total * slot[0]:
                    fillers.pop(0)()

            order = list(range(ns))
            if sorder == 1:
                order = order[::-1]
            elif sorder == 2:
                order = [order[-1 - n // 2] if n % 2 == 0 else order[n // 2] for n in range(ns)]
            elif sorder == 3:
                order = [order[n // 2] if n % 2 == 0 else order[-1 - n // 2] for n in range(ns)]
            for n in range(min(lookahead, ns)):
                head.qk(order[n])
            for n in range(ns):
                if n + lookahead < ns:
                    head.qk(order[n + lookahead])
                if fill_slots == 2:
                    fill()
                i = order[n]
                _st(ctx_s.at[p, pl.ds(i * bq // 2, bq // 2), pl.ds(t * 128, 128)], head.pv(i), 'a')
                fill()
            while fillers:
                fillers.pop(0)()

        npair = H // 2
        for cp in pair_cps(0, 0):
            cp.wait()
        for u in project_units(0, 0, qkv0_s, 2048):
            u()

        def pair_step(p, last):
            s0 = p % 3
            attend(p, 0, qkv0_s, project_units(s0, 1, qkv1_s, frows))
            if last:
                attend(p, 1, qkv1_s, [], *last_cfg)
            else:
                attend(p, 1, qkv1_s, project_units((p + 1) % 3, 0, qkv0_s, frows))

        def a_body(p, carry):
            for cp in pair_cps(p + 1, (p + 1) % 3):
                cp.wait()

            @pl.when(p + 2 < npair)
            def _():
                for cp in pair_cps(p + 2, (p + 2) % 3):
                    cp.start()

            @pl.when(p == 2)
            def _():
                wo_cp.start()

            if afence:
                pl.when(fence)(lambda: pair_step(p, False))
            else:
                pair_step(p, False)
            return carry

        jax.lax.fori_loop(0, npair - 1, a_body, 0)
        if b3_at == 1 and do_b:
            b3()
        pair_step(npair - 1, True)
        if b3_at == 2 and do_b:
            b3()

        wo_cp.wait()

        def oa_cp(i):
            return pltpu.make_async_copy(oa_s.at[i % 2], outh.at[pl.ds(16 * i, 16), :, pl.ds(0, 1024)],
                                         sem_oa.at[i % 2])

        def o_body(i, carry):
            r0 = pl.multiple_of(i * 128, 128)
            lhs = _bf(jnp.concatenate([ctx_s[p, pl.ds(r0, 128), :] for p in range(H // 2)], axis=1))
            res = _dot(lhs, _bf(wo_s[...]))

            @pl.when(i >= 2)
            def _():
                oa_cp(i - 2).wait()

            _st(oa_s.at[i % 2], res.reshape(16, 16, M))
            oa_cp(i).start()
            return carry

        jax.lax.fori_loop(0, 8, o_body, 0)
        oa_cp(6).wait()
        oa_cp(7).wait()

    if do_b:
        for p in range(8):
            ob_cp(p).wait()


def _run(A_x, A_c_kv, A_w_q, A_w_uk, A_w_uv, A_w_o, B_x, B_w_r, B_w_i, *, bq=256, do_a=True, do_b=True, rg_rows=8, n_pre=3, frows=128, fill_slots=2, lookahead=1, dbg=0, wide=True, bx_win=3, w_at=5, b3_at=0, b3_p=2, sorder=2, last_cfg=(128, 0), pad=8, cp=dict(disable_bounds_checks=True, disable_semaphore_checks=True), afence=0, chain=0, b1_pipe=0, b1_grp=1, sta=0, stb=0, flags=None):
    _STMODE['a'], _STMODE['b'] = sta, stb
    any_spec = pl.BlockSpec(memory_space=pltpu.HBM)
    vm = pltpu.VMEM
    dma = pltpu.SemaphoreType.DMA
    scratch = [
        vm((pad, 128), _U32),
        vm((1024, 1024), _U32),
        vm((1024, 512), _U32),
        vm((2048, 1024), _U32),
        vm((3, 2, 512, 128), _U32),
        vm((3, 2, 256, 128), _U32),
        vm((3, 2, 256, 128), _U32),
        vm((1024, 384), _U32), vm((1024, 384), _U32),
        vm((16, 1024, 256), _U32),
        vm((2, 16, 8, 1024), _U32),
        vm((8, 2, 64, 1024), _U32),
        vm((17, 256, 128), _U32),
        vm((17, 256, 128), _U32),
        vm((1, 2048), _BF16),
        vm((1, 2048), _BF16),
        vm((4, 128, 256), _U32),
        vm((4, 128, 256), _U32),
        vm((288, 128), _F32),
        vm((16, 128, 256), _U32),
        vm((16, 4, 64, 256), _U32),
        vm((8, 2048), _U32),
        vm((16, 4, 64, 256), _U32),
        vm((8, 128, 1024), _U32),
        vm((17, 128, 256), _F32), vm((17, 128, 256), _F32), vm((17, 128, 256), _F32), vm((17, 128, 256), _F32),
        *([vm((16, 128, 256), _F32)] * 2 if rg_rows == 8 else [vm((16, 64, 256), _U32)] * 2),
        vm((16, 128, 128), _F32),
        dma((16,)), dma((9,)), dma((32,)), dma((18,)), dma((8,)), dma((2,)),
    ]
    out = pl.pallas_call(
        functools.partial(_kernel, bq=bq, do_a=do_a, do_b=do_b, rg_rows=rg_rows, n_pre=n_pre, frows=frows, fill_slots=fill_slots, lookahead=lookahead, dbg=dbg, wide=wide, bx_win=bx_win, w_at=w_at, b3_at=b3_at, b3_p=b3_p, sorder=sorder, last_cfg=last_cfg, afence=afence, chain=chain, b1_pipe=b1_pipe, b1_grp=b1_grp),
        out_shape=jax.ShapeDtypeStruct((128, 16, 2048), _BF16),
        in_specs=[pl.BlockSpec(memory_space=pltpu.SMEM)] + [any_spec] * 12,
        out_specs=any_spec,
        scratch_shapes=scratch,
        compiler_params=pltpu.CompilerParams(vmem_limit_bytes=112 * 1024 * 1024, flags=flags, **(cp or {})),
    )(jnp.asarray(np.arange(1, 9, dtype=np.int32)), *[pltpu.with_memory_space_constraint(a, pltpu.HBM) for a in (
        A_x.reshape(S, M), A_c_kv.reshape(S, DC),
        A_w_q.reshape(512, 64, HD), A_w_uk.reshape(256, 64, HD), A_w_uv.reshape(256, 64, HD),
        A_w_o.reshape(H * HD, M),
        B_x.reshape(64, 32, BD), B_w_r.T, B_w_i.T,
        jnp.asarray(_FC), jnp.asarray(_IC_NAT if rg_rows == 8 else _IC), jnp.asarray(_GT),
    )])
    return out.reshape(1, S, 2048)


@jax.jit
def pallas_concat_heads__compressed_kv_cla__spectral_gfnet__prompt_kernel(
    A_x: jax.Array,
    A_c_kv: jax.Array,
    A_w_q: jax.Array,
    A_w_uk: jax.Array,
    A_w_uv: jax.Array,
    A_w_o: jax.Array,
    B_x: jax.Array,
    B_w_r: jax.Array,
    B_w_i: jax.Array,
):
    return _run(A_x, A_c_kv, A_w_q, A_w_uk, A_w_uv, A_w_o, B_x, B_w_r, B_w_i)
```

```python
import functools

import numpy as np
import jax
import jax.numpy as jnp
import jax.experimental.pallas as pl
import jax.experimental.pallas.tpu as pltpu

S = 2048
M = 1024
H = 32
HD = 128
DC = 512
BD = 1024
NG = 8

_U32 = jnp.uint32
_BF16 = jnp.bfloat16
_F32 = jnp.float32
_NT = (((1,), (1,)), ((), ()))
_QSCALE = float(HD ** -0.5 * np.log2(np.e))
_MASKED = -1e9


def _to_bf16_bits(a):
    u = np.ascontiguousarray(a, dtype=np.float32).view(np.uint32).astype(np.uint64)
    r = (u + 0x7FFF + ((u >> 16) & 1)) >> 16
    return r.astype(np.uint32) & 0xFFFF


def _pack_rows(a):
    b = _to_bf16_bits(a)
    return (b[0::2] | (b[1::2] << 16)).astype(np.uint32)


def _neg(p):
    return None if p is None else (-p[0], p[1])


def _add(p, q):
    if p is None:
        return q
    if q is None:
        return p
    if p[0] == q[0]:
        return (p[0], p[1] + q[1])
    if p[0] > 0:
        return (1, p[1] - q[1])
    return (1, q[1] - p[1])


def _sub(p, q):
    return _add(p, _neg(q))


def _scale(p, f):
    if p is None:
        return None
    return (p[0] * (1 if f > 0 else -1), p[1] * abs(f))


def _cadd(x, y):
    return (_add(x[0], y[0]), _add(x[1], y[1]))


def _csub(x, y):
    return (_sub(x[0], y[0]), _sub(x[1], y[1]))


def _cmul_i(x, s):
    return (_neg(x[1]), x[0]) if s > 0 else (x[1], _neg(x[0]))


def _cmul_w(x, n, sgn):
    n = n % 16
    if n == 0:
        return x
    if n == 4:
        return _cmul_i(x, sgn)
    if n == 8:
        return (_neg(x[0]), _neg(x[1]))
    if n == 12:
        return _cmul_i(x, -sgn)
    wr = float(np.cos(2 * np.pi * n / 16))
    wi = float(sgn * np.sin(2 * np.pi * n / 16))
    re, im = x
    if n % 2 == 0:
        r = abs(wr)
        sr = 1 if wr > 0 else -1
        si = 1 if wi > 0 else -1
        a = _sub(re if sr > 0 else _neg(re), im if si > 0 else _neg(im))
        b = _add(re if si > 0 else _neg(re), im if sr > 0 else _neg(im))
        return (_scale(a, r), _scale(b, r))
    return (_sub(_scale(re, wr), _scale(im, wi)), _add(_scale(re, wi), _scale(im, wr)))


def _dft4(x0, x1, x2, x3, sgn):
    s02, d02 = _cadd(x0, x2), _csub(x0, x2)
    s13, d13 = _cadd(x1, x3), _csub(x1, x3)
    r = _cmul_i(d13, sgn)
    return [_cadd(s02, s13), _cadd(d02, r), _csub(s02, s13), _csub(d02, r)]


def _fft16(xs, sgn):
    t = [_dft4(xs[a0], xs[4 + a0], xs[8 + a0], xs[12 + a0], sgn) for a0 in range(4)]
    t = [[_cmul_w(t[a0][j0], a0 * j0, sgn) for j0 in range(4)] for a0 in range(4)]
    out = [None] * 16
    for j0 in range(4):
        r = _dft4(t[0][j0], t[1][j0], t[2][j0], t[3][j0], sgn)
        for j1 in range(4):
            out[j0 + 4 * j1] = r[j1]
    return out


def _net_signs(sgn):
    out = _fft16([((1, 1.0), (1, 1.0)) for _ in range(16)], sgn)
    return [(o[0][0], o[1][0]) for o in out]


_INV_SIGNS = _net_signs(+1)
_CLS = ((0, 4), (1, 7), (2, 6), (3, 5))
_R2 = float(np.sqrt(0.5))


def _build_consts():
    n2 = np.arange(128)
    kap = np.arange(64)

    def wl(l):
        return np.exp(-2j * np.pi * np.outer(l, n2) / 1024)

    fc = np.zeros((4, 256, 256))
    w = wl(8 * kap)
    fc[0, 0:64, 0:128] = w.real
    fc[0, 64:128, 0:128] = w.imag
    fc[0, 64, 0:128] = (-1.0) ** n2
    w = wl(4 + 8 * kap)
    fc[0, 0:64, 128:256] = w.real
    fc[0, 64:128, 128:256] = w.imag
    for j in (1, 2, 3):
        si = 1.0 if j == 3 else -1.0
        w1, w2 = wl(j + 8 * kap), wl(8 - j + 8 * kap)
        fc[j, 0:64, 0:128], fc[j, 0:64, 128:] = w1.real, -w1.imag * si
        fc[j, 64:128, 0:128], fc[j, 64:128, 128:] = w2.real, w2.imag * si
        fc[j, 128:192, 0:128], fc[j, 128:192, 128:] = w1.imag, w1.real * si
        fc[j, 192:256, 0:128], fc[j, 192:256, 128:] = w2.imag, -w2.real * si

    def cs(l, c):
        ph = 2 * np.pi * np.outer(l, n2) / 1024
        return c[:, None] * np.cos(ph) / 1024, c[:, None] * np.sin(ph) / 1024

    ic = np.zeros((4, 256, 256))
    two = np.full(64, 2.0)
    co, si = cs(8 * kap, np.where(kap == 0, 1.0, 2.0))
    ic[0, 0:64, 0:128], ic[0, 128:192, 0:128] = co, -si
    ic[0, 128, 0:128] = (-1.0) ** n2 / 1024
    co, si = cs(4 + 8 * kap, two)
    ic[0, 64:128, 128:], ic[0, 192:256, 128:] = co, -si
    for j in (1, 2, 3):
        co, si = cs(j + 8 * kap, two)
        ic[j, 0:64, 0:128], ic[j, 128:192, 0:128] = co, -si
        ic[j, 0:64, 128:], ic[j, 128:192, 128:] = si, co
        co, si = cs(8 - j + 8 * kap, two)
        ic[j, 64:128, 0:128], ic[j, 192:256, 0:128] = co, -si
        ic[j, 64:128, 128:], ic[j, 192:256, 128:] = -si, -co

    f128 = np.exp(-2j * np.pi * np.outer(n2, n2) / 128)
    tw = np.exp(-2j * np.pi * np.outer(np.arange(16), n2) / 2048)

    def even_odd(m, blk):
        r = m.reshape(-1, blk // 2, 2, m.shape[-1])
        return np.concatenate([r[:, :, 0], r[:, :, 1]], axis=1).reshape(m.shape)

    fc[0] = even_odd(fc[0], 64)
    for j in (1, 2, 3):
        fc[j] = even_odd(fc[j], 128)
    il = np.arange(256).reshape(16, 2, 8).transpose(0, 2, 1).reshape(-1)
    ic_nat = ic
    ic = ic[:, il, :]
    sigma = np.concatenate([np.arange(0, 128, 2), np.arange(1, 128, 2)])
    fpos = f128[sigma]
    gt = np.concatenate([fpos[0::2].real, fpos[1::2].real, fpos[0::2].imag, fpos[1::2].imag,
                         tw.real, tw.imag], axis=0).astype(np.float32)

    def pk(m):
        return np.stack([_pack_rows(x) for x in m])

    return pk(fc), pk(ic / 2048), pk(ic_nat / 2048), gt


_FC, _IC, _IC_NAT, _GT = _build_consts()
assert all(sg == (1, 1) for sg in _INV_SIGNS)


def _bf(x_u32):
    return pltpu.bitcast(x_u32, _BF16)


def _pk(x_f32):
    return pltpu.bitcast(x_f32.astype(_BF16), _U32)


_STMODE = {"a": 1, "b": 1}


def _st(ref, x_f32, part="b"):
    if _STMODE[part]:
        ref.bitcast(_BF16)[...] = x_f32.astype(_BF16)
    else:
        ref[...] = _pk(x_f32)


def _pk2(x_f32):
    r = x_f32.shape[0] // 2
    return pltpu.pack_elementwise([x_f32[:r], x_f32[r:]], packed_dtype=_BF16)


def _dot(a, b):
    return jnp.dot(a, b, preferred_element_type=_F32)


def _val(p, like):
    if p is None:
        return jnp.zeros_like(like)
    return p[1] if p[0] > 0 else -p[1]


class _Head:
    def __init__(self, q, k, v, bq):
        self.q, self.k, self.v, self.bq = q, k, v, bq
        self.state = {}
        row = jax.lax.broadcasted_iota(jnp.int32, (128, 128), 0)
        col = jax.lax.broadcasted_iota(jnp.int32, (128, 128), 1)
        self.causal = col <= row

    def qk(self, i):
        bq = self.bq
        q0 = i * bq
        qq = self.q[q0:q0 + bq]
        nt = (q0 + bq) // 128
        mx = None
        ss = []
        for j in range(nt):
            r0 = max(0, j * 128 - q0)
            s = jax.lax.dot_general(qq[r0:], self.k[j * 128:(j + 1) * 128], _NT,
                                    preferred_element_type=_F32)
            if j * 128 >= q0:
                sd = jnp.where(self.causal, s[:128], _MASKED)
                s = jnp.concatenate([sd, s[128:]], axis=0) if s.shape[0] > 128 else sd
            ss.append(s)
            if mx is None:
                mx = s
            elif r0 == 0:
                mx = jnp.maximum(mx, s)
            else:
                mx = jnp.concatenate([mx[:r0], jnp.maximum(mx[r0:], s)], axis=0)
        self.state[i] = (ss, jnp.max(mx, axis=1, keepdims=True))

    def pv(self, i):
        bq = self.bq
        q0 = i * bq
        ss, m = self.state.pop(i)
        acc = None
        lsum = None
        for j, s in enumerate(ss):
            r0 = max(0, j * 128 - q0)
            p = jnp.exp2(s - m[r0:])
            pv = _dot(p.astype(_BF16), self.v[j * 128:(j + 1) * 128])
            if acc is None:
                acc, lsum = pv, p
            elif r0 == 0:
                acc, lsum = acc + pv, lsum + p
            else:
                acc = jnp.concatenate([acc[:r0], acc[r0:] + pv], axis=0)
                lsum = jnp.concatenate([lsum[:r0], lsum[r0:] + p], axis=0)
        l = jnp.sum(lsum, axis=1, keepdims=True)
        r = pl.reciprocal(l, approx=True)
        r = r * (2.0 - l * r)
        return acc * r


class _HeadWide(_Head):
    def qk(self, i):
        bq = self.bq
        q0 = i * bq
        parts = []
        for r in range(bq // 128):
            c0, c1 = (0, q0 + 128) if r == 0 else (q0 + 128 * r, q0 + 128 * (r + 1))
            s = jax.lax.dot_general(self.q[q0 + 128 * r:q0 + bq], self.k[c0:c1], _NT,
                                    preferred_element_type=_F32)
            w = c1 - c0
            top = jnp.where(self.causal, s[:128, w - 128:], _MASKED)
            if w > 128:
                top = jnp.concatenate([s[:128, :w - 128], top], axis=1)
            s = jnp.concatenate([top, s[128:]], axis=0) if s.shape[0] > 128 else top
            parts.append(s)
        mx = jnp.max(parts[0], axis=1, keepdims=True)
        for r in range(1, bq // 128):
            mr = jnp.max(parts[r], axis=1, keepdims=True)
            mx = jnp.concatenate([mx[:128 * r], jnp.maximum(mx[128 * r:], mr)], axis=0)
        self.state[i] = (parts, mx)

    def pv(self, i):
        bq = self.bq
        q0 = i * bq
        parts, m = self.state.pop(i)
        acc = l = None
        for r, s in enumerate(parts):
            c0, c1 = (0, q0 + 128) if r == 0 else (q0 + 128 * r, q0 + 128 * (r + 1))
            p = jnp.exp2(s - m[128 * r:])
            lr = jnp.sum(p, axis=1, keepdims=True)
            o = _dot(p.astype(_BF16), self.v[c0:c1])
            if r == 0:
                acc, l = o, lr
            else:
                acc = jnp.concatenate([acc[:128 * r], acc[128 * r:] + o], axis=0)
                l = jnp.concatenate([l[:128 * r], l[128 * r:] + lr], axis=0)
        rc = pl.reciprocal(l, approx=True)
        rc = rc * (2.0 - l * rc)
        return acc * rc


def _kernel(flag_ref, x_hbm, c_hbm, wq_hbm, wk_hbm, wv_hbm, wo_hbm, bx_hbm, wr_hbm, wi_hbm,
            fc_hbm, ic_hbm, gt_hbm,
            out_hbm,
            pad_s, x_s, c_s, wo_s, wq_s, wk_s, wv_s, qkv0_s, qkv1_s, ctx_s, oa_s,
            bx_s, wr_s, wi_s, wnr_s, wni_s, fc_s, ic_s, gt_s, gf_s, x1_s, nq_s, v_s, ob_s, u0_s, u1_s, u2_s, u3_s, q0_s, q1_s, vc_s,
            sem_bx, sem_misc, sem_w, sem_pair, sem_ob, sem_oa, *, bq, do_a, do_b, rg_rows, n_pre, frows, fill_slots, lookahead, dbg, wide, bx_win, w_at, b3_at, b3_p, sorder, last_cfg, afence, chain, b1_pipe, b1_grp, orows):
    xh = x_hbm.bitcast(_U32)
    ch = c_hbm.bitcast(_U32)
    wqh = wq_hbm.bitcast(_U32)
    wkh = wk_hbm.bitcast(_U32)
    wvh = wv_hbm.bitcast(_U32)
    woh = wo_hbm.bitcast(_U32)
    bxh = bx_hbm.bitcast(_U32)
    wrh = wr_hbm.at[pl.ds(0, 512)].bitcast(_U32)
    wih = wi_hbm.at[pl.ds(0, 512)].bitcast(_U32)
    outh = out_hbm.bitcast(_U32)

    def bx_cp(p, par):
        return pltpu.make_async_copy(bxh.at[:, par * 8 + p], bx_s.at[p, par], sem_bx.at[2 * p + par])

    def w_cp(j, which):
        src, dst = (wrh, wr_s) if which == 0 else (wih, wi_s)
        return pltpu.make_async_copy(src.at[:, pl.ds(128 * j, 128)], dst.at[j], sem_w.at[2 * j + which])

    fc_cp = pltpu.make_async_copy(fc_hbm, fc_s, sem_misc.at[0])
    ic_cp = pltpu.make_async_copy(ic_hbm, ic_s, sem_misc.at[1])
    wnr_cp = pltpu.make_async_copy(wr_hbm.at[pl.ds(512, 1)], wnr_s, sem_misc.at[2])
    x_cp = pltpu.make_async_copy(xh, x_s, sem_misc.at[5])
    c_cp = pltpu.make_async_copy(ch, c_s, sem_misc.at[6])
    wo_cp = pltpu.make_async_copy(woh, wo_s, sem_misc.at[7])
    wni_cp = pltpu.make_async_copy(wi_hbm.at[pl.ds(512, 1)], wni_s, sem_misc.at[8])

    def pair_cps(p, slot):
        cps = []
        for i, (src, dst) in enumerate(((wqh, wq_s), (wkh, wk_s), (wvh, wv_s))):
            for par in range(2):
                cps.append(pltpu.make_async_copy(
                    src.at[:, par * 16 + p], dst.at[slot, par], sem_pair.at[slot * 6 + 2 * i + par]))
        return cps

    gt_cp = pltpu.make_async_copy(gt_hbm, gt_s, sem_misc.at[3])

    def start_a_inputs():
        x_cp.start()
        c_cp.start()
        for cp in pair_cps(0, 0) + pair_cps(1, 1):
            cp.start()

    if do_b:
        gt_cp.start()
        fc_cp.start()
        bx_cp(0, 0).start()
        bx_cp(0, 1).start()
        for p in range(1, bx_win):
            bx_cp(p, 0).start()
            bx_cp(p, 1).start()
        wnr_cp.start()
        wni_cp.start()
    if do_a and not do_b:
        start_a_inputs()

    zero = flag_ref[0] - 1
    fence = flag_ref[0] > 0

    if do_b:
        lane0 = jax.lax.broadcasted_iota(jnp.int32, (1, 128), 1) == 0
        row0 = jax.lax.broadcasted_iota(jnp.int32, (8, 128), 0) == 0

        gt_cp.wait()
        f_r, f_i = gt_s[pl.ds(0, 128), :], gt_s[pl.ds(128, 128), :]
        for ap in range(16):
            t_r, t_i = gt_s[pl.ds(256 + ap, 1), :], gt_s[pl.ds(272 + ap, 1), :]
            g_r = _pk2(f_r * t_r - f_i * t_i)
            g_i = _pk2(f_r * t_i + f_i * t_r)
            gf_s[ap] = jnp.concatenate([jnp.concatenate([g_r, g_i], axis=1),
                                        jnp.concatenate([g_i ^ jnp.uint32(0x80008000), g_r], axis=1)], axis=0)
        fc_cp.wait()

        def b1_prep(p):
            if p % b1_grp == 0:
                for q in range(p, p + b1_grp):
                    bx_cp(q, 0).wait()
                    bx_cp(q, 1).wait()
                for q in range(p, p + b1_grp):
                    if q + bx_win < 8:
                        bx_cp(q + bx_win, 0).start()
                        bx_cp(q + bx_win, 1).start()
                if p <= w_at < p + b1_grp:
                    for j in range(16):
                        w_cp(j, 0).start()
                        w_cp(j, 1).start()
            planes = []
            for h in range(2):
                halves = []
                for par in range(2):
                    xf = pltpu.unpack_elementwise(bx_s[p, par], index=h, packed_dtype=_BF16,
                                                  unpacked_dtype=_F32)
                    xs = [xf[:, 128 * n:128 * (n + 1)] for n in range(8)]
                    a_, b_ = xs[0] + xs[4], xs[0] - xs[4]
                    c_, d_ = xs[2] + xs[6], xs[2] - xs[6]
                    e_, f_ = xs[1] + xs[5], xs[1] - xs[5]
                    g_, h_ = xs[3] + xs[7], xs[3] - xs[7]
                    u_ = (f_ - h_) * _R2
                    v_ = (f_ + h_) * _R2
                    ac, eg = a_ + c_, e_ + g_
                    halves.append([ac + eg, ac - eg, b_ + u_, d_ + v_, a_ - c_, e_ - g_, b_ - u_, d_ - v_])
                planes.append([jnp.concatenate([halves[0][i], halves[1][i]], axis=0).astype(_BF16)
                               for i in range(8)])
            return planes

        def b1_mm(p, planes, hs=(0, 1)):
            for h in hs:
                pln = planes[h]
                ap = 2 * p + h
                f0 = _bf(fc_s[0, pl.ds(0, 64), :])
                o0 = jax.lax.dot_general(f0[:, 0:128], pln[0], _NT, preferred_element_type=_F32)
                o4 = jax.lax.dot_general(f0[:, 128:256], pln[1], _NT, preferred_element_type=_F32)
                nq = jnp.where(row0, o0[64:72], 0.0)
                im0 = jnp.concatenate([jnp.where(row0, 0.0, o0[64:72]), o0[72:128]], axis=0)
                nq_s[:, pl.ds(128 * ap, 128)] = _pk2(jnp.concatenate([nq, jnp.zeros_like(nq)], axis=0))
                x1_s[ap, 0] = jnp.concatenate(
                    [jnp.concatenate([_pk2(o0[0:64]), _pk2(o4[0:64])], axis=0),
                     jnp.concatenate([_pk2(im0), _pk2(o4[64:128])], axis=0)], axis=1)
                for j in (1, 2, 3):
                    rhs = jnp.concatenate([pln[2 * j], pln[2 * j + 1]], axis=1)
                    o = jax.lax.dot_general(_bf(fc_s[j]), rhs, _NT, preferred_element_type=_F32)
                    x1_s[ap, j] = jnp.concatenate([_pk2(o[0:128]), _pk2(o[128:256])], axis=1)

        if b1_pipe == 2:
            cur = b1_prep(0)
            b1_mm(0, cur, (0,))
            for p in range(8):
                if p + 1 < 8:
                    nxt = b1_prep(p + 1)
                b1_mm(p, cur, (1,))
                if p + 1 < 8:
                    b1_mm(p + 1, nxt, (0,))
                    cur = nxt
        elif b1_pipe:
            nxt = b1_prep(0)
            for p in range(8):
                cur = nxt
                if p + 1 < 8:
                    nxt = b1_prep(p + 1)
                b1_mm(p, cur)
        else:
            for p in range(8):
                b1_mm(p, b1_prep(p))

        def spectral(us, w_of):
            xs = _fft16(us, -1)
            qs = []
            for j in range(16):
                (sr, xr), (si, xi) = xs[j]
                wr, wi = w_of(j)
                qs.append((_sub((sr, xr * wr), (si, xi * wi)), _add((sr, xr * wi), (si, xi * wr))))
            res = _fft16(qs, +1)
            assert all(r[0][0] == 1 and r[1][0] == 1 for r in res)
            return [(r[0][1], r[1][1]) for r in res]

        u_s, q_s = (u0_s, u1_s, u2_s, u3_s), (q0_s, q1_s)

        def s_fwd(t, ap):
            u_s[t][ap] = _dot(_bf(x1_s[ap, t]), _bf(gf_s[ap]))

        def filt(t, g):
            R = rg_rows
            r0 = R * g
            cls = _CLS[t][r0 // 64]
            k0 = r0 % 64
            rows = pl.ds(pl.multiple_of(r0 + zero, R), R)

            def w_of(j):
                return tuple(pltpu.unpack_elementwise(
                    ws.at[j, pl.ds(pl.multiple_of(zero, 64), 256)][pl.ds(cls // 2 + 4 * k0, R, stride=4), :],
                    index=cls % 2, packed_dtype=_BF16, unpacked_dtype=_F32) for ws in (wr_s, wi_s))

            res = spectral([((1, u_s[t][ap, rows, pl.ds(0, 128)]), (1, u_s[t][ap, rows, pl.ds(128, 128)]))
                            for ap in range(16)], w_of)
            for ap in range(16):
                if R == 8:
                    q_s[t % 2][ap, pl.ds(r0, 8), :] = jnp.concatenate([res[ap][0], res[ap][1]], axis=1)
                else:
                    q_s[t % 2][ap, pl.ds(r0 // 2, 8), :] = jnp.concatenate([_pk2(res[ap][0]), _pk2(res[ap][1])], axis=1)
            if chain:
                tail = res[15][1][0:8]
                u_s[t][16, pl.ds(pl.multiple_of(zero, 8), 8), pl.ds(0, 128)] = tail
                for ws in (wr_s, wi_s):
                    ws[16, pl.ds(pl.multiple_of(zero, 8), 8), :] = pltpu.bitcast(tail, _U32)

        def s_inv(t, ap):
            q = q_s[t % 2][ap].astype(_BF16) if rg_rows == 8 else _bf(q_s[t % 2][ap])
            o = jax.lax.dot_general(_bf(gf_s[ap]), q, _NT, preferred_element_type=_F32)
            vi = o[128:256]
            if t == 0:
                vi = jnp.where(lane0, vc_s[ap], vi)
            v_s[ap, t] = jnp.concatenate([_pk2(o[0:128]), _pk2(vi)], axis=1)

        def nyquist(un):
            wnr = wnr_s[...].astype(_F32)
            wni = wni_s[...].astype(_F32)
            qn = spectral([((1, u[:, 0:128]), (1, u[:, 128:256])) for u in un],
                          lambda j: (wnr[:, 128 * j:128 * (j + 1)], wni[:, 128 * j:128 * (j + 1)]))
            for ap in range(16):
                lhs = jnp.concatenate([qn[ap][0], qn[ap][1]], axis=1).astype(_BF16)
                vn = jax.lax.dot_general(lhs, _bf(gf_s[ap, pl.ds(0, 64), :]), _NT,
                                         preferred_element_type=_F32)
                vn = jnp.concatenate([vn, jnp.zeros((112, 128), _F32)], axis=0)
                vc_s[ap] = vn.T

        def b2_head():
            un = [_dot(_bf(nq_s[:, pl.ds(128 * ap, 128)]), _bf(gf_s[ap, pl.ds(0, 64), :])) for ap in range(16)]
            for ap in range(16):
                u = _dot(_bf(x1_s[ap, 0:n_pre].reshape(64 * n_pre, 256)), _bf(gf_s[ap]))
                for t in range(n_pre):
                    u_s[t][ap] = u[128 * t:128 * (t + 1)]
                if ap == 7:
                    nyquist(un)

        wnr_cp.wait()
        wni_cp.wait()
        pl.when(fence)(b2_head)
        for j in range(16):
            w_cp(j, 0).wait()
            w_cp(j, 1).wait()
        ic_cp.start()
        if do_a:
            start_a_inputs()
        def b2_slot(t):
            ng = 128 // rg_rows
            for g in range(ng):
                filt(t, g)
                for k in range(16 // ng):
                    if t + n_pre < 4:
                        s_fwd(t + n_pre, (16 // ng) * g + k)
                    if t > 0:
                        s_inv(t - 1, (16 // ng) * g + k)

        for t in range(4):
            pl.when(flag_ref[t + 1] > 0)(functools.partial(b2_slot, t))

        def b2_tail():
            for ap in range(16):
                s_inv(3, ap)

        pl.when(fence)(b2_tail)

        def ob_cp(p):
            return pltpu.make_async_copy(ob_s.at[p], outh.at[:, p, pl.ds(1024, 1024)], sem_ob.at[p])

        def b3():
            ic_cp.wait()

            for pq in range(8 // b3_p):
                aps = range(2 * b3_p * pq, 2 * b3_p * (pq + 1))
                cc = [_dot(_bf(jnp.concatenate([v_s[ap, t] for ap in aps], axis=0)), _bf(ic_s[t]))
                      for t in range(4)]
                c0, c4 = cc[0][:, 0:128], cc[0][:, 128:256]
                c1r, c1i = cc[1][:, 0:128], cc[1][:, 128:256]
                c2r, c2i = cc[2][:, 0:128], cc[2][:, 128:256]
                c3r, c3i = cc[3][:, 0:128], cc[3][:, 128:256]
                pp, mm = c0 + c4, c0 - c4
                u1, u2, u3, u4 = c1r + c3r, c1i - c3i, c1r - c3r, c1i + c3i
                t1, t2 = (u3 - u4) * _R2, (u3 + u4) * _R2
                e0, e1, e2, e3 = pp + c2r, pp - c2r, mm - c2i, mm + c2i
                ys = [e0 + u1, e2 + t1, e1 - u2, e3 - t2, e0 - u1, e2 - t1, e1 + u2, e3 + t2]
                for k in range(b3_p):
                    p = b3_p * pq + k
                    ob_s[p] = jnp.concatenate(
                        [pltpu.pack_elementwise([y[256 * k:256 * k + 128], y[256 * k + 128:256 * k + 256]],
                                                packed_dtype=_BF16) for y in ys], axis=1)
                    ob_cp(p).start()

        if b3_at == 0 or not do_a:
            b3()

    if do_a:
        x_cp.wait()
        c_cp.wait()

        def project_units(slot, half, dst, rows):
            def split(ref):
                a = ref[slot, 0]
                b = ref[slot, 1]
                if half == 1:
                    a, b = a >> 16, b >> 16
                return _bf(pltpu.pack_elementwise([a, b], packed_dtype=jnp.uint16))

            wq = split(wq_s)
            wkv = jnp.concatenate([split(wk_s), split(wv_s)], axis=1)

            def q_unit(r0):
                q = _dot(_bf(x_s[pl.ds(r0 // 2, rows // 2), :]), wq) * _QSCALE
                _st(dst.at[pl.ds(r0 // 2, rows // 2), pl.ds(0, 128)], q, 'a')

            def kv_unit(r0):
                kv = _dot(_bf(c_s[pl.ds(r0 // 2, rows // 2), :]), wkv)
                _st(dst.at[pl.ds(r0 // 2, rows // 2), pl.ds(128, 256)], kv, 'a')

            units = []
            for r0 in range(0, S, rows):
                units.append(functools.partial(kv_unit, r0))
                units.append(functools.partial(q_unit, r0))
            return units

        def attend(p, t, src, fillers, bq=bq, sorder=sorder, last_cfg=last_cfg, afence=afence, chain=chain, b1_pipe=b1_pipe, b1_grp=b1_grp, orows=orows):
            head = (_HeadWide if wide else _Head)(*[_bf(src[:, pl.ds(128 * i, 128)]) for i in range(3)], bq)
            ns = S // bq
            fillers = list(fillers)
            nslots = ns * fill_slots
            total = len(fillers)
            slot = [0]

            def fill():
                slot[0] += 1
                while fillers and (total - len(fillers)) * nslots < total * slot[0]:
                    fillers.pop(0)()

            order = list(range(ns))
            if sorder == 1:
                order = order[::-1]
            elif sorder == 2:
                order = [order[-1 - n // 2] if n % 2 == 0 else order[n // 2] for n in range(ns)]
            elif sorder == 3:
                order = [order[n // 2] if n % 2 == 0 else order[-1 - n // 2] for n in range(ns)]
            for n in range(min(lookahead, ns)):
                head.qk(order[n])
            for n in range(ns):
                if n + lookahead < ns:
                    head.qk(order[n + lookahead])
                if fill_slots == 2:
                    fill()
                i = order[n]
                _st(ctx_s.at[p, pl.ds(i * bq // 2, bq // 2), pl.ds(t * 128, 128)], head.pv(i), 'a')
                fill()
            while fillers:
                fillers.pop(0)()

        npair = H // 2
        for cp in pair_cps(0, 0):
            cp.wait()
        for u in project_units(0, 0, qkv0_s, 2048):
            u()

        def pair_step(p, last):
            s0 = p % 3
            attend(p, 0, qkv0_s, project_units(s0, 1, qkv1_s, frows))
            if last:
                attend(p, 1, qkv1_s, [], *last_cfg)
            else:
                attend(p, 1, qkv1_s, project_units((p + 1) % 3, 0, qkv0_s, frows))

        def a_body(p, carry):
            for cp in pair_cps(p + 1, (p + 1) % 3):
                cp.wait()

            @pl.when(p + 2 < npair)
            def _():
                for cp in pair_cps(p + 2, (p + 2) % 3):
                    cp.start()

            @pl.when(p == 2)
            def _():
                wo_cp.start()

            if afence:
                pl.when(fence)(lambda: pair_step(p, False))
            else:
                pair_step(p, False)
            return carry

        jax.lax.fori_loop(0, npair - 1, a_body, 0)
        if b3_at == 1 and do_b:
            b3()
        pair_step(npair - 1, True)
        if b3_at == 2 and do_b:
            b3()

        wo_cp.wait()

        def oa_cp(i):
            return pltpu.make_async_copy(oa_s.at[i], outh.at[pl.ds(orows // 16 * i, orows // 16), :, pl.ds(0, 1024)],
                                         sem_oa.at[i])

        def o_body(i, carry):
            r0 = pl.multiple_of(i * (orows // 2), orows // 2)
            lhs = _bf(jnp.concatenate([ctx_s[p, pl.ds(r0, orows // 2), :] for p in range(H // 2)], axis=1))
            res = _dot(lhs, _bf(wo_s[...]))
            oa_s[i] = _pk(res).reshape(orows // 16, 8, M)
            oa_cp(i).start()
            return carry

        jax.lax.fori_loop(0, S // orows, o_body, 0)
        for i in range(S // orows):
            oa_cp(i).wait()

    if do_b:
        for p in range(8):
            ob_cp(p).wait()


def _run(A_x, A_c_kv, A_w_q, A_w_uk, A_w_uv, A_w_o, B_x, B_w_r, B_w_i, *, bq=256, do_a=True, do_b=True, rg_rows=8, n_pre=3, frows=128, fill_slots=2, lookahead=1, dbg=0, wide=True, bx_win=3, w_at=5, b3_at=0, b3_p=2, sorder=2, last_cfg=(128, 0), pad=8, cp=dict(disable_bounds_checks=True, disable_semaphore_checks=True), afence=0, chain=0, b1_pipe=0, b1_grp=1, orows=256, sta=0, stb=0, flags=None):
    _STMODE['a'], _STMODE['b'] = sta, stb
    any_spec = pl.BlockSpec(memory_space=pltpu.HBM)
    vm = pltpu.VMEM
    dma = pltpu.SemaphoreType.DMA
    scratch = [
        vm((pad, 128), _U32),
        vm((1024, 1024), _U32),
        vm((1024, 512), _U32),
        vm((2048, 1024), _U32),
        vm((3, 2, 512, 128), _U32),
        vm((3, 2, 256, 128), _U32),
        vm((3, 2, 256, 128), _U32),
        vm((1024, 384), _U32), vm((1024, 384), _U32),
        vm((16, 1024, 256), _U32),
        vm((S // orows, orows // 16, 8, 1024), _U32),
        vm((8, 2, 64, 1024), _U32),
        vm((17, 256, 128), _U32),
        vm((17, 256, 128), _U32),
        vm((1, 2048), _BF16),
        vm((1, 2048), _BF16),
        vm((4, 128, 256), _U32),
        vm((4, 128, 256), _U32),
        vm((288, 128), _F32),
        vm((16, 128, 256), _U32),
        vm((16, 4, 64, 256), _U32),
        vm((8, 2048), _U32),
        vm((16, 4, 64, 256), _U32),
        vm((8, 128, 1024), _U32),
        vm((17, 128, 256), _F32), vm((17, 128, 256), _F32), vm((17, 128, 256), _F32), vm((17, 128, 256), _F32),
        *([vm((16, 128, 256), _F32)] * 2 if rg_rows == 8 else [vm((16, 64, 256), _U32)] * 2),
        vm((16, 128, 128), _F32),
        dma((16,)), dma((9,)), dma((32,)), dma((18,)), dma((8,)), dma((S // orows,)),
    ]
    out = pl.pallas_call(
        functools.partial(_kernel, bq=bq, do_a=do_a, do_b=do_b, rg_rows=rg_rows, n_pre=n_pre, frows=frows, fill_slots=fill_slots, lookahead=lookahead, dbg=dbg, wide=wide, bx_win=bx_win, w_at=w_at, b3_at=b3_at, b3_p=b3_p, sorder=sorder, last_cfg=last_cfg, afence=afence, chain=chain, b1_pipe=b1_pipe, b1_grp=b1_grp, orows=orows),
        out_shape=jax.ShapeDtypeStruct((128, 16, 2048), _BF16),
        in_specs=[pl.BlockSpec(memory_space=pltpu.SMEM)] + [any_spec] * 12,
        out_specs=any_spec,
        scratch_shapes=scratch,
        compiler_params=pltpu.CompilerParams(vmem_limit_bytes=112 * 1024 * 1024, flags=flags, **(cp or {})),
    )(jnp.asarray(np.arange(1, 9, dtype=np.int32)), *[pltpu.with_memory_space_constraint(a, pltpu.HBM) for a in (
        A_x.reshape(S, M), A_c_kv.reshape(S, DC),
        A_w_q.reshape(512, 64, HD), A_w_uk.reshape(256, 64, HD), A_w_uv.reshape(256, 64, HD),
        A_w_o.reshape(H * HD, M),
        B_x.reshape(64, 32, BD), B_w_r.T, B_w_i.T,
        jnp.asarray(_FC), jnp.asarray(_IC_NAT if rg_rows == 8 else _IC), jnp.asarray(_GT),
    )])
    return out.reshape(1, S, 2048)


@jax.jit
def pallas_concat_heads__compressed_kv_cla__spectral_gfnet__prompt_kernel(
    A_x: jax.Array,
    A_c_kv: jax.Array,
    A_w_q: jax.Array,
    A_w_uk: jax.Array,
    A_w_uv: jax.Array,
    A_w_o: jax.Array,
    B_x: jax.Array,
    B_w_r: jax.Array,
    B_w_i: jax.Array,
):
    return _run(A_x, A_c_kv, A_w_q, A_w_uk, A_w_uv, A_w_o, B_x, B_w_r, B_w_i)
```

```python
import functools

import numpy as np
import jax
import jax.numpy as jnp
import jax.experimental.pallas as pl
import jax.experimental.pallas.tpu as pltpu

S = 2048
M = 1024
H = 32
HD = 128
DC = 512
BD = 1024

_U32 = jnp.uint32
_BF16 = jnp.bfloat16
_F32 = jnp.float32
_NT = (((1,), (1,)), ((), ()))
_QSCALE = float(HD ** -0.5 * np.log2(np.e))
_MASKED = -1e9


def _to_bf16_bits(a):
    u = np.ascontiguousarray(a, dtype=np.float32).view(np.uint32).astype(np.uint64)
    r = (u + 0x7FFF + ((u >> 16) & 1)) >> 16
    return r.astype(np.uint32) & 0xFFFF


def _pack_rows(a):
    b = _to_bf16_bits(a)
    return (b[0::2] | (b[1::2] << 16)).astype(np.uint32)


def _neg(p):
    return None if p is None else (-p[0], p[1])


def _add(p, q):
    if p is None:
        return q
    if q is None:
        return p
    if p[0] == q[0]:
        return (p[0], p[1] + q[1])
    if p[0] > 0:
        return (1, p[1] - q[1])
    return (1, q[1] - p[1])


def _sub(p, q):
    return _add(p, _neg(q))


def _scale(p, f):
    if p is None:
        return None
    return (p[0] * (1 if f > 0 else -1), p[1] * abs(f))


def _cadd(x, y):
    return (_add(x[0], y[0]), _add(x[1], y[1]))


def _csub(x, y):
    return (_sub(x[0], y[0]), _sub(x[1], y[1]))


def _cmul_i(x, s):
    return (_neg(x[1]), x[0]) if s > 0 else (x[1], _neg(x[0]))


def _cmul_w(x, n, sgn):
    n = n % 16
    if n == 0:
        return x
    if n == 4:
        return _cmul_i(x, sgn)
    if n == 8:
        return (_neg(x[0]), _neg(x[1]))
    if n == 12:
        return _cmul_i(x, -sgn)
    wr = float(np.cos(2 * np.pi * n / 16))
    wi = float(sgn * np.sin(2 * np.pi * n / 16))
    re, im = x
    if n % 2 == 0:
        r = abs(wr)
        sr = 1 if wr > 0 else -1
        si = 1 if wi > 0 else -1
        a = _sub(re if sr > 0 else _neg(re), im if si > 0 else _neg(im))
        b = _add(re if si > 0 else _neg(re), im if sr > 0 else _neg(im))
        return (_scale(a, r), _scale(b, r))
    return (_sub(_scale(re, wr), _scale(im, wi)), _add(_scale(re, wi), _scale(im, wr)))


def _dft4(x0, x1, x2, x3, sgn):
    s02, d02 = _cadd(x0, x2), _csub(x0, x2)
    s13, d13 = _cadd(x1, x3), _csub(x1, x3)
    r = _cmul_i(d13, sgn)
    return [_cadd(s02, s13), _cadd(d02, r), _csub(s02, s13), _csub(d02, r)]


def _fft16(xs, sgn):
    t = [_dft4(xs[a0], xs[4 + a0], xs[8 + a0], xs[12 + a0], sgn) for a0 in range(4)]
    t = [[_cmul_w(t[a0][j0], a0 * j0, sgn) for j0 in range(4)] for a0 in range(4)]
    out = [None] * 16
    for j0 in range(4):
        r = _dft4(t[0][j0], t[1][j0], t[2][j0], t[3][j0], sgn)
        for j1 in range(4):
            out[j0 + 4 * j1] = r[j1]
    return out


_CLS = ((0, 4), (1, 7), (2, 6), (3, 5))
_R2 = float(np.sqrt(0.5))


def _build_consts():
    n2 = np.arange(128)
    kap = np.arange(64)

    def wl(l):
        return np.exp(-2j * np.pi * np.outer(l, n2) / 1024)

    fc = np.zeros((4, 256, 256))
    w = wl(8 * kap)
    fc[0, 0:64, 0:128] = w.real
    fc[0, 64:128, 0:128] = w.imag
    fc[0, 64, 0:128] = (-1.0) ** n2
    w = wl(4 + 8 * kap)
    fc[0, 0:64, 128:256] = w.real
    fc[0, 64:128, 128:256] = w.imag
    for j in (1, 2, 3):
        si = 1.0 if j == 3 else -1.0
        w1, w2 = wl(j + 8 * kap), wl(8 - j + 8 * kap)
        fc[j, 0:64, 0:128], fc[j, 0:64, 128:] = w1.real, -w1.imag * si
        fc[j, 64:128, 0:128], fc[j, 64:128, 128:] = w2.real, w2.imag * si
        fc[j, 128:192, 0:128], fc[j, 128:192, 128:] = w1.imag, w1.real * si
        fc[j, 192:256, 0:128], fc[j, 192:256, 128:] = w2.imag, -w2.real * si

    def cs(l, c):
        ph = 2 * np.pi * np.outer(l, n2) / 1024
        return c[:, None] * np.cos(ph) / 1024, c[:, None] * np.sin(ph) / 1024

    ic = np.zeros((4, 256, 256))
    two = np.full(64, 2.0)
    co, si = cs(8 * kap, np.where(kap == 0, 1.0, 2.0))
    ic[0, 0:64, 0:128], ic[0, 128:192, 0:128] = co, -si
    ic[0, 128, 0:128] = (-1.0) ** n2 / 1024
    co, si = cs(4 + 8 * kap, two)
    ic[0, 64:128, 128:], ic[0, 192:256, 128:] = co, -si
    for j in (1, 2, 3):
        co, si = cs(j + 8 * kap, two)
        ic[j, 0:64, 0:128], ic[j, 128:192, 0:128] = co, -si
        ic[j, 0:64, 128:], ic[j, 128:192, 128:] = si, co
        co, si = cs(8 - j + 8 * kap, two)
        ic[j, 64:128, 0:128], ic[j, 192:256, 0:128] = co, -si
        ic[j, 64:128, 128:], ic[j, 192:256, 128:] = -si, -co

    f128 = np.exp(-2j * np.pi * np.outer(n2, n2) / 128)
    tw = np.exp(-2j * np.pi * np.outer(np.arange(16), n2) / 2048)

    def even_odd(m, blk):
        r = m.reshape(-1, blk // 2, 2, m.shape[-1])
        return np.concatenate([r[:, :, 0], r[:, :, 1]], axis=1).reshape(m.shape)

    fc[0] = even_odd(fc[0], 64)
    for j in (1, 2, 3):
        fc[j] = even_odd(fc[j], 128)
    sigma = np.concatenate([np.arange(0, 128, 2), np.arange(1, 128, 2)])
    fpos = f128[sigma]
    gt = np.concatenate([fpos[0::2].real, fpos[1::2].real, fpos[0::2].imag, fpos[1::2].imag,
                         tw.real, tw.imag], axis=0).astype(np.float32)

    def pk(m):
        return np.stack([_pack_rows(x) for x in m])

    return pk(fc), pk(ic / 2048), gt


_FC, _IC, _GT = _build_consts()


def _bf(x_u32):
    return pltpu.bitcast(x_u32, _BF16)


def _pk(x_f32):
    return pltpu.bitcast(x_f32.astype(_BF16), _U32)


def _pk2(x_f32):
    r = x_f32.shape[0] // 2
    return pltpu.pack_elementwise([x_f32[:r], x_f32[r:]], packed_dtype=_BF16)


def _dot(a, b):
    return jnp.dot(a, b, preferred_element_type=_F32)


def _dot_nt(a, b):
    return jax.lax.dot_general(a, b, _NT, preferred_element_type=_F32)


class _Head:
    def __init__(self, q, k, v, bq):
        self.q, self.k, self.v, self.bq = q, k, v, bq
        self.state = {}
        row = jax.lax.broadcasted_iota(jnp.int32, (128, 128), 0)
        col = jax.lax.broadcasted_iota(jnp.int32, (128, 128), 1)
        self.causal = col <= row

    def _cols(self, i, r):
        q0 = i * self.bq
        return (0, q0 + 128) if r == 0 else (q0 + 128 * r, q0 + 128 * (r + 1))

    def qk(self, i):
        bq = self.bq
        q0 = i * bq
        parts = []
        for r in range(bq // 128):
            c0, c1 = self._cols(i, r)
            s = _dot_nt(self.q[q0 + 128 * r:q0 + bq], self.k[c0:c1])
            w = c1 - c0
            top = jnp.where(self.causal, s[:128, w - 128:], _MASKED)
            if w > 128:
                top = jnp.concatenate([s[:128, :w - 128], top], axis=1)
            parts.append(jnp.concatenate([top, s[128:]], axis=0) if s.shape[0] > 128 else top)
        mx = jnp.max(parts[0], axis=1, keepdims=True)
        for r in range(1, bq // 128):
            mr = jnp.max(parts[r], axis=1, keepdims=True)
            mx = jnp.concatenate([mx[:128 * r], jnp.maximum(mx[128 * r:], mr)], axis=0)
        self.state[i] = (parts, mx)

    def pv(self, i):
        parts, m = self.state.pop(i)
        acc = l = None
        for r, s in enumerate(parts):
            c0, c1 = self._cols(i, r)
            p = jnp.exp2(s - m[128 * r:])
            lr = jnp.sum(p, axis=1, keepdims=True)
            o = _dot(p.astype(_BF16), self.v[c0:c1])
            if r == 0:
                acc, l = o, lr
            else:
                acc = jnp.concatenate([acc[:128 * r], acc[128 * r:] + o], axis=0)
                l = jnp.concatenate([l[:128 * r], l[128 * r:] + lr], axis=0)
        rc = pl.reciprocal(l, approx=True)
        rc = rc * (2.0 - l * rc)
        return acc * rc


_BQ = 256
_FROWS = 128
_NPRE = 3
_BX_WIN = 3
_W_AT = 5
_OROWS = 256


def _kernel(flag_ref, x_hbm, c_hbm, wq_hbm, wk_hbm, wv_hbm, wo_hbm, bx_hbm, wr_hbm, wi_hbm,
            fc_hbm, ic_hbm, gt_hbm,
            out_hbm,
            x_s, c_s, wo_s, wq_s, wk_s, wv_s, qkv0_s, qkv1_s, ctx_s, oa_s,
            bx_s, wr_s, wi_s, wnr_s, wni_s, fc_s, ic_s, gt_s, gf_s, x1_s, nq_s, v_s, ob_s,
            u0_s, u1_s, u2_s, u3_s, q0_s, q1_s, vc_s,
            sem_bx, sem_misc, sem_w, sem_pair, sem_ob, sem_oa):
    xh = x_hbm.bitcast(_U32)
    ch = c_hbm.bitcast(_U32)
    wqh = wq_hbm.bitcast(_U32)
    wkh = wk_hbm.bitcast(_U32)
    wvh = wv_hbm.bitcast(_U32)
    woh = wo_hbm.bitcast(_U32)
    bxh = bx_hbm.bitcast(_U32)
    wrh = wr_hbm.at[pl.ds(0, 512)].bitcast(_U32)
    wih = wi_hbm.at[pl.ds(0, 512)].bitcast(_U32)
    outh = out_hbm.bitcast(_U32)

    def bx_cp(p, par):
        return pltpu.make_async_copy(bxh.at[:, par * 8 + p], bx_s.at[p, par], sem_bx.at[2 * p + par])

    def w_cp(j, which):
        src, dst = (wrh, wr_s) if which == 0 else (wih, wi_s)
        return pltpu.make_async_copy(src.at[:, pl.ds(128 * j, 128)], dst.at[j], sem_w.at[2 * j + which])

    def pair_cps(pair, slot):
        cps = []
        for i, (src, dst) in enumerate(((wqh, wq_s), (wkh, wk_s), (wvh, wv_s))):
            for par in range(2):
                cps.append(pltpu.make_async_copy(
                    src.at[:, par * 16 + pair], dst.at[slot, par], sem_pair.at[slot * 6 + 2 * i + par]))
        return cps

    def ob_cp(p):
        return pltpu.make_async_copy(ob_s.at[p], outh.at[:, p, pl.ds(1024, 1024)], sem_ob.at[p])

    def oa_cp(i):
        rows = pl.ds(_OROWS // 16 * i, _OROWS // 16)
        return pltpu.make_async_copy(oa_s.at[i], outh.at[rows, :, pl.ds(0, 1024)], sem_oa.at[i])

    fc_cp = pltpu.make_async_copy(fc_hbm, fc_s, sem_misc.at[0])
    ic_cp = pltpu.make_async_copy(ic_hbm, ic_s, sem_misc.at[1])
    wnr_cp = pltpu.make_async_copy(wr_hbm.at[pl.ds(512, 1)], wnr_s, sem_misc.at[2])
    gt_cp = pltpu.make_async_copy(gt_hbm, gt_s, sem_misc.at[3])
    wni_cp = pltpu.make_async_copy(wi_hbm.at[pl.ds(512, 1)], wni_s, sem_misc.at[4])
    x_cp = pltpu.make_async_copy(xh, x_s, sem_misc.at[5])
    c_cp = pltpu.make_async_copy(ch, c_s, sem_misc.at[6])
    wo_cp = pltpu.make_async_copy(woh, wo_s, sem_misc.at[7])

    gt_cp.start()
    fc_cp.start()
    for p in range(_BX_WIN):
        bx_cp(p, 0).start()
        bx_cp(p, 1).start()
    wnr_cp.start()
    wni_cp.start()

    def fenced(i, fn):
        pl.when(flag_ref[i] > 0)(fn)

    lane0 = jax.lax.broadcasted_iota(jnp.int32, (1, 128), 1) == 0
    row0 = jax.lax.broadcasted_iota(jnp.int32, (8, 128), 0) == 0

    gt_cp.wait()
    f_r, f_i = gt_s[pl.ds(0, 128), :], gt_s[pl.ds(128, 128), :]
    for ap in range(16):
        t_r, t_i = gt_s[pl.ds(256 + ap, 1), :], gt_s[pl.ds(272 + ap, 1), :]
        g_r = _pk2(f_r * t_r - f_i * t_i)
        g_i = _pk2(f_r * t_i + f_i * t_r)
        gf_s[ap] = jnp.concatenate([jnp.concatenate([g_r, g_i], axis=1),
                                    jnp.concatenate([g_i ^ jnp.uint32(0x80008000), g_r], axis=1)], axis=0)

    fc_cp.wait()
    for p in range(8):
        bx_cp(p, 0).wait()
        bx_cp(p, 1).wait()
        if p + _BX_WIN < 8:
            bx_cp(p + _BX_WIN, 0).start()
            bx_cp(p + _BX_WIN, 1).start()
        if p == _W_AT:
            for j in range(16):
                w_cp(j, 0).start()
                w_cp(j, 1).start()
        planes = []
        for h in range(2):
            halves = []
            for par in range(2):
                xf = pltpu.unpack_elementwise(bx_s[p, par], index=h, packed_dtype=_BF16,
                                              unpacked_dtype=_F32)
                xs = [xf[:, 128 * n:128 * (n + 1)] for n in range(8)]
                a_, b_ = xs[0] + xs[4], xs[0] - xs[4]
                c_, d_ = xs[2] + xs[6], xs[2] - xs[6]
                e_, f_ = xs[1] + xs[5], xs[1] - xs[5]
                g_, h_ = xs[3] + xs[7], xs[3] - xs[7]
                u_ = (f_ - h_) * _R2
                v_ = (f_ + h_) * _R2
                ac, eg = a_ + c_, e_ + g_
                halves.append([ac + eg, ac - eg, b_ + u_, d_ + v_, a_ - c_, e_ - g_, b_ - u_, d_ - v_])
            planes.append([jnp.concatenate([halves[0][i], halves[1][i]], axis=0).astype(_BF16)
                           for i in range(8)])
        for h in range(2):
            pln = planes[h]
            ap = 2 * p + h
            f0 = _bf(fc_s[0, pl.ds(0, 64), :])
            o0 = _dot_nt(f0[:, 0:128], pln[0])
            o4 = _dot_nt(f0[:, 128:256], pln[1])
            nq = jnp.where(row0, o0[64:72], 0.0)
            im0 = jnp.concatenate([jnp.where(row0, 0.0, o0[64:72]), o0[72:128]], axis=0)
            nq_s[:, pl.ds(128 * ap, 128)] = _pk2(jnp.concatenate([nq, jnp.zeros_like(nq)], axis=0))
            x1_s[ap, 0] = jnp.concatenate(
                [jnp.concatenate([_pk2(o0[0:64]), _pk2(o4[0:64])], axis=0),
                 jnp.concatenate([_pk2(im0), _pk2(o4[64:128])], axis=0)], axis=1)
            for j in (1, 2, 3):
                o = _dot_nt(_bf(fc_s[j]), jnp.concatenate([pln[2 * j], pln[2 * j + 1]], axis=1))
                x1_s[ap, j] = jnp.concatenate([_pk2(o[0:128]), _pk2(o[128:256])], axis=1)

    u_s, q_s = (u0_s, u1_s, u2_s, u3_s), (q0_s, q1_s)

    def spectral(us, w_of):
        xs = _fft16(us, -1)
        qs = []
        for j in range(16):
            (sr, xr), (si, xi) = xs[j]
            wr, wi = w_of(j)
            qs.append((_sub((sr, xr * wr), (si, xi * wi)), _add((sr, xr * wi), (si, xi * wr))))
        res = _fft16(qs, +1)
        assert all(r[0][0] == 1 and r[1][0] == 1 for r in res)
        return [(r[0][1], r[1][1]) for r in res]

    def s_fwd(t, ap):
        u_s[t][ap] = _dot(_bf(x1_s[ap, t]), _bf(gf_s[ap]))

    def filt(t, g):
        r0 = 8 * g
        cls = _CLS[t][r0 // 64]
        rows = pl.ds(r0, 8)
        wrows = pl.ds(cls // 2 + 4 * (r0 % 64), 8, stride=4)

        def w_of(j):
            return tuple(pltpu.unpack_elementwise(ws[j, wrows, :], index=cls % 2, packed_dtype=_BF16,
                                                  unpacked_dtype=_F32) for ws in (wr_s, wi_s))

        res = spectral([((1, u_s[t][ap, rows, pl.ds(0, 128)]), (1, u_s[t][ap, rows, pl.ds(128, 128)]))
                        for ap in range(16)], w_of)
        for ap in range(16):
            q_s[t % 2][ap, rows, :] = jnp.concatenate([res[ap][0], res[ap][1]], axis=1)

    def s_inv(t, ap):
        o = _dot_nt(_bf(gf_s[ap]), q_s[t % 2][ap].astype(_BF16))
        vi = o[128:256]
        if t == 0:
            vi = jnp.where(lane0, vc_s[ap], vi)
        v_s[ap, t] = jnp.concatenate([_pk2(o[0:128]), _pk2(vi)], axis=1)

    def nyquist(un):
        wnr = wnr_s[...].astype(_F32)
        wni = wni_s[...].astype(_F32)
        qn = spectral([((1, u[:, 0:128]), (1, u[:, 128:256])) for u in un],
                      lambda j: (wnr[:, 128 * j:128 * (j + 1)], wni[:, 128 * j:128 * (j + 1)]))
        for ap in range(16):
            lhs = jnp.concatenate([qn[ap][0], qn[ap][1]], axis=1).astype(_BF16)
            vn = _dot_nt(lhs, _bf(gf_s[ap, pl.ds(0, 64), :]))
            vn = jnp.concatenate([vn, jnp.zeros((112, 128), _F32)], axis=0)
            vc_s[ap] = vn.T

    def b2_head():
        un = [_dot(_bf(nq_s[:, pl.ds(128 * ap, 128)]), _bf(gf_s[ap, pl.ds(0, 64), :])) for ap in range(16)]
        for ap in range(16):
            u = _dot(_bf(x1_s[ap, 0:_NPRE].reshape(64 * _NPRE, 256)), _bf(gf_s[ap]))
            for t in range(_NPRE):
                u_s[t][ap] = u[128 * t:128 * (t + 1)]
            if ap == 7:
                nyquist(un)

    def b2_slot(t):
        for g in range(16):
            filt(t, g)
            if t + _NPRE < 4:
                s_fwd(t + _NPRE, g)
            if t > 0:
                s_inv(t - 1, g)

    def b2_tail():
        for ap in range(16):
            s_inv(3, ap)

    wnr_cp.wait()
    wni_cp.wait()
    fenced(0, b2_head)
    for j in range(16):
        w_cp(j, 0).wait()
        w_cp(j, 1).wait()
    ic_cp.start()
    x_cp.start()
    c_cp.start()
    for cp in pair_cps(0, 0) + pair_cps(1, 1):
        cp.start()
    for t in range(4):
        fenced(t + 1, functools.partial(b2_slot, t))
    fenced(0, b2_tail)

    ic_cp.wait()
    for pq in range(4):
        aps = range(4 * pq, 4 * pq + 4)
        cc = [_dot(_bf(jnp.concatenate([v_s[ap, t] for ap in aps], axis=0)), _bf(ic_s[t]))
              for t in range(4)]
        c0, c4 = cc[0][:, 0:128], cc[0][:, 128:256]
        c1r, c1i = cc[1][:, 0:128], cc[1][:, 128:256]
        c2r, c2i = cc[2][:, 0:128], cc[2][:, 128:256]
        c3r, c3i = cc[3][:, 0:128], cc[3][:, 128:256]
        pp, mm = c0 + c4, c0 - c4
        u1, u2, u3, u4 = c1r + c3r, c1i - c3i, c1r - c3r, c1i + c3i
        t1, t2 = (u3 - u4) * _R2, (u3 + u4) * _R2
        e0, e1, e2, e3 = pp + c2r, pp - c2r, mm - c2i, mm + c2i
        ys = [e0 + u1, e2 + t1, e1 - u2, e3 - t2, e0 - u1, e2 - t1, e1 + u2, e3 + t2]
        for k in range(2):
            p = 2 * pq + k
            ob_s[p] = jnp.concatenate(
                [pltpu.pack_elementwise([y[256 * k:256 * k + 128], y[256 * k + 128:256 * k + 256]],
                                        packed_dtype=_BF16) for y in ys], axis=1)
            ob_cp(p).start()

    def project_units(slot, half, dst, rows):
        def split(ref):
            a = ref[slot, 0]
            b = ref[slot, 1]
            if half == 1:
                a, b = a >> 16, b >> 16
            return _bf(pltpu.pack_elementwise([a, b], packed_dtype=jnp.uint16))

        wq = split(wq_s)
        wkv = jnp.concatenate([split(wk_s), split(wv_s)], axis=1)

        def q_unit(r0):
            rr = pl.ds(r0 // 2, rows // 2)
            dst[rr, pl.ds(0, 128)] = _pk(_dot(_bf(x_s[rr, :]), wq) * _QSCALE)

        def kv_unit(r0):
            rr = pl.ds(r0 // 2, rows // 2)
            dst[rr, pl.ds(128, 256)] = _pk(_dot(_bf(c_s[rr, :]), wkv))

        units = []
        for r0 in range(0, S, rows):
            units.append(functools.partial(kv_unit, r0))
            units.append(functools.partial(q_unit, r0))
        return units

    def attend(p, t, src, fillers, bq=_BQ):
        head = _Head(*[_bf(src[:, pl.ds(128 * i, 128)]) for i in range(3)], bq)
        ns = S // bq
        fillers = list(fillers)
        nslots = 2 * ns
        total = len(fillers)
        slot = [0]

        def fill():
            slot[0] += 1
            while fillers and (total - len(fillers)) * nslots < total * slot[0]:
                fillers.pop(0)()

        order = list(range(ns))
        if fillers:
            order = [order[-1 - n // 2] if n % 2 == 0 else order[n // 2] for n in range(ns)]
        head.qk(order[0])
        for n, i in enumerate(order):
            if n + 1 < ns:
                head.qk(order[n + 1])
            fill()
            ctx_s[p, pl.ds(i * bq // 2, bq // 2), pl.ds(t * 128, 128)] = _pk(head.pv(i))
            fill()
        while fillers:
            fillers.pop(0)()

    npair = H // 2
    x_cp.wait()
    c_cp.wait()
    for cp in pair_cps(0, 0):
        cp.wait()
    for u in project_units(0, 0, qkv0_s, S):
        u()

    def pair_step(p, last):
        attend(p, 0, qkv0_s, project_units(p % 3, 1, qkv1_s, _FROWS))
        if last:
            attend(p, 1, qkv1_s, [], bq=128)
        else:
            attend(p, 1, qkv1_s, project_units((p + 1) % 3, 0, qkv0_s, _FROWS))

    def a_body(p, carry):
        for cp in pair_cps(p + 1, (p + 1) % 3):
            cp.wait()

        @pl.when(p + 2 < npair)
        def _():
            for cp in pair_cps(p + 2, (p + 2) % 3):
                cp.start()

        @pl.when(p == 2)
        def _():
            wo_cp.start()

        pair_step(p, False)
        return carry

    jax.lax.fori_loop(0, npair - 1, a_body, 0)
    pair_step(npair - 1, True)

    wo_cp.wait()

    def o_body(i, carry):
        r0 = pl.multiple_of(i * (_OROWS // 2), _OROWS // 2)
        lhs = _bf(jnp.concatenate([ctx_s[p, pl.ds(r0, _OROWS // 2), :] for p in range(npair)], axis=1))
        oa_s[i] = _pk(_dot(lhs, _bf(wo_s[...]))).reshape(_OROWS // 16, 8, M)
        oa_cp(i).start()
        return carry

    jax.lax.fori_loop(0, S // _OROWS, o_body, 0)
    for i in range(S // _OROWS):
        oa_cp(i).wait()
    for p in range(8):
        ob_cp(p).wait()


@jax.jit
def pallas_concat_heads__compressed_kv_cla__spectral_gfnet__prompt_kernel(
    A_x: jax.Array,
    A_c_kv: jax.Array,
    A_w_q: jax.Array,
    A_w_uk: jax.Array,
    A_w_uv: jax.Array,
    A_w_o: jax.Array,
    B_x: jax.Array,
    B_w_r: jax.Array,
    B_w_i: jax.Array,
):
    hbm = pl.BlockSpec(memory_space=pltpu.HBM)
    vm = pltpu.VMEM
    dma = pltpu.SemaphoreType.DMA
    scratch = [
        vm((1024, 1024), _U32),
        vm((1024, 512), _U32),
        vm((2048, 1024), _U32),
        vm((3, 2, 512, 128), _U32),
        vm((3, 2, 256, 128), _U32),
        vm((3, 2, 256, 128), _U32),
        vm((1024, 384), _U32),
        vm((1024, 384), _U32),
        vm((16, 1024, 256), _U32),
        vm((S // _OROWS, _OROWS // 16, 8, 1024), _U32),
        vm((8, 2, 64, 1024), _U32),
        vm((16, 256, 128), _U32),
        vm((16, 256, 128), _U32),
        vm((1, 2048), _BF16),
        vm((1, 2048), _BF16),
        vm((4, 128, 256), _U32),
        vm((4, 128, 256), _U32),
        vm((288, 128), _F32),
        vm((16, 128, 256), _U32),
        vm((16, 4, 64, 256), _U32),
        vm((8, 2048), _U32),
        vm((16, 4, 64, 256), _U32),
        vm((8, 128, 1024), _U32),
        *[vm((16, 128, 256), _F32)] * 6,
        vm((16, 128, 128), _F32),
        dma((16,)), dma((8,)), dma((32,)), dma((18,)), dma((8,)), dma((S // _OROWS,)),
    ]
    out = pl.pallas_call(
        _kernel,
        out_shape=jax.ShapeDtypeStruct((128, 16, 2048), _BF16),
        in_specs=[pl.BlockSpec(memory_space=pltpu.SMEM)] + [hbm] * 12,
        out_specs=hbm,
        scratch_shapes=scratch,
        compiler_params=pltpu.CompilerParams(vmem_limit_bytes=112 * 1024 * 1024,
                                             disable_bounds_checks=True, disable_semaphore_checks=True),
    )(
        np.arange(1, 9, dtype=np.int32),
        A_x.reshape(S, M), A_c_kv.reshape(S, DC),
        A_w_q.reshape(512, 64, HD), A_w_uk.reshape(256, 64, HD), A_w_uv.reshape(256, 64, HD),
        A_w_o.reshape(H * HD, M),
        B_x.reshape(64, 32, BD), B_w_r.T, B_w_i.T,
        _FC, _IC, _GT,
    )
    return out.reshape(1, S, 2048)
```
